```python
import os as _os
_os.environ.setdefault("JAX_PLATFORMS", "cpu")
import jax
import jax.numpy as jnp

def _softmax(x, axis=-1):
    return jax.nn.softmax(x, axis=axis)
def _gelu(x):
    return jax.nn.gelu(x, approximate=True)
def _silu(x):
    return jax.nn.silu(x)
def _sigmoid(x):
    return jax.nn.sigmoid(x)
def _layernorm(x, axis=-1, eps=1e-5):
    m = jnp.mean(x, axis=axis, keepdims=True)
    v = jnp.var(x, axis=axis, keepdims=True)
    return (x - m) / jnp.sqrt(v + eps)
def _scatter_add(tgt, idx, src, axis=0):
    return tgt.at[idx].add(src)
def _segment_sum(src, seg, n):
    return jax.ops.segment_sum(src, seg, n)
class _Rng:
    def __init__(self, key):
        self._k = key
    def _next(self):
        self._k, sub = jax.random.split(self._k)
        return sub
    def normal(self, shape):
        return jax.random.normal(self._next(), shape, dtype=jnp.bfloat16)
    def randint(self, lo, hi, shape):
        return jax.random.randint(self._next(), shape, lo, hi, dtype=jnp.int32)
    def uniform(self, shape, lo=0.0, hi=1.0):
        return jax.random.uniform(self._next(), shape, jnp.bfloat16, lo, hi)
    def permutation(self, n):
        return jax.random.permutation(self._next(), n)


kernel_name = 'concat_heads__linear_attn_block__ssm_conv_s4__prompt'

def setup_inputs():
    _rng = _Rng(jax.random.key(int.from_bytes(__import__("os").urandom(4), "little")))
    _w = (lambda a: (lambda t: t.astype(jnp.bfloat16) if jnp.issubdtype(t.dtype, jnp.floating) else t)(jnp.asarray(a)))
    def _A_setup():
        B, S, D = 1, 2048, 512
        return {
            "x": _w((lambda *s: _rng.normal(s) * 0.05)(B, S, D)),
            "wqkv": _w((lambda *s: _rng.normal(s) * 0.8)(D, 3 * D)),
            "wo": _w((lambda *s: _rng.normal(s) * 0.05)(D, D)),
        }
    _A_in = _A_setup()

    def _B_setup():
        B, L, D, N = 1, 2048, 512, 128
        A_re = -jnp.exp((lambda *s: _rng.normal(s) * 0.2)(D, N))
        A_im = jnp.pi * (lambda *s: _rng.normal(s) * 0.2)(D, N)
        B_re = (lambda *s: _rng.normal(s) * 0.2)(D, N)
        B_im = (lambda *s: _rng.normal(s) * 0.2)(D, N)
        C_re = (lambda *s: _rng.normal(s) * 0.2)(D, N)
        C_im = (lambda *s: _rng.normal(s) * 0.2)(D, N)
        log_dt = (lambda *s: _rng.normal(s) * 0.2)(D) * 0.5 - 4.0
        Dskip = (lambda *s: _rng.normal(s) * 0.05)(D)
        return {
            "u": _w((lambda *s: _rng.normal(s) * 0.05)(B, L, D)),
            "A_re": _w(A_re),
            "A_im": _w(A_im),
            "B_re": _w(B_re),
            "B_im": _w(B_im),
            "C_re": _w(C_re),
            "C_im": _w(C_im),
            "log_dt": _w(log_dt),
            "Dskip": _w(Dskip),
        }
    _B_in = _B_setup()

    return {
        "A_x": _A_in["x"],
        "A_wqkv": _A_in["wqkv"],
        "A_wo": _A_in["wo"],
        "B_u": _B_in["u"],
        "B_A_re": _B_in["A_re"],
        "B_A_im": _B_in["A_im"],
        "B_B_re": _B_in["B_re"],
        "B_B_im": _B_in["B_im"],
        "B_C_re": _B_in["C_re"],
        "B_C_im": _B_in["C_im"],
        "B_log_dt": _B_in["log_dt"],
        "B_Dskip": _B_in["Dskip"],
    }

def reference(A_x, A_wqkv, A_wo, B_u, B_A_re, B_A_im, B_B_re, B_B_im, B_C_re, B_C_im, B_log_dt, B_Dskip):
    def _A_ref(x, wqkv, wo):
        B, S, D = x.shape
        H = 32; Dh = D // H
        qkv = (lambda x, *d: x.transpose(*d))((x @ wqkv).reshape(B, S, 3, H, Dh), 2, 0, 3, 1, 4)
        q, k, v = qkv[0], qkv[1], qkv[2]
        phi = lambda t: jnp.where(t > 0, t + 1, jnp.exp(t)) + 1e-6
        pq, pk = phi(q), phi(k)
        kv = jnp.einsum("bhsd,bhse->bhde", pk, v)
        z = jnp.einsum("bhsd->bhd", pk)
        num = jnp.einsum("bhqd,bhde->bhqe", pq, kv)
        den = jnp.einsum("bhqd,bhd->bhq", pq, z)[..., None] + 1e-6
        o = num / den
        return (lambda x, *d: x.transpose(*d))(o, 0, 2, 1, 3).reshape(B, S, D) @ wo

    def _B_ref(u, A_re, A_im, B_re, B_im, C_re, C_im, log_dt, Dskip):
        Bsz, L, D = u.shape
        dt = jnp.exp(log_dt)[:, None]
        A = A_re + 1j * A_im
        Bc = B_re + 1j * B_im
        Cc = C_re + 1j * C_im
        logdA = dt * A
        dB = dt * Bc
        l = (lambda x, dt: x.astype(dt))(jnp.arange(L), A_re.dtype)
        P = jnp.exp(logdA[:, :, None] * l[None, None, :])
        K = jnp.einsum("dn,dnl,dn->dl", Cc, P, dB).real
        L2 = 2 * L
        Kp = jnp.pad(K, ((0, 0), (0, L)))
        up = (lambda x, *d: x.transpose(*d))(u, 0, 2, 1)
        up = jnp.pad(up, ((0, 0), (0, 0), (0, L)))
        Kf = (lambda x, axes=(-2,-1): jnp.fft.rfft2(x.astype(jnp.float32), axes=axes))(Kp[:, None, :], axes=(-2, -1))
        Uf = (lambda x, axes=(-2,-1): jnp.fft.rfft2(x.astype(jnp.float32), axes=axes))(up[:, :, None, :], axes=(-2, -1))
        Yf = Uf * Kf[None, :, :, :]
        y = (lambda x, s, axes=(-2,-1): jnp.fft.irfft2(x, s=s, axes=axes).astype(jnp.bfloat16))(Yf, (1, L2), axes=(-2, -1))[:, :, 0, :L]
        y = (lambda x, *d: x.transpose(*d))(y, 0, 2, 1) + u * Dskip[None, None, :]
        return y

    a = _A_ref(A_x, A_wqkv, A_wo)
    b = _B_ref(B_u, B_A_re, B_A_im, B_B_re, B_B_im, B_C_re, B_C_im, B_log_dt, B_Dskip)
    return jnp.concatenate([a, b], axis=-1)
```

```python
import functools
import os
import numpy as np
import jax
import jax.numpy as jnp
from jax import lax
import jax.experimental.pallas as pl
import jax.experimental.pallas.tpu as pltpu

S = 2048
D = 512
F32 = jnp.float32
BF16 = jnp.bfloat16
U32 = jnp.uint32

_BASE = np.array([[1, 5], [2, 6], [3, 7], [4, 8], [258, 262], [260, 264],
                  [516, 520], [772, 776], [1032, 1288], [1544, 1800]])
_TILE_OF_CHUNK = [0, 1, 2, 2, 3, 3, 3, 3] + [4] * 8
_BCH = (0, 2, 4, 8)


def _bf16_bits(v):
    u = np.ascontiguousarray(v, np.float32).view(np.uint32)
    return ((u + 0x7FFF + ((u >> 16) & 1)) >> 16).astype(np.uint32)


def _pack_rows(v):
    b = _bf16_bits(v)
    return b[0::2] | (b[1::2] << 16)


@functools.lru_cache(maxsize=None)
def _tables():
    lr = (_bf16_bits(np.arange(S)) << 16).view(np.float32).astype(np.int64)
    val = np.zeros((5, 128), np.int64)
    for lam in range(128):
        mu, tau = 15 - (lam >> 3), lam & 7
        e, x = tau >> 1, tau & 1
        for h in range(2):
            val[h, lam] = _BASE[e, x ^ h] + 8 * (mu + 16 * h)
        hp, ab, h = tau >> 2, (tau >> 1) & 1, tau & 1
        for q in range(3):
            val[2 + q, lam] = _BASE[4 + 2 * q + ab, hp] + 8 * (mu + 16 * h)
    om = 2 * np.pi * (np.arange(128) + 0.25) / 128.0
    phase = np.exp(1j * om * 191.5)

    def stack(z):
        return np.concatenate([z.real[:64], z.imag[:64], z.real[64:], z.imag[64:]], axis=0)

    fk = []
    g = np.zeros((4, 128), np.complex128)
    g[0] = phase
    for k in range(16):
        slot = {int(v): i for i, v in enumerate(val[_TILE_OF_CHUNK[k]])}
        m = np.zeros((128, 128), np.complex128)
        for p in range(1, 129):
            lag = 128 * k + p
            if lag >= S:
                continue
            v = int(lr[lag])
            z = np.exp(-1j * om * p) * phase
            if v in slot:
                m[:, slot[v]] += z
            else:
                assert v == 128 * k and k in _BCH
                g[_BCH.index(k)] += z
        fk.append(stack(m))
    for q in (1, 2, 3):
        sel = np.zeros((16, 128))
        sel[:, list(val[q]).index(128 << q)] = 1.0
        fk.append(sel)
    fu = stack(np.exp(-1j * om[:, None] * np.arange(128)[None, :]))
    fk.append(fu)
    fk = np.concatenate(fk, axis=0)
    jj = np.arange(64)[:, None] - 63.5
    finv = np.concatenate([np.cos(om[None, :] * jj) / 128.0, -np.sin(om[None, :] * jj) / 128.0,
                           np.stack([g.real, g.imag], axis=1).reshape(8, 128)], axis=0)
    return _pack_rows(fk), finv.astype(np.float32)


FK_SEL = 4096
FK_FU = 4096 + 48
FK_ROWS = 4096 + 48 + 256


def _cmul(a, b):
    return a[0] * b[0] - a[1] * b[1], a[0] * b[1] + a[1] * b[0]


def _csq(a):
    return a[0] * a[0] - a[1] * a[1], (a[0] + a[0]) * a[1]


def _phi(t):
    return jnp.where(t > 0, t + 1.0, jnp.exp(t)) + 1e-6


def _nt(a, b):
    return lax.dot_general(a, b, (((1,), (1,)), ((), ())), preferred_element_type=F32)


def _nn(a, b):
    return jnp.dot(a, b, preferred_element_type=F32)


def _bf(v):
    return pltpu.bitcast(v, BF16)


def _pk(v):
    return pltpu.bitcast(v.astype(BF16), U32)


B_W1, B_W2, B_W8C, B_W256, B_W512, B_E0, B_N0 = range(7)
_MAGIC = 12582912.0
_SC_LIMIT = 8192.0


def _sincos(x):
    t = x * 0.6366197723675814 + _MAGIC
    n = pltpu.bitcast(t, jnp.int32)
    k = t - _MAGIC
    r = ((x - k * 1.5703125) - k * 4.837512969970703125e-4) - k * 7.54978995489188216e-8
    r2 = r * r
    sn = r + r * r2 * (-1.6666654611e-1 + r2 * (8.3321608736e-3 + r2 * -1.9515295891e-4))
    cs = 1.0 + r2 * (-0.5 + r2 * (4.166664568298827e-2 + r2 * (-1.388731625493765e-3 + r2 * 2.443315711809948e-5)))
    swap = (n & 1) == 1
    s_, c_ = jnp.where(swap, cs, sn), jnp.where(swap, sn, cs)
    ssign = (n & 2) << 30
    csign = ((n + 1) & 2) << 30
    s_ = pltpu.bitcast(pltpu.bitcast(s_, jnp.int32) ^ ssign, F32)
    c_ = pltpu.bitcast(pltpu.bitcast(c_, jnp.int32) ^ csign, F32)
    return s_, c_


def _emit(pieces, filler, fill_total, cap=3.4):
    room = [max(cap * c - v, 0.0) for _, c, v in pieces]
    tot = sum(room[:-1]) or 1.0
    done, target = 0.0, 0.0
    for (fn, _, _), r in zip(pieces, room):
        fn()
        target += fill_total * r / tot
        while done < target - 8:
            n = next(filler, None)
            if n is None:
                break
            done += n
    for _ in filler:
        pass


def _merge(*lists):
    tot = [sum(p[1] for p in l) or 1.0 for l in lists]
    pos = [0] * len(lists)
    acc = [0.0] * len(lists)
    out = []
    while True:
        best = None
        for i, l in enumerate(lists):
            if pos[i] < len(l):
                key = (acc[i] + 0.5 * l[pos[i]][1]) / tot[i]
                if best is None or key < best[0]:
                    best = (key, i)
        if best is None:
            return out
        i = best[1]
        out.append(lists[i][pos[i]])
        acc[i] += lists[i][pos[i]][1]
        pos[i] += 1


def _chain(*gens):
    for g in gens:
        yield from g


def _kernel(x_hbm, w_hbm, wo_hbm, u_hbm, are_hbm, aim_hbm, bre_hbm, bim_hbm, cre_hbm, cim_hbm,
            ldt_hbm, dsk_hbm, fk_hbm, fi_hbm, o_hbm,
            xp, wp, wop, up, prm, vec, fk, fi, stage,
            dtb, gb, base, cr, wt, bv, kw, u3, y, wkt, pkt, zacc, gp, mp, zb, pq, pp, flag, sem_in, sem_out):

    def iotas():
        return (lax.broadcasted_iota(jnp.int32, (8, 128), 0), lax.broadcasted_iota(jnp.int32, (8, 128), 1))

    def setup():
        ldt = vec[0][...].reshape(1, D).astype(F32)
        dt_row = jnp.exp(ldt).astype(BF16).astype(F32)
        for j in range(4):
            dtb[j * 128:(j + 1) * 128, :] = jnp.broadcast_to(dt_row[:, j * 128:(j + 1) * 128], (128, 128)).T
        for i in range(8):
            gb[i] = jnp.broadcast_to(fi[128 + i:129 + i, :], (128, 128)).T

    def wk_transpose():
        for b in range(4):
            for a in range(4):
                t = _bf(wp[a * 64:(a + 1) * 64, D + b * 128:D + (b + 1) * 128]).T
                wkt[b * 64:(b + 1) * 64, a * 128:(a + 1) * 128] = pltpu.bitcast(t, U32)

    def pro_rows(r0, exact):
        rows = pl.ds(r0, 16)
        dt = dtb[rows, :]
        ar = dt * prm[0, rows, :].astype(F32)
        ai = dt * prm[1, rows, :].astype(F32)
        mag = jnp.exp(ar)
        sn, cs = (jnp.sin(ai), jnp.cos(ai)) if exact else _sincos(ai)
        w1 = (mag * cs, mag * sn)
        yield 90
        db = (dt * prm[2, rows, :].astype(F32), dt * prm[3, rows, :].astype(F32))
        c = _cmul((prm[4, rows, :].astype(F32), prm[5, rows, :].astype(F32)), db)
        cr[rows, :] = c[0]
        lo = (lax.broadcasted_iota(jnp.int32, (16, 128), 0) & 4) == 0

        def put(i, v0, v1=None):
            for t in range(2):
                ev, od = (v0[t], v0[t]) if v1 is None else (jnp.where(lo, v0[t], v1[t]), jnp.where(lo, v1[t], v0[t]))
                base[2 * i + t, pl.ds(2 * r0, 16, stride=2), :] = ev
                base[2 * i + t, pl.ds(2 * r0 + 1, 16, stride=2), :] = od
        put(B_W1, w1)
        w2 = _csq(w1)
        put(B_W2, w2)
        w4 = _csq(w2)
        cw1 = _cmul(c, w1)
        put(B_N0, cw1, _cmul(cw1, w4))
        yield 80
        w8 = _csq(w4)
        put(B_W8C, (w8[0], -w8[1]))
        w128 = _csq(_csq(_csq(_csq(w8))))
        put(B_E0, (jnp.ones((16, 128), F32), jnp.zeros((16, 128), F32)), (w128[0], -w128[1]))
        w256 = _csq(w128)
        put(B_W256, w256)
        put(B_W512, _csq(w256))
        yield 84

    def pro(j):
        for r in range(j * 8, (j + 1) * 8):
            yield from pro_rows(r * 16, False)
    PRO_OPS = 8 * 254

    def range_check():
        m = None
        for r in range(32):
            a = jnp.abs(dtb[r * 16:(r + 1) * 16, :] * prm[1, r * 16:(r + 1) * 16, :].astype(F32))
            m = a if m is None else jnp.maximum(m, a)
            if r % 8 == 7:
                yield 64
        flag[0] = jnp.where(jnp.max(m) <= _SC_LIMIT, 0, 1).astype(jnp.int32)

    def pro_exact(j0, j1):
        @pl.when(flag[0] != 0)
        def _():
            def body(r, c):
                for _ in pro_rows(pl.multiple_of(r * 16, 16), True):
                    pass
                return c
            lax.fori_loop(j0 * 8, j1 * 8, body, 0)

    def kgen_pieces(j):
        st = {}

        def half(gi, g):
            sub, lane = iotas()
            odd = (sub & 1) == 1
            rows = slice(gi * 16 + g * 8, gi * 16 + g * 8 + 8)

            def ld(i):
                return base[2 * i, rows, :], base[2 * i + 1, rows, :]
            hi = odd if g == 0 else jnp.logical_not(odd)
            w8c = ld(B_W8C)
            e0 = [ld(B_E0)]
            for mu in range(1, 16):
                e0.append(_cmul(e0[-1], w8c))
            e0 = e0[::-1]
            w1, w2, w256, w512 = ld(B_W1), ld(B_W2), ld(B_W256), ld(B_W512)
            n0 = ld(B_N0)
            n1 = _cmul(n0, w1)
            n2 = _cmul(n0, w2)
            n3 = _cmul(n1, w2)
            n4 = _cmul(n1, w256)
            n5 = _cmul(n3, w256)
            n6 = _cmul(n5, w256)
            n7 = _cmul(n6, w256)
            sh = 7 if g == 0 else 1
            t = (jnp.where(hi, n7[0], pltpu.roll(n6[0], sh, 0)), jnp.where(hi, n7[1], pltpu.roll(n6[1], sh, 0)))
            n8 = _cmul(t, w512)
            n9 = _cmul(n8, w512)
            e1 = [n0, n1, n2, n3, n4, n5, n6, n7, n8, n9]
            lhs = jnp.concatenate([jnp.concatenate([v[0] for v in e1], axis=0),
                                   jnp.concatenate([v[1] for v in e1], axis=0)], axis=1)
            rhs = jnp.concatenate([jnp.concatenate([v[0] for v in e0], axis=0),
                                   jnp.concatenate([v[1] for v in e0], axis=0)], axis=1)
            o = _nt(lhs, rhs)
            o = [o[8 * i:8 * i + 8, :] for i in range(10)]

            emask = ((sub >> 1) - (lane >> 1)) & 3
            ea, xa = (lane >> 1) & 3, lane & 1
            lidx_a = (lane & 120) | ((((sub >> 1) - ea) & 3) << 1) | (xa ^ (sub & 1))
            sidx_a = ((((sub & 3) + ea) & 3) << 1) | (xa ^ (sub >> 2))

            def put(acc, src, e):
                if e == 0:
                    return src
                return jnp.where(emask == e, pltpu.roll(src, 2 * e, 0), acc)

            s = None
            for e in range(4):
                s = put(s, o[e], e)
            s = jnp.take_along_axis(s, lidx_a, axis=1)
            a2 = jnp.take_along_axis(s, sidx_a, axis=0)
            if g == 0:
                st["a"] = a2
                st["b"] = [put(o[4 + 2 * q], o[5 + 2 * q], 1) for q in range(3)]
                return
            hp, ab, hh = (lane >> 2) & 1, (lane >> 1) & 1, lane & 1
            gg = hp ^ (sub & 1)
            lidx_b = (lane & 120) | ((((sub >> 1) - (2 * gg + ab)) & 3) << 1) | (hh ^ gg)
            g2 = sub >> 2
            sidx_b = ((((sub & 3) + 2 * g2 + ab) & 3) << 1) | (hp ^ g2)
            lo = sub < 4
            res = [jnp.where(lo, st["a"], a2), pltpu.roll(jnp.where(lo, a2, st["a"]), 4, 0)]
            for q in range(3):
                s = put(put(st["b"][q], o[4 + 2 * q], 2), o[5 + 2 * q], 3)
                s = jnp.take_along_axis(s, lidx_b, axis=1)
                res.append(jnp.take_along_axis(s, sidx_b, axis=0))
            if gi % 2 == 0:
                st["r"] = res
            else:
                for q in range(5):
                    wt[q, (gi // 2) * 8:(gi // 2) * 8 + 8, :] = _pk(jnp.concatenate([st["r"][q], res[q]], axis=0))

        return [(functools.partial(half, gi, g), 40, 180) for gi in range(j * 16, (j + 1) * 16) for g in range(2)]

    def kdft_pieces(j):
        def bvals():
            dsk_row = vec[1][...].reshape(1, D).astype(F32)
            k0 = _nt(jnp.ones((8, 128), F32), cr[j * 128:(j + 1) * 128, :])
            bv[j, 0] = k0 + dsk_row[:, j * 128:(j + 1) * 128]
            for q in (1, 2, 3):
                o = FK_SEL // 2 + 8 * (q - 1)
                r = _nt(_bf(fk[o:o + 8, :]), _bf(wt[q, j * 64:(j + 1) * 64, :]))
                bv[j, q] = r[0:8]

        def piece(k, hf):
            o = k * 128 + hf * 64
            r = _nt(_bf(fk[o:o + 64, :]), _bf(wt[_TILE_OF_CHUNK[k], j * 64:(j + 1) * 64, :]))
            rr, ri = r[:64], r[64:]
            rows = slice(hf * 64, hf * 64 + 64)
            if k in _BCH:
                b = _BCH.index(k)
                bval = jnp.concatenate([bv[j, b]] * 8, axis=0)
                rr = rr + gb[2 * b, rows, :] * bval
                ri = ri + gb[2 * b + 1, rows, :] * bval
            kw[j, 0, k, rows, :] = rr
            kw[j, 1, k, rows, :] = ri
            kw[j, 2, k, rows, :] = rr + ri

        order = [k for k in range(16) if k not in _BCH] + list(_BCH)
        return [(bvals, 64, 4)] + [(functools.partial(piece, k, hf), 32, 40 if k in _BCH else 8)
                                   for k in order for hf in range(2)]

    def udft_pieces(j):
        def piece(i, hf):
            o = FK_FU // 2 + hf * 64
            r = _nn(_bf(fk[o:o + 64, :]), _bf(up[i * 64:(i + 1) * 64, j * 128:(j + 1) * 128]))
            rr, ri = r[:64], r[64:]
            rows = slice(hf * 64, hf * 64 + 64)
            u3[j, 0, i, rows, :] = rr
            u3[j, 1, i, rows, :] = ri
            u3[j, 2, i, rows, :] = rr + ri
        return [(functools.partial(piece, i, hf), 32, 8) for i in range(16) for hf in range(2)]

    def conv(p0, p1):
        BL = 4
        for pp_ in range(p0, p1):
            j, p = divmod(pp_, 16)
            rs = slice(p * 8, p * 8 + 8)
            prev = None
            for ib in range(16 // BL):
                a = zr = None
                for c in range(3):
                    acc = [None] * BL
                    for ub in range(ib + 1):
                        n = 0
                        uu = [u3[j, c, ub * BL + t, rs, :] for t in range(BL)]
                        dlt = (ib - ub) * BL
                        for dk in range(-(BL - 1), BL):
                            k = dlt + dk
                            if k < 0:
                                continue
                            kk = kw[j, c, k, rs, :]
                            for t in range(BL):
                                o = t + dk
                                if 0 <= o < BL:
                                    pr = kk * uu[t]
                                    acc[o] = pr if acc[o] is None else acc[o] + pr
                                    n += 2
                        if ub < ib:
                            yield n
                    if c == 0:
                        a = acc
                    elif c == 1:
                        zr = [a[o] - acc[o] for o in range(BL)]
                        a = [a[o] + acc[o] for o in range(BL)]
                    else:
                        for o in range(BL):
                            zi = acc[o] - a[o]
                            if prev is None:
                                yr, yi = zi, -zr[o]
                            else:
                                yr, yi = prev[0] + zi, prev[1] - zr[o]
                            y[j, 0, ib * BL + o, rs, :] = yr
                            y[j, 1, ib * BL + o, rs, :] = yi
                            prev = (zr[o], zi)
                        n += 8
                    yield n
    CONV_OPS = 848

    def inv_pieces(j):
        def piece(i):
            sub, _ = iotas()
            rev = 7 - sub
            s = _nn(fi[0:64, :], y[j, 0, i])
            a = _nn(fi[64:128, :], y[j, 1, i])
            lo_ = s + a
            hi_ = s - a
            hi_ = jnp.concatenate(
                [jnp.take_along_axis(hi_[8 * v:8 * v + 8], rev, axis=0) for v in range(7, -1, -1)], axis=0)
            stage[i * 64:(i + 1) * 64, D + j * 128:D + (j + 1) * 128] = _pk(jnp.concatenate([lo_, hi_], axis=0))
        return [(functools.partial(piece, i), 32, 32) for i in range(16)]

    def kt_pieces(pb0, pb1):
        def piece(fb, pb):
            pk = _phi(_nt(_bf(wkt[fb * 64:(fb + 1) * 64, :]), _bf(xp[pb * 64:(pb + 1) * 64, :])))
            pkt[fb * 64:(fb + 1) * 64, pb * 128:(pb + 1) * 128] = _pk(pk)
            rows = slice(fb * 128, (fb + 1) * 128)
            if pb == 0:
                zacc[rows, :] = pk
            else:
                zacc[rows, :] += pk
        return [(functools.partial(piece, fb, pb), 128, 152) for pb in range(pb0, pb1) for fb in range(4)]

    def g_pieces(fb0, fb1):
        st = {}

        def piece(fb, cb, kb):
            r = _nn(_bf(pkt[fb * 32:(fb + 1) * 32, kb * 512:(kb + 1) * 512]),
                    _bf(xp[kb * 256:(kb + 1) * 256, cb * 128:(cb + 1) * 128]))
            if kb > 0:
                r = r + st["acc"]
            if kb == 3:
                gp[fb * 32:(fb + 1) * 32, cb * 128:(cb + 1) * 128] = _pk(r)
            else:
                st["acc"] = r
        return [(functools.partial(piece, fb, cb, kb), 64, 32)
                for fb in range(fb0, fb1) for cb in range(4) for kb in range(4)]

    def mid_pieces():
        st = {}

        def bd():
            r128 = lax.broadcasted_iota(jnp.int32, (128, 128), 0)
            c128 = lax.broadcasted_iota(jnp.int32, (128, 128), 1)
            return (r128 >> 4) == (c128 >> 4)

        def kv(g):
            r = _nn(_bf(gp[g * 64:(g + 1) * 64, :]), _bf(wp[:, 2 * D + g * 128:2 * D + (g + 1) * 128]))
            st[g] = jnp.where(bd(), r, 0.0).astype(BF16)
            z = jnp.sum(zacc[g * 128:(g + 1) * 128, :], axis=1, keepdims=True)
            zb[g] = jnp.where(bd(), jnp.broadcast_to(z, (128, 128)), 0.0)

        def mm(g):
            mp[g * 64:(g + 1) * 64, :] = _pk(_nn(st[g], _bf(wop[g * 64:(g + 1) * 64, :])))
        return ([(functools.partial(kv, g), 128, 100) for g in range(4)],
                [(functools.partial(mm, g), 128, 32) for g in range(4)])

    def q_pieces(rb0, rb1):
        def piece(rb, g):
            pq[rb * 64:(rb + 1) * 64, g * 128:(g + 1) * 128] = _phi(
                _nn(_bf(xp[rb * 32:(rb + 1) * 32, :]), _bf(wp[:, g * 128:(g + 1) * 128])))
        return [(functools.partial(piece, rb, g), 64, 64) for rb in range(rb0, rb1) for g in range(4)]

    def o_pieces(rb0, rb1, skew=2):
        def den(rb):
            rows = slice(rb * 64, (rb + 1) * 64)
            for g in range(4):
                cols = slice(g * 128, (g + 1) * 128)
                d = _nn(pq[rows, cols], zb[g]) + 1e-6
                pp[rb * 32:(rb + 1) * 32, cols] = _pk(pq[rows, cols] * pl.reciprocal(d, approx=True))

        def out(rb, g):
            stage[rb * 32:(rb + 1) * 32, g * 128:(g + 1) * 128] = _pk(
                _nn(_bf(pp[rb * 32:(rb + 1) * 32, :]), _bf(mp[:, g * 128:(g + 1) * 128])))
        res = []
        for rb in range(rb0, rb1 + skew):
            if rb < rb1:
                res.append((functools.partial(den, rb), 64, 80))
            if rb - skew >= rb0:
                res += [(functools.partial(out, rb - skew, g), 64, 28) for g in range(4)]
        return res

    prm_hbm = (are_hbm, aim_hbm, bre_hbm, bim_hbm, cre_hbm, cim_hbm)
    xb, wb, wob, ub_, sb = (r.bitcast(BF16) for r in (xp, wp, wop, up, stage))
    srcs = {
        "wq": (w_hbm.at[:, 0:D], wb.at[:, 0:D]),
        "x0": (x_hbm.at[0:256], xb.at[0:256]),
        "ldt": (ldt_hbm, vec[0]),
        "dsk": (dsk_hbm, vec[1]),
        "fi": (fi_hbm, fi),
        "x1": (x_hbm.at[256:768], xb.at[256:768]),
        "p0": (prm_hbm[0], prm.at[0]),
        "p1": (prm_hbm[1], prm.at[1]),
        "x2": (x_hbm.at[768:1280], xb.at[768:1280]),
        "p2": (prm_hbm[2], prm.at[2]),
        "p3": (prm_hbm[3], prm.at[3]),
        "p4": (prm_hbm[4], prm.at[4]),
        "p5": (prm_hbm[5], prm.at[5]),
        "x3": (x_hbm.at[1280:2048], xb.at[1280:2048]),
        "u": (u_hbm, ub_),
        "fk": (fk_hbm, fk),
        "wk": (w_hbm.at[:, D:2 * D], wb.at[:, D:2 * D]),
        "wv": (w_hbm.at[:, 2 * D:3 * D], wb.at[:, 2 * D:3 * D]),
        "wo": (wo_hbm, wob),
    }
    cin = {k: pltpu.make_async_copy(a, b, sem_in.at[i]) for i, (k, (a, b)) in enumerate(srcs.items())}
    for c in cin.values():
        c.start()
    couts = []

    def wait(*names):
        for n in names:
            cin[n].wait()

    def out_copy(i, r0, r1, c0, c1):
        return pltpu.make_async_copy(sb.at[r0:r1, c0:c1], o_hbm.at[r0:r1, c0:c1], sem_out.at[i])

    def store(*box):
        out_copy(len(couts), *box).start()
        couts.append(box)

    none = iter(())
    mid1, mid2 = mid_pieces()
    C1, C2, C3 = 34, 48, 64
    O1, O2 = 13, 27
    steps = [
        (lambda: wait("wq", "x0", "ldt", "dsk", "fi"),
         lambda: (setup(), _emit(q_pieces(0, 4), none, 0))),
        (lambda: wait("x1"),
         lambda: _emit(q_pieces(4, 12), none, 0)),
        (lambda: wait("p0", "p1", "x2", "p2", "p3", "p4", "p5"),
         lambda: _emit(q_pieces(12, 20), _chain(range_check(), pro(0), pro(1)), 256 + 2 * PRO_OPS)),
        (lambda: (pro_exact(0, 2), wait("x3")),
         lambda: _emit(_merge(q_pieces(20, 32), kgen_pieces(0) + kgen_pieces(1)), _chain(pro(2), pro(3)), 2 * PRO_OPS)),
        (lambda: (pro_exact(2, 4), wait("u", "fk", "wk")),
         lambda: (wk_transpose(),
                  _emit(_merge(kgen_pieces(2) + kgen_pieces(3),
                               udft_pieces(0) + kdft_pieces(0) + udft_pieces(1) + kdft_pieces(1) + udft_pieces(2)
                               + kdft_pieces(2)), none, 0))),
        (lambda: wait("wv", "wo"),
         lambda: _emit(_merge(kt_pieces(0, 16), udft_pieces(3) + kdft_pieces(3)) + g_pieces(0, 7)
                       + _merge(mid1[:3], g_pieces(7, 8)) + mid2[:2] + mid1[3:] + mid2[2:],
                       conv(0, C1), C1 * CONV_OPS)),
        (lambda: None,
         lambda: _emit(inv_pieces(0)[:4] + _merge(o_pieces(0, O1), inv_pieces(0)[4:] + inv_pieces(1)),
                       conv(C1, C2), (C2 - C1) * CONV_OPS)),
        (lambda: (store(0, S, D, D + 256), store(0, O1 * 64, 0, D)),
         lambda: _emit(_merge(o_pieces(O1, O2), inv_pieces(2)), conv(C2, C3), (C3 - C2) * CONV_OPS)),
        (lambda: (store(0, S, D + 256, D + 384), store(O1 * 64, O2 * 64, 0, D)),
         lambda: _emit(_merge(o_pieces(O2, 32), inv_pieces(3)), none, 0)),
    ]
    only = os.environ.get("BLK")
    only = None if only is None else [int(t) for t in only.split(",")]

    def outer(i, c):
        for k, (pre, blk) in enumerate(steps):
            @pl.when(i + 2 * k == 2 * k)
            def _():
                pre()

            if only is None or k in only:
                @pl.when(i + 2 * k + 1 == 2 * k + 1)
                def _():
                    blk()
        return c

    lax.fori_loop(0, 2, outer, 0)
    store(0, S, D + 384, 2 * D)
    store(O2 * 64, S, 0, D)
    for i, box in enumerate(couts):
        out_copy(i, *box).wait()


def _kernel_entry(*refs):
    refs = list(refs)
    n_in = 15
    ins, scr = refs[:n_in], refs[n_in:]
    xp, wp, wop, up, prm, v0, v1 = scr[:7]
    return _kernel(*ins, xp, wp, wop, up, prm, (v0, v1), *scr[7:])


@jax.jit
def pallas_concat_heads__linear_attn_block__ssm_conv_s4__prompt_kernel(
    A_x, A_wqkv, A_wo, B_u, B_A_re, B_A_im, B_B_re, B_B_im, B_C_re, B_C_im, B_log_dt, B_Dskip,
):
    fk, fi = _tables()
    V = pltpu.VMEM
    out = pl.pallas_call(
        _kernel_entry,
        out_shape=jax.ShapeDtypeStruct((S, 2 * D), BF16),
        in_specs=[pl.BlockSpec(memory_space=pl.ANY)] * 14,
        out_specs=pl.BlockSpec(memory_space=pl.ANY),
        scratch_shapes=[
            V((S // 2, D), U32),
            V((D // 2, 3 * D), U32),
            V((D // 2, D), U32),
            V((S // 2, D), U32),
            V((6, D, 128), BF16),
            V((D,), BF16), V((D,), BF16),
            V((FK_ROWS // 2, 128), U32),
            V((136, 128), F32),
            V((S // 2, 2 * D), U32),
            V((D, 128), F32),
            V((8, 128, 128), F32),
            V((14, 2 * D, 128), F32),
            V((D, 128), F32),
            V((5, D // 2, 128), U32),
            V((4, 4, 8, 128), F32),
            V((4, 3, 16, 128, 128), F32),
            V((4, 3, 16, 128, 128), F32),
            V((4, 2, 16, 128, 128), F32),
            V((D // 2, D), U32),
            V((D // 2, S), U32),
            V((D, 128), F32),
            V((D // 2, D), U32),
            V((D // 2, D), U32),
            V((4, 128, 128), F32),
            V((S, D), F32),
            V((S // 2, D), U32),
            pltpu.SMEM((1,), jnp.int32),
            pltpu.SemaphoreType.DMA((24,)),
            pltpu.SemaphoreType.DMA((16,)),
        ],
        compiler_params=pltpu.CompilerParams(vmem_limit_bytes=110 * 2**20),
    )(A_x.reshape(S, D), A_wqkv, A_wo, B_u.reshape(S, D), B_A_re, B_A_im, B_B_re, B_B_im, B_C_re, B_C_im,
      B_log_dt, B_Dskip, jnp.asarray(fk), jnp.asarray(fi))
    return out.reshape(1, S, 2 * D)
```

```python
import functools

import numpy as np
import jax
import jax.numpy as jnp
from jax import lax
import jax.experimental.pallas as pl
import jax.experimental.pallas.tpu as pltpu

S = 2048
D = 512
F32 = jnp.float32
BF16 = jnp.bfloat16
U32 = jnp.uint32

_BASE = np.array([[1, 5], [2, 6], [3, 7], [4, 8], [258, 262], [260, 264],
                  [516, 520], [772, 776], [1032, 1288], [1544, 1800]])
_TILE_OF_CHUNK = [0, 1, 2, 2, 3, 3, 3, 3] + [4] * 8

FK_OFF = [0, 256, 528, 784] + [1056 + 144 * k for k in range(4)] + [1632 + 80 * k for k in range(8)]
FK_FU = 1632 + 640
FK_ROWS = FK_FU + 256

X0, X1 = 384, 896
QOLD = X0 // 64
G0 = 12
R0 = 8 * G0
O1, O2, O3, O4 = 15, 24, 29, 30
GS = 120
C3 = 50

B_W1, B_W2, B_W8C, B_W256, B_W512, B_E0, B_N0 = range(7)
_SC_LIMIT = 8192.0


def _bf16_bits(v):
    u = np.ascontiguousarray(v, np.float32).view(np.uint32)
    return ((u + 0x7FFF + ((u >> 16) & 1)) >> 16).astype(np.uint32)


def _pack_rows(v):
    b = _bf16_bits(v)
    return b[0::2] | (b[1::2] << 16)


@functools.lru_cache(maxsize=None)
def _tables():
    lr = (_bf16_bits(np.arange(S)) << 16).view(np.float32).astype(np.int64)
    val = np.zeros((5, 128), np.int64)
    for lam in range(128):
        mu, tau = 15 - (lam >> 3), lam & 7
        e, x = tau >> 1, tau & 1
        for h in range(2):
            val[h, lam] = _BASE[e, x ^ h] + 8 * (mu + 16 * h)
        hp, ab, h = tau >> 2, (tau >> 1) & 1, tau & 1
        for q in range(3):
            val[2 + q, lam] = _BASE[4 + 2 * q + ab, hp] + 8 * (mu + 16 * h)
    om = 2 * np.pi * (np.arange(128) + 0.25) / 128.0
    phase = np.exp(1j * om * 191.5)

    def stack(z):
        return np.concatenate([p[32 * t:32 * t + 32] for t in range(4) for p in (z.real, z.imag)], axis=0)

    fk = []
    g = np.zeros(128, np.complex128)
    for k in range(4):
        slot = {int(v): i for i, v in enumerate(val[_TILE_OF_CHUNK[k]])}
        m = np.zeros((128, 128), np.complex128)
        for p in range(1, 129):
            lag = 128 * k + p
            v = int(lr[lag])
            z = np.exp(-1j * om * p) * (0.5 if lag == 512 else 1.0)
            if v in slot:
                m[:, slot[v]] += z
            else:
                assert v == 256 and k == 2
                g += z
        if k in (1, 3):
            sel = np.zeros((16, 128))
            sel[:, slot[128 * (k + 1)]] = 1.0
            fk += [stack(m)[:128], sel, stack(m)[128:]]
        else:
            fk.append(stack(m))
    for k in range(4, 16):
        st = 4 if k < 8 else 8
        per = 128 // st
        slot = {int(v): i for i, v in enumerate(val[_TILE_OF_CHUNK[k]])}
        for lag in range(128 * k + 1, min(128 * k + 128, S)):
            m_ = int(lr[lag]) // st
            assert int(lr[lag]) % st == 0 and abs(lag - st * m_) <= (st // 2 if m_ % 2 == 0 else st // 2 - 1)
        od = np.zeros((per, 128), np.complex128)
        ev = np.zeros((per, 128), np.complex128)
        edge = np.zeros((16, 128))
        for m_ in range(per + 1):
            v = 128 * k + st * m_
            if v not in slot:
                assert m_ == 0 and k in (4, 8)
                continue
            z = np.exp(-1j * om[:per] * st * m_)
            if m_ % 2:
                od[:, slot[v]] = z
            else:
                ev[:, slot[v]] = z * (0.5 if m_ in (0, per) else 1.0)
            if m_ in (0, per):
                edge[8 * (m_ // per):8 * (m_ // per) + 8, slot[v]] = 1.0
        fk += [edge, od.real, od.imag, ev.real, ev.imag]
    fk.append(stack(np.exp(-1j * om[:, None] * np.arange(128)[None, :]) * phase[:, None]))
    fk = np.concatenate(fk, axis=0)
    assert fk.shape[0] == FK_ROWS
    tabs = [g.real, g.imag]
    for h in (2, 4):
        tabs += [sum(np.cos(om * p) for p in range(1 - h, h)), sum(np.cos(om * p) for p in range(-h, h + 1)),
                 -sum(np.sin(om * p) for p in range(1, h + 1))]
    jj = np.arange(64)[:, None] - 63.5
    finv = np.concatenate([np.cos(om[None, :] * jj) / 128.0, -np.sin(om[None, :] * jj) / 128.0,
                           np.stack(tabs)], axis=0)
    return _pack_rows(fk), finv.astype(np.float32)


def _cmul(a, b):
    return a[0] * b[0] - a[1] * b[1], a[0] * b[1] + a[1] * b[0]


def _csq(a):
    return a[0] * a[0] - a[1] * a[1], (a[0] + a[0]) * a[1]


def _phi(t):
    return jnp.where(t > 0, t + 1.0, jnp.exp(t)) + 1e-6


def _nt(a, b):
    return lax.dot_general(a, b, (((1,), (1,)), ((), ())), preferred_element_type=F32)


def _nn(a, b):
    return jnp.dot(a, b, preferred_element_type=F32)


def _bf(v):
    return pltpu.bitcast(v, BF16)


def _pk(v):
    return pltpu.bitcast(v.astype(BF16), U32)


def _sincos(x):
    t = x * 0.6366197723675814 + 12582912.0
    n = pltpu.bitcast(t, jnp.int32) - 0x4B400000
    k = n.astype(F32)
    r = ((x - k * 1.5703125) - k * 4.837512969970703125e-4) - k * 7.54978995489188216e-8
    r2 = r * r
    sn = r + r * r2 * (-1.6666654611e-1 + r2 * (8.3321608736e-3 + r2 * -1.9515295891e-4))
    cs = 1.0 + r2 * (-0.5 + r2 * (4.166664568298827e-2 + r2 * (-1.388731625493765e-3 + r2 * 2.443315711809948e-5)))
    swap = (n & 1) == 1
    s_, c_ = jnp.where(swap, cs, sn), jnp.where(swap, sn, cs)
    ssign = (n & 2) << 30
    csign = ((n + 1) & 2) << 30
    s_ = pltpu.bitcast(pltpu.bitcast(s_, jnp.int32) ^ ssign, F32)
    c_ = pltpu.bitcast(pltpu.bitcast(c_, jnp.int32) ^ csign, F32)
    return s_, c_


def _emit(pieces, filler=None, fill_total=0, cap=3.0, tail=100):
    filler = iter(()) if filler is None else filler
    room = [max(cap * c - v, 0.0) for _, c, v in pieces]
    tot = sum(room[:-1]) or 1.0
    done, target = 0.0, 0.0
    for (fn, _, _), r in zip(pieces, room):
        fn()
        target += max(fill_total - tail, 0) * r / tot
        while done < target - 8:
            n = next(filler, None)
            if n is None:
                break
            done += n
    for _ in filler:
        pass


def _merge(*lists):
    tot = [sum(p[1] for p in l) or 1.0 for l in lists]
    pos = [0] * len(lists)
    acc = [0.0] * len(lists)
    out = []
    while True:
        best = None
        for i, l in enumerate(lists):
            if pos[i] < len(l):
                key = (acc[i] + 0.5 * l[pos[i]][1]) / tot[i]
                if best is None or key < best[0]:
                    best = (key, i)
        if best is None:
            return out
        i = best[1]
        out.append(lists[i][pos[i]])
        acc[i] += lists[i][pos[i]][1]
        pos[i] += 1


def _group(pieces, n):
    out = []
    for i in range(0, len(pieces), n):
        grp = pieces[i:i + n]

        def run(grp=grp):
            for f, _, _ in grp:
                f()
        out.append((run, sum(p[1] for p in grp), sum(p[2] for p in grp)))
    return out


def _reim(r):
    n = r.shape[0] // 64
    return (jnp.concatenate([r[64 * t:64 * t + 32] for t in range(n)], axis=0),
            jnp.concatenate([r[64 * t + 32:64 * t + 64] for t in range(n)], axis=0))


def _kernel(x_hbm, w_hbm, wo_hbm, u_hbm, are_hbm, aim_hbm, bre_hbm, bim_hbm, cre_hbm, cim_hbm,
            ldt_hbm, dsk_hbm, fk_hbm, fi_hbm, o_hbm,
            xp, wb, wob, up, prm, ldt, dsk, xb, ub, fk, fi, sta, stb, w1s, flag,
            dtb, gb, base, cr, wt, bv, k0s, kw, u3, y, wkt, pkt, zacc, gp, mp, zb, pq, pp,
            wqt, wqp, zpk, zrow, kf, zc, sem_in, sem_out):

    def iotas():
        return (lax.broadcasted_iota(jnp.int32, (8, 128), 0), lax.broadcasted_iota(jnp.int32, (8, 128), 1))

    packed = set()

    def tile(kind, r0, n, cols=slice(None)):
        src, dst = (xb, xp) if kind == "x" else (ub, up)
        parts = []
        for r in range(r0, r0 + n, 64):
            key = (kind, r, cols.start)
            if key in packed:
                parts.append(_bf(dst[r // 2:r // 2 + 32, cols]))
            else:
                packed.add(key)
                v = src[r:r + 64, cols]
                dst[r // 2:r // 2 + 32, cols] = pltpu.bitcast(v, U32)
                parts.append(v)
        return parts[0] if len(parts) == 1 else jnp.concatenate(parts, axis=0)

    def setup_dt(j0, j1):
        dt_row = jnp.exp(ldt[...].reshape(1, D).astype(F32)).astype(BF16).astype(F32)
        for j in range(j0, j1):
            dtb[j * 128:(j + 1) * 128, :] = jnp.broadcast_to(dt_row[:, j * 128:(j + 1) * 128], (128, 128)).T

    def setup_g():
        for i in range(8):
            gb[i] = jnp.broadcast_to(fi[128 + i:129 + i, :], (128, 128)).T

    def perm_rows(ref):
        return jnp.concatenate([ref[pl.ds(t, 64, stride=4), :] for t in range(4)], axis=0)

    def wq_perm_a():
        for a in range(4):
            for b in range(4):
                t = wb[a * 128:(a + 1) * 128, b * 128:(b + 1) * 128].T
                wqt[a, b * 64:(b + 1) * 64, :] = pltpu.bitcast(t, U32)

    def wq_perm_b():
        for b in range(4):
            for a in range(4):
                t = _bf(wqt[a, pl.ds(b, 64, stride=4), :]).T
                wqp[a * 64:(a + 1) * 64, b * 128:(b + 1) * 128] = pltpu.bitcast(t, U32)

    def wk_transpose():
        for b in range(4):
            for a in range(4):
                t = wb[a * 128:(a + 1) * 128, D + b * 128:D + (b + 1) * 128].T
                wkt[b * 64:(b + 1) * 64, a * 128:(a + 1) * 128] = pltpu.bitcast(t, U32)

    def w1_rows(r0, exact):
        rows = pl.ds(r0, 16)
        dt = dtb[rows, :]
        ar = dt * prm[0, rows, :].astype(F32)
        ai = dt * prm[1, rows, :].astype(F32)
        mag = jnp.exp(ar)
        sn, cs = (jnp.sin(ai), jnp.cos(ai)) if exact else _sincos(ai)
        w1s[0, rows, :] = mag * cs
        w1s[1, rows, :] = mag * sn

    def range_check(i, r0, r1):
        m = jnp.max(jnp.abs(prm[1, r0:r1, :].astype(F32)).reshape((r1 - r0) // 8, 8, 128), axis=0)
        dmax = jnp.max(dtb[r0:r1, :].reshape((r1 - r0) // 8, 8, 128), axis=0)
        bound = jnp.max(m) * jnp.max(dmax)
        flag[i] = jnp.where(bound <= _SC_LIMIT, 0, 1).astype(jnp.int32)

    def stage1():
        for r in range(G0 // 2, 32):
            w1_rows(r * 16, False)
            yield 90

    def stage1_exact():
        @pl.when(flag[0] != 0)
        def _():
            def body(r, c):
                w1_rows(pl.multiple_of(r * 16, 16), True)
                return c
            lax.fori_loop(G0 // 2, 32, body, 0)

    def stage2(r):
        r0 = r * 16 if isinstance(r, int) else pl.multiple_of(r * 16, 16)
        rows = pl.ds(r0, 16)
        dt = dtb[rows, :]
        w1 = (w1s[0, rows, :], w1s[1, rows, :])
        db = (dt * prm[2, rows, :].astype(F32), dt * prm[3, rows, :].astype(F32))
        c = _cmul((prm[4, rows, :].astype(F32), prm[5, rows, :].astype(F32)), db)
        cr[rows, :] = c[0]
        lo = (lax.broadcasted_iota(jnp.int32, (16, 128), 0) & 4) == 0

        def put(i, v0, v1=None):
            for t in range(2):
                ev, od = (v0[t], v0[t]) if v1 is None else (jnp.where(lo, v0[t], v1[t]), jnp.where(lo, v1[t], v0[t]))
                base[2 * i + t, pl.ds(2 * r0, 16, stride=2), :] = ev
                base[2 * i + t, pl.ds(2 * r0 + 1, 16, stride=2), :] = od
        put(B_W1, w1)
        w2 = _csq(w1)
        put(B_W2, w2)
        w4 = _csq(w2)
        cw1 = _cmul(c, w1)
        put(B_N0, cw1, _cmul(cw1, w4))
        yield 80
        w8 = _csq(w4)
        put(B_W8C, (w8[0], -w8[1]))
        w128 = _csq(_csq(_csq(_csq(w8))))
        put(B_E0, (jnp.ones((16, 128), F32), jnp.zeros((16, 128), F32)), (w128[0], -w128[1]))
        w256 = _csq(w128)
        put(B_W256, w256)
        put(B_W512, _csq(w256))
        yield 84

    def stage2_fill(r0, r1):
        for r in range(r0, r1):
            yield from stage2(r)

    def early_prep():
        range_check(1, 0, R0)
        for r in range(G0 // 2):
            w1_rows(r * 16, False)
        for _ in stage2_fill(0, G0 // 2):
            pass

    def early_exact():
        @pl.when(flag[1] != 0)
        def _():
            def body(r, c):
                w1_rows(pl.multiple_of(r * 16, 16), True)
                for _ in stage2(r):
                    pass
                return c
            lax.fori_loop(0, G0 // 2, body, 0)

    def kgen_pieces(g0, g1):
        st = {}

        def half(gi, g):
            sub, lane = iotas()
            odd = (sub & 1) == 1
            rows = slice(gi * 16 + g * 8, gi * 16 + g * 8 + 8)

            def ld(i):
                return base[2 * i, rows, :], base[2 * i + 1, rows, :]
            hi = odd if g == 0 else jnp.logical_not(odd)
            w8c = ld(B_W8C)
            e0 = [ld(B_E0)]
            for _ in range(1, 16):
                e0.append(_cmul(e0[-1], w8c))
            e0 = e0[::-1]
            w1, w2, w256, w512 = ld(B_W1), ld(B_W2), ld(B_W256), ld(B_W512)
            n0 = ld(B_N0)
            n1 = _cmul(n0, w1)
            n2 = _cmul(n0, w2)
            n3 = _cmul(n1, w2)
            n4 = _cmul(n1, w256)
            n5 = _cmul(n3, w256)
            n6 = _cmul(n5, w256)
            n7 = _cmul(n6, w256)
            sh = 7 if g == 0 else 1
            t = (jnp.where(hi, n7[0], pltpu.roll(n6[0], sh, 0)), jnp.where(hi, n7[1], pltpu.roll(n6[1], sh, 0)))
            n8 = _cmul(t, w512)
            n9 = _cmul(n8, w512)
            e1 = [n0, n1, n2, n3, n4, n5, n6, n7, n8, n9]
            lhs = jnp.concatenate([jnp.concatenate([v[0] for v in e1], axis=0),
                                   jnp.concatenate([v[1] for v in e1], axis=0)], axis=1)
            rhs = jnp.concatenate([jnp.concatenate([v[0] for v in e0], axis=0),
                                   jnp.concatenate([v[1] for v in e0], axis=0)], axis=1)
            o = _nt(lhs, rhs)
            o = [o[8 * i:8 * i + 8, :] for i in range(10)]

            emask = ((sub >> 1) - (lane >> 1)) & 3
            ea, xa = (lane >> 1) & 3, lane & 1
            lidx_a = (lane & 120) | ((((sub >> 1) - ea) & 3) << 1) | (xa ^ (sub & 1))
            sidx_a = ((((sub & 3) + ea) & 3) << 1) | (xa ^ (sub >> 2))

            def put(acc, src, e):
                if e == 0:
                    return src
                return jnp.where(emask == e, pltpu.roll(src, 2 * e, 0), acc)

            s = None
            for e in range(4):
                s = put(s, o[e], e)
            s = jnp.take_along_axis(s, lidx_a, axis=1)
            a2 = jnp.take_along_axis(s, sidx_a, axis=0)
            if g == 0:
                st["a"] = a2
                st["b"] = [put(o[4 + 2 * q], o[5 + 2 * q], 1) for q in range(3)]
                return
            hp, ab, hh = (lane >> 2) & 1, (lane >> 1) & 1, lane & 1
            gg = hp ^ (sub & 1)
            lidx_b = (lane & 120) | ((((sub >> 1) - (2 * gg + ab)) & 3) << 1) | (hh ^ gg)
            g2 = sub >> 2
            sidx_b = ((((sub & 3) + 2 * g2 + ab) & 3) << 1) | (hp ^ g2)
            lo = sub < 4
            res = [jnp.where(lo, st["a"], a2), pltpu.roll(jnp.where(lo, a2, st["a"]), 4, 0)]
            for q in range(3):
                s = put(put(st["b"][q], o[4 + 2 * q], 2), o[5 + 2 * q], 3)
                s = jnp.take_along_axis(s, lidx_b, axis=1)
                res.append(jnp.take_along_axis(s, sidx_b, axis=0))
            if gi % 2 == 0:
                st["r"] = res
            else:
                for q in range(5):
                    wt[q, (gi // 2) * 8:(gi // 2) * 8 + 8, :] = _pk(jnp.concatenate([st["r"][q], res[q]], axis=0))

        return _group([(functools.partial(half, gi, g), 40, 180) for gi in range(g0, g1) for g in range(2)], 2)

    def k0_all():
        k0s[...] = _nt(jnp.ones((8, 128), F32), cr[...]) + dsk[...].reshape(1, D).astype(F32)

    def kdft_pieces(j, extra):
        def wtile(k):
            return _bf(wt[_TILE_OF_CHUNK[k], j * 64:(j + 1) * 64, :])

        def near(k, hf):
            o = FK_OFF[k] // 2 + hf * 64
            if k in (1, 3):
                r = _nt(_bf(fk[o:o + 72, :]), wtile(k))
                bv[j, k // 2, hf * 8:hf * 8 + 8, :] = r[128:136] if hf == 0 else r[0:8]
                r = r[:128] if hf == 0 else r[16:]
            else:
                r = _nt(_bf(fk[o:o + 64, :]), wtile(k))
            rr, ri = _reim(r)
            rows = slice(hf * 64, hf * 64 + 64)
            if k == 0:
                rr = rr + jnp.concatenate([k0s[:, j * 128:(j + 1) * 128]] * 8, axis=0)
            elif k == 2:
                bval = jnp.concatenate([bv[j, 0]] * 4, axis=0)
                rr = rr + gb[0, rows, :] * bval
                ri = ri + gb[1, rows, :] * bval
            kw[j, 0, k, rows, :] = rr
            kw[j, 1, k, rows, :] = ri
            kw[j, 2, k, rows, :] = rr + ri

        def far(k):
            per = 32 if k < 8 else 16
            n = 16 + 4 * per
            o = FK_OFF[k] // 2
            r = _nt(_bf(fk[o:o + n // 2, :]), wtile(k))
            if k in (4, 8):
                e0 = 16 + 2 * per
                v0 = bv[j, 1] if k == 4 else jnp.concatenate([kf[j, 3, 8:16, :]] * 2, axis=0)
                r = jnp.concatenate([v0[0:8], r[8:e0], r[e0:e0 + per] + 0.5 * jnp.concatenate([v0] * (per // 16), axis=0),
                                     r[e0 + per:]], axis=0)
            kf[j, k - 4, 0:n, :] = r

        def nears(ks, v):
            return _group([(functools.partial(near, k, hf), 32, v + extra) for k in ks for hf in range(2)], 4)

        def fars(ks):
            return _group([(functools.partial(far, k), 36 if k < 8 else 20, extra) for k in ks], 4)
        return (nears((1, 3), 8) + fars((12, 13, 14, 15)) + fars((7, 6, 5, 4))
                + nears((0, 2), 28) + fars((9, 10, 11, 8)))

    def udft_pieces(j):
        def piece(ib, qf):
            o = FK_FU // 2 + qf * 32
            w = jnp.concatenate([tile("u", i * 128, 128, slice(j * 128, (j + 1) * 128))
                                 for i in range(ib * 4, ib * 4 + 4)], axis=1)
            r = _nn(_bf(fk[o:o + 32, :]), w)
            rows = slice(qf * 32, qf * 32 + 32)
            for t in range(4):
                rr, ri = r[:32, t * 128:(t + 1) * 128], r[32:, t * 128:(t + 1) * 128]
                u3[j, 0, ib * 4 + t, rows, :] = rr
                u3[j, 1, ib * 4 + t, rows, :] = ri
                u3[j, 2, ib * 4 + t, rows, :] = rr + ri
        return [(functools.partial(piece, ib, qf), 64, 16) for ib in range(4) for qf in range(4)]

    def conv_ops(items):
        return sum((68, 204, 300, 396)[ib] for _, i0, i1 in items for ib in range(i0, i1))

    def conv(items):
        for pos, ib0, ib1 in items:
            j, p = divmod(pos, 16)
            rs = slice(p * 8, p * 8 + 8)
            prev = None if ib0 == 0 else (zc[0, rs, :], zc[1, rs, :])
            for ib in range(ib0, ib1):
                if ib > 0:
                    t0 = 2 if ib == 1 else 5
                    d_od, d_ev, sh = gb[t0, rs, :], gb[t0 + 1, rs, :], gb[t0 + 2, rs, :]
                    per = 32 if ib == 1 else 16
                    h = 16 + (8 * p) % per
                    left = sh * kf[j, 4 * ib - 4, 0:8, :]
                    for k in range(4 * ib, 4 * ib + 4):
                        o_r, o_i, e_r, e_i = (kf[j, k - 4, per * t + h:per * t + h + 8, :] for t in range(4))
                        right = sh * kf[j, k - 4, 8:16, :]
                        rr = d_od * o_r + d_ev * e_r - right
                        ri = d_od * o_i + d_ev * e_i + left
                        left = right
                        kw[j, 0, k, rs, :] = rr
                        kw[j, 1, k, rs, :] = ri
                        kw[j, 2, k, rs, :] = rr + ri
                        if k % 2:
                            yield 20
                a = zr = None
                for c in range(3):
                    acc = [None] * 4
                    for ub_ in range(ib + 1):
                        n = 0
                        uu = [u3[j, c, ub_ * 4 + t, rs, :] for t in range(4)]
                        for dk in range(-3, 4):
                            k = (ib - ub_) * 4 + dk
                            if k < 0:
                                continue
                            kk = kw[j, c, k, rs, :]
                            for t in range(4):
                                o = t + dk
                                if 0 <= o < 4:
                                    pr = kk * uu[t]
                                    if acc[o] is None:
                                        acc[o] = pr - a[o] if c == 2 else pr
                                    else:
                                        acc[o] = acc[o] + pr
                                    n += 2
                        if ub_ < ib:
                            yield n
                    if c == 0:
                        a = acc
                    elif c == 1:
                        zr = [a[o] - acc[o] for o in range(4)]
                        a = [a[o] + acc[o] for o in range(4)]
                    else:
                        for o in range(4):
                            zi = acc[o]
                            if prev is None:
                                yr, yi = zi, -zr[o]
                            else:
                                yr, yi = prev[0] + zi, prev[1] - zr[o]
                            y[j, 0, ib * 4 + o, rs, :] = yr
                            y[j, 1, ib * 4 + o, rs, :] = yi
                            prev = (zr[o], zi)
                        n += 8
                        if ib == ib1 - 1 and ib1 < 4:
                            zc[0, rs, :], zc[1, rs, :] = prev
                    yield n

    def inv_pieces(j):
        def piece(i):
            sub, _ = iotas()
            s = _nn(fi[0:64, :], y[j, 0, i])
            a = _nn(fi[64:128, :], y[j, 1, i])
            lo = s + a
            hi = s - a
            hi = jnp.concatenate(
                [jnp.take_along_axis(hi[8 * v:8 * v + 8], 7 - sub, axis=0) for v in range(7, -1, -1)], axis=0)
            stb[j, i * 128:(i + 1) * 128, :] = jnp.concatenate([lo, hi], axis=0).astype(BF16)
        return _group([(functools.partial(piece, i), 32, 32) for i in range(16)], 2)

    def kt_pieces(pb0, pb1, fb_outer=False):
        def piece(fb, pb):
            pk = _phi(_nt(_bf(wkt[fb * 64:(fb + 1) * 64, :]), tile("x", pb * 128, 128)))
            pkt[fb * 64:(fb + 1) * 64, pb * 128:(pb + 1) * 128] = _pk(pk)
            rows = slice(fb * 128, (fb + 1) * 128)
            if pb == 0:
                zacc[rows, :] = pk
            else:
                zacc[rows, :] += pk
        idx = [(fb, pb) for pb in range(pb0, pb1) for fb in range(4)]
        if fb_outer:
            idx.sort()
        return [(functools.partial(piece, fb, pb), 128, 230) for fb, pb in idx]

    def g_pieces():
        st = {}

        def piece(fb, cb, kb):
            r = _nn(_bf(pkt[fb * 32:(fb + 1) * 32, kb * 512:(kb + 1) * 512]),
                    _bf(xp[kb * 256:(kb + 1) * 256, cb * 128:(cb + 1) * 128]))
            if kb > 0:
                r = r + st["acc"]
            if kb == 3:
                gp[fb * 32:(fb + 1) * 32, cb * 128:(cb + 1) * 128] = _pk(r)
            else:
                st["acc"] = r
        return [(functools.partial(piece, fb, cb, kb), 64, 32)
                for fb in range(8) for cb in range(4) for kb in range(4)]

    def mid_pieces():
        st = {}

        def bd():
            r128 = lax.broadcasted_iota(jnp.int32, (128, 128), 0)
            c128 = lax.broadcasted_iota(jnp.int32, (128, 128), 1)
            return (r128 >> 4) == (c128 >> 4)

        def kv(fb):
            g = fb // 2
            r = _nn(_bf(gp[fb * 32:(fb + 1) * 32, :]), wb[:, 2 * D + g * 128:2 * D + (g + 1) * 128])
            st[fb] = jnp.where(bd()[(fb % 2) * 64:(fb % 2) * 64 + 64], r, 0.0).astype(BF16)

        def mm(fb):
            g = fb // 2
            m = _pk(_nn(st[fb], wob[g * 128:(g + 1) * 128, :]))
            for c in range(4):
                mp[c, fb * 32:(fb + 1) * 32, :] = m[:, c * 128:(c + 1) * 128]

        def zz():
            for g in range(4):
                za = zacc[g * 128:(g + 1) * 128, :]
                z = jnp.sum(za, axis=1, keepdims=True)
                zb[g] = jnp.where(bd(), jnp.broadcast_to(z, (128, 128)), 0.0)
                zpk[g * 64:(g + 1) * 64, :] = _pk(za)
            zrow[...] = _nt(jnp.ones((16, 128), BF16), _bf(perm_rows(zpk)))[0:8]
        return ([(functools.partial(kv, fb), 64, 40) for fb in range(8)],
                [(functools.partial(mm, fb), 64, 16) for fb in range(8)], [(zz, 64, 120)])

    def q_pieces(rb0, rb1):
        def piece(rb, g):
            w = wb[:, g * 128:(g + 1) * 128] if rb < QOLD else _bf(wqp[:, g * 128:(g + 1) * 128])
            pq[rb * 64:(rb + 1) * 64, g * 128:(g + 1) * 128] = _phi(_nn(tile("x", rb * 64, 64), w))
        return [(functools.partial(piece, rb, g), 64, 64) for rb in range(rb0, rb1) for g in range(4)]

    def o_stream(rb0, rb1, q0):
        st = {}

        def den_mxu(rb):
            rows = slice(rb * 64, (rb + 1) * 64)
            for g in range(4):
                cols = slice(g * 128, (g + 1) * 128)
                d = _nn(pq[rows, cols], zb[g]) + 1e-6
                pp[rb * 32:(rb + 1) * 32, cols] = _pk(pq[rows, cols] * pl.reciprocal(d, approx=True))

        def den_vpu(rb):
            _, lane = iotas()
            for v in range(rb * 4, rb * 4 + 4):
                rs = []
                for r0 in (v * 16, v * 16 + 8):
                    t = None
                    for g in range(4):
                        cols = slice(g * 128, (g + 1) * 128)
                        p = pq[r0:r0 + 8, cols] * zrow[:, cols]
                        t = p if t is None else t + p
                    t = t + jnp.take_along_axis(t, lane ^ 2, axis=1)
                    t = t + jnp.take_along_axis(t, lane ^ 1, axis=1)
                    rs.append(pl.reciprocal(t + 1e-6, approx=True))
                r = jnp.concatenate(rs, axis=0)
                for g in range(4):
                    cols = slice(g * 128, (g + 1) * 128)
                    pp[v * 8:v * 8 + 8, cols] = _pk(pq[v * 16:v * 16 + 16, cols] * r)

        def out(rb, g):
            m = mp[g, 0:D // 2, :] if rb < QOLD else perm_rows(mp.at[g])
            r = _nn(_bf(pp[rb * 32:(rb + 1) * 32, :]), _bf(m))
            if g % 2 == 0:
                st["r"] = r
            else:
                sta[rb * 64:(rb + 1) * 64, (g - 1) * 128:(g + 1) * 128] = jnp.concatenate(
                    [st["r"], r], axis=1).astype(BF16)

        res = []
        for t in range(rb0 - 2, rb1):
            step = []
            ov = 60 if t + 1 >= q0 else 28
            if q0 <= t + 2 < rb1:
                step += q_pieces(t + 2, t + 3)
            if rb0 <= t:
                step += [(functools.partial(out, t, g), 64, ov) for g in (0, 1)]
            if rb0 <= t + 1 < rb1:
                step.append((functools.partial(den_mxu, t + 1), 64, 80) if t + 1 < QOLD
                            else (functools.partial(den_vpu, t + 1), 0, 128))
            if rb0 <= t:
                step += [(functools.partial(out, t, g), 64, ov) for g in (2, 3)]
            res.append(step)

        def seg(a, b):
            return [p for step in res[a - rb0 + 2:b - rb0 + 2] for p in step]
        return seg

    prm_hbm = (are_hbm, aim_hbm, bre_hbm, bim_hbm, cre_hbm, cim_hbm)

    def prm_rest(i):
        return prm_hbm[i].at[R0:D], prm.at[i, R0:D]

    srcs = {"ldt": (ldt_hbm, ldt)}
    srcs.update({"a%d" % i: (prm_hbm[i].at[0:R0], prm.at[i, 0:R0]) for i in range(6)})
    srcs.update({
        "wq": (w_hbm.at[:, 0:D], wb.at[:, 0:D]),
        "x0": (x_hbm.at[0:X0], xb.at[0:X0]),
        "dsk": (dsk_hbm, dsk),
        "p0": prm_rest(0),
        "p1": prm_rest(1),
        "wk": (w_hbm.at[:, D:2 * D], wb.at[:, D:2 * D]),
        "p2": prm_rest(2),
        "p3": prm_rest(3),
        "p4": prm_rest(4),
        "p5": prm_rest(5),
        "x1": (x_hbm.at[X0:X1], xb.at[X0:X1]),
        "fi": (fi_hbm, fi),
        "fk": (fk_hbm, fk),
        "ua": (u_hbm.at[:, 0:256], ub.at[:, 0:256]),
        "x2": (x_hbm.at[X1:S], xb.at[X1:S]),
        "ub": (u_hbm.at[:, 256:D], ub.at[:, 256:D]),
        "wv": (w_hbm.at[:, 2 * D:3 * D], wb.at[:, 2 * D:3 * D]),
        "wo": (wo_hbm, wob),
    })
    cin = {k: pltpu.make_async_copy(a, b, sem_in.at[i]) for i, (k, (a, b)) in enumerate(srcs.items())}
    for c in cin.values():
        c.start()
    couts = []

    def wait(*names):
        for n in names:
            cin[n].wait()

    def out_copy(i, kind, a, b):
        if kind == "a":
            return pltpu.make_async_copy(sta.at[a * 64:b * 64], o_hbm.at[a * 64:b * 64, 0:D], sem_out.at[i])
        c0 = D + kind * 128
        return pltpu.make_async_copy(stb.at[kind, a * 128:b * 128],
                                     o_hbm.at[a * 128:b * 128, c0:c0 + 128], sem_out.at[i])

    def store(*box):
        out_copy(len(couts), *box).start()
        couts.append(box)

    q0, q1 = X0 // 64, X1 // 64
    p0, p1 = X0 // 128, X1 // 128
    qe = q_pieces(q1, q1 + 3)
    mid1, mid2, midz = mid_pieces()
    gps = g_pieces()
    gs = []
    for fb in range(8):
        blk = gps[fb * 16:(fb + 1) * 16]
        if fb:
            blk = blk[:4] + [mid1[fb - 1]] + blk[4:9] + [mid2[fb - 1]] + blk[9:]
        gs += blk
    kds = [kdft_pieces(j, 20 if j >= 2 else 0) for j in range(4)]
    uds = [udft_pieces(j) for j in range(4)]
    cv = [[(p, 0, 4) for p in range(32)],
          [(p, 0, 4) for p in range(32, 48)],
          [(p, 0, 3) for p in range(48, 64)] + [(p, 3, 4) for p in range(48, C3)],
          [(p, 3, 4) for p in range(C3, 64)]]
    oseg = o_stream(0, O3, q1 + 3)
    oseg2 = o_stream(O3, 32, O3)

    main3 = uds[0][:8] + [(k0_all, 8, 0)] + uds[0][8:] + kds[0] + uds[1][:10] + kds[1] + uds[1][10:]
    blk3 = main3[:3] + _merge(main3[3:-4], kgen_pieces(G0, 64)) + main3[-4:]
    blk4 = (_merge(kt_pieces(p1, 16), uds[2][:13]) + uds[2][13:]
            + _merge(gs[:GS], midz + kds[2] + kds[3], uds[3]))
    blk5 = _merge(gs[GS:] + qe[:4] + [mid1[7]] + oseg(-2, 0) + qe[4:8] + [mid2[7]] + qe[8:] + oseg(0, O1),
                  inv_pieces(0) + inv_pieces(1))
    blk5 = [(f, c, v + (50 if 8 <= i < 32 else 0)) for i, (f, c, v) in enumerate(blk5)]
    last = oseg2(O4, 32)
    ta = oseg2(O3, O4)
    blk8 = oseg2(O3 - 2, O3) + ta[:-5] + inv_pieces(3)[6:] + [p for p in last if p[1] == 0] + ta[-5:]
    blk9 = [p for p in last if p[1] != 0]

    steps = [
        (lambda: wait("ldt"), lambda: setup_dt(0, 1)),
        (lambda: wait("a0", "a1", "a2", "a3", "a4", "a5"), early_prep),
        (early_exact, lambda: _emit(kgen_pieces(0, G0))),
        (lambda: wait("wq", "x0", "dsk"),
         lambda: (setup_dt(1, 4), wq_perm_a(), _emit(q_pieces(0, q0 - 1)))),
        (lambda: wait("p0", "p1", "wk"),
         lambda: (wk_transpose(), range_check(0, R0, D),
                  _emit(q_pieces(q0 - 1, q0) + kt_pieces(0, p0, True), stage1(), (32 - G0 // 2) * 90))),
        (lambda: (stage1_exact(), wait("p2", "p3", "p4", "p5", "x1")),
         lambda: (wq_perm_b(),
                  _emit(kt_pieces(p0, p1) + q_pieces(q0, q1), stage2_fill(G0 // 2, 32), (32 - G0 // 2) * 164))),
        (lambda: wait("fi", "fk", "ua"), lambda: (setup_g(), _emit(blk3))),
        (lambda: wait("x2", "ub", "wv", "wo"), lambda: _emit(blk4, conv(cv[0]), conv_ops(cv[0]))),
        (None, lambda: _emit(blk5, conv(cv[1]), conv_ops(cv[1]))),
        (lambda: (store(0, 0, 16), store(1, 0, 16), store("a", 0, O1)),
         lambda: _emit(_merge(oseg(O1, O2), inv_pieces(2)), conv(cv[2]), conv_ops(cv[2]))),
        (lambda: (store(2, 0, 16), store("a", O1, O2)),
         lambda: _emit(_merge(oseg(O2, O3), inv_pieces(3)[:6]), conv(cv[3]), conv_ops(cv[3]))),
        (lambda: (store(3, 0, 12), store("a", O2, O3)), lambda: _emit(blk8)),
        (lambda: (store(3, 12, 16), store("a", O3, O4)), lambda: _emit(blk9)),
        (lambda: store("a", O4, 32), None),
    ]

    def outer(i, c):
        packed.clear()
        couts.clear()
        for k, fn in enumerate(f for step in steps for f in step):
            if fn is not None:
                @pl.when(i + k == k)
                def _():
                    fn()
        return c

    lax.fori_loop(0, 2, outer, 0)
    for i, box in enumerate(couts):
        out_copy(i, *box).wait()


@jax.jit
def pallas_concat_heads__linear_attn_block__ssm_conv_s4__prompt_kernel(
    A_x, A_wqkv, A_wo, B_u, B_A_re, B_A_im, B_B_re, B_B_im, B_C_re, B_C_im, B_log_dt, B_Dskip,
):
    fk, fi = _tables()
    V = pltpu.VMEM
    out = pl.pallas_call(
        _kernel,
        out_shape=jax.ShapeDtypeStruct((S, 2 * D), BF16),
        in_specs=[pl.BlockSpec(memory_space=pl.ANY)] * 14,
        out_specs=pl.BlockSpec(memory_space=pl.ANY),
        scratch_shapes=[
            V((S // 2, D), U32),
            V((D, 3 * D), BF16),
            V((D, D), BF16),
            V((S // 2, D), U32),
            V((6, D, 128), BF16),
            V((D,), BF16),
            V((D,), BF16),
            V((S, D), BF16),
            V((S, D), BF16),
            V((FK_ROWS // 2, 128), U32),
            V((136, 128), F32),
            V((S, D), BF16),
            V((4, S, 128), BF16),
            V((2, D, 128), F32),
            pltpu.SMEM((2,), jnp.int32),
            V((D, 128), F32),
            V((8, 128, 128), F32),
            V((14, 2 * D + 8, 128), F32),
            V((D, 128), F32),
            V((5, D // 2, 128), U32),
            V((4, 2, 16, 128), F32),
            V((8, D), F32),
            V((4, 3, 16, 128, 128), F32),
            V((4, 3, 16, 128, 128), F32),
            V((4, 2, 16, 128, 128), F32),
            V((D // 2, D), U32),
            V((D // 2, S), U32),
            V((D, 128), F32),
            V((D // 2, D), U32),
            V((4, D // 2 + 8, 128), U32),
            V((4, 128, 128), F32),
            V((S, D), F32),
            V((S // 2, D), U32),
            V((4, D // 2 + 8, 128), U32),
            V((D // 2, D), U32),
            V((D // 2 + 8, 128), U32),
            V((8, D), F32),
            V((4, 12, 144, 128), F32),
            V((2, 128, 128), F32),
            pltpu.SemaphoreType.DMA((25,)),
            pltpu.SemaphoreType.DMA((10,)),
        ],
        compiler_params=pltpu.CompilerParams(vmem_limit_bytes=110 * 2**20, disable_semaphore_checks=True),
    )(A_x.reshape(S, D), A_wqkv, A_wo, B_u.reshape(S, D), B_A_re, B_A_im, B_B_re, B_B_im, B_C_re, B_C_im,
      B_log_dt, B_Dskip, jnp.asarray(fk), jnp.asarray(fi))
    return out.reshape(1, S, 2 * D)
```

```python
import functools

import numpy as np
import jax
import jax.numpy as jnp
from jax import lax
import jax.experimental.pallas as pl
import jax.experimental.pallas.tpu as pltpu

S = 2048
D = 512
F32 = jnp.float32
BF16 = jnp.bfloat16
U32 = jnp.uint32

_BASE = np.array([[1, 5], [2, 6], [3, 7], [4, 8], [258, 262], [260, 264],
                  [516, 520], [772, 776], [1032, 1288], [1544, 1800]])
_TILE_OF_CHUNK = [0, 1, 2, 2, 3, 3, 3, 3] + [4] * 8

FK_OFF = [0, 256, 528, 784] + [1056 + 144 * k for k in range(4)] + [1632 + 80 * k for k in range(8)]
FK_FU = 1632 + 640
FK_ROWS = FK_FU + 256

X0, X1 = 384, 896
QOLD = X0 // 64
G0 = 12
R0 = 8 * G0
O1, O2, O3, O4 = 15, 24, 29, 31
GS = 120
C3 = 52

B_W1, B_W2, B_W8C, B_W256, B_W512, B_E0, B_N0 = range(7)
_SC_LIMIT = 8192.0


def _bf16_bits(v):
    u = np.ascontiguousarray(v, np.float32).view(np.uint32)
    return ((u + 0x7FFF + ((u >> 16) & 1)) >> 16).astype(np.uint32)


def _pack_rows(v):
    b = _bf16_bits(v)
    return b[0::2] | (b[1::2] << 16)


@functools.lru_cache(maxsize=None)
def _tables():
    lr = (_bf16_bits(np.arange(S)) << 16).view(np.float32).astype(np.int64)
    val = np.zeros((5, 128), np.int64)
    for lam in range(128):
        mu, tau = 15 - (lam >> 3), lam & 7
        e, x = tau >> 1, tau & 1
        for h in range(2):
            val[h, lam] = _BASE[e, x ^ h] + 8 * (mu + 16 * h)
        hp, ab, h = tau >> 2, (tau >> 1) & 1, tau & 1
        for q in range(3):
            val[2 + q, lam] = _BASE[4 + 2 * q + ab, hp] + 8 * (mu + 16 * h)
    om = 2 * np.pi * (np.arange(128) + 0.25) / 128.0
    phase = np.exp(1j * om * 191.5)

    def stack(z):
        return np.concatenate([p[32 * t:32 * t + 32] for t in range(4) for p in (z.real, z.imag)], axis=0)

    fk = []
    g = np.zeros(128, np.complex128)
    for k in range(4):
        slot = {int(v): i for i, v in enumerate(val[_TILE_OF_CHUNK[k]])}
        m = np.zeros((128, 128), np.complex128)
        for p in range(1, 129):
            lag = 128 * k + p
            v = int(lr[lag])
            z = np.exp(-1j * om * p) * (0.5 if lag == 512 else 1.0)
            if v in slot:
                m[:, slot[v]] += z
            else:
                assert v == 256 and k == 2
                g += z
        if k in (1, 3):
            sel = np.zeros((16, 128))
            sel[:, slot[128 * (k + 1)]] = 1.0
            fk += [stack(m)[:128], sel, stack(m)[128:]]
        else:
            fk.append(stack(m))
    for k in range(4, 16):
        st = 4 if k < 8 else 8
        per = 128 // st
        slot = {int(v): i for i, v in enumerate(val[_TILE_OF_CHUNK[k]])}
        for lag in range(128 * k + 1, min(128 * k + 128, S)):
            m_ = int(lr[lag]) // st
            assert int(lr[lag]) % st == 0 and abs(lag - st * m_) <= (st // 2 if m_ % 2 == 0 else st // 2 - 1)
        od = np.zeros((per, 128), np.complex128)
        ev = np.zeros((per, 128), np.complex128)
        edge = np.zeros((16, 128))
        for m_ in range(per + 1):
            v = 128 * k + st * m_
            if v not in slot:
                assert m_ == 0 and k in (4, 8)
                continue
            z = np.exp(-1j * om[:per] * st * m_)
            if m_ % 2:
                od[:, slot[v]] = z
            else:
                ev[:, slot[v]] = z * (0.5 if m_ in (0, per) else 1.0)
            if m_ in (0, per):
                edge[8 * (m_ // per):8 * (m_ // per) + 8, slot[v]] = 1.0
        fk += [edge, od.real, od.imag, ev.real, ev.imag]
    fk.append(stack(np.exp(-1j * om[:, None] * np.arange(128)[None, :]) * phase[:, None]))
    fk = np.concatenate(fk, axis=0)
    assert fk.shape[0] == FK_ROWS
    tabs = [g.real, g.imag]
    for h in (2, 4):
        tabs += [sum(np.cos(om * p) for p in range(1 - h, h)), sum(np.cos(om * p) for p in range(-h, h + 1)),
                 -sum(np.sin(om * p) for p in range(1, h + 1))]
    jj = np.arange(64)[:, None] - 63.5
    finv = np.concatenate([np.cos(om[None, :] * jj) / 128.0, -np.sin(om[None, :] * jj) / 128.0,
                           np.stack(tabs)], axis=0)
    return _pack_rows(fk), finv.astype(np.float32)


def _cmul(a, b):
    return a[0] * b[0] - a[1] * b[1], a[0] * b[1] + a[1] * b[0]


def _csq(a):
    return a[0] * a[0] - a[1] * a[1], (a[0] + a[0]) * a[1]


def _phi(t):
    return jnp.where(t > 0, t + 1.0, jnp.exp(t)) + 1e-6


def _nt(a, b):
    return lax.dot_general(a, b, (((1,), (1,)), ((), ())), preferred_element_type=F32)


def _nn(a, b):
    return jnp.dot(a, b, preferred_element_type=F32)


def _bf(v):
    return pltpu.bitcast(v, BF16)


def _pk(v):
    return pltpu.bitcast(v.astype(BF16), U32)


def _sincos(x):
    t = x * 0.6366197723675814 + 12582912.0
    n = pltpu.bitcast(t, jnp.int32) - 0x4B400000
    k = n.astype(F32)
    r = ((x - k * 1.5703125) - k * 4.837512969970703125e-4) - k * 7.54978995489188216e-8
    r2 = r * r
    sn = r + r * r2 * (-1.6666654611e-1 + r2 * (8.3321608736e-3 + r2 * -1.9515295891e-4))
    cs = 1.0 + r2 * (-0.5 + r2 * (4.166664568298827e-2 + r2 * (-1.388731625493765e-3 + r2 * 2.443315711809948e-5)))
    swap = (n & 1) == 1
    s_, c_ = jnp.where(swap, cs, sn), jnp.where(swap, sn, cs)
    ssign = (n & 2) << 30
    csign = ((n + 1) & 2) << 30
    s_ = pltpu.bitcast(pltpu.bitcast(s_, jnp.int32) ^ ssign, F32)
    c_ = pltpu.bitcast(pltpu.bitcast(c_, jnp.int32) ^ csign, F32)
    return s_, c_


def _emit(pieces, filler=None, fill_total=0, cap=3.0, tail=100):
    filler = iter(()) if filler is None else filler
    room = [max(cap * c - v, 0.0) for _, c, v in pieces]
    tot = sum(room[:-1]) or 1.0
    done, target = 0.0, 0.0
    for (fn, _, _), r in zip(pieces, room):
        fn()
        target += max(fill_total - tail, 0) * r / tot
        while done < target - 8:
            n = next(filler, None)
            if n is None:
                break
            done += n
    for _ in filler:
        pass


def _merge(*lists):
    tot = [sum(p[1] for p in l) or 1.0 for l in lists]
    pos = [0] * len(lists)
    acc = [0.0] * len(lists)
    out = []
    while True:
        best = None
        for i, l in enumerate(lists):
            if pos[i] < len(l):
                key = (acc[i] + 0.5 * l[pos[i]][1]) / tot[i]
                if best is None or key < best[0]:
                    best = (key, i)
        if best is None:
            return out
        i = best[1]
        out.append(lists[i][pos[i]])
        acc[i] += lists[i][pos[i]][1]
        pos[i] += 1


def _group(pieces, n):
    out = []
    for i in range(0, len(pieces), n):
        grp = pieces[i:i + n]

        def run(grp=grp):
            for f, _, _ in grp:
                f()
        out.append((run, sum(p[1] for p in grp), sum(p[2] for p in grp)))
    return out


def _reim(r):
    n = r.shape[0] // 64
    return (jnp.concatenate([r[64 * t:64 * t + 32] for t in range(n)], axis=0),
            jnp.concatenate([r[64 * t + 32:64 * t + 64] for t in range(n)], axis=0))


def _kernel(x_hbm, w_hbm, wo_hbm, u_hbm, are_hbm, aim_hbm, bre_hbm, bim_hbm, cre_hbm, cim_hbm,
            ldt_hbm, dsk_hbm, fk_hbm, fi_hbm, o_hbm,
            xp, wb, wob, up, prm, ldt, dsk, xb, ub, fk, fi, sta, stb, w1s, flag,
            dtb, gb, base, cr, wt, bv, k0s, kw, u3, y, wkt, pkt, zacc, gp, mp, zb, pq, pp,
            wqt, wqp, zpk, zrow, kf, zc, sem_in, sem_out):

    def iotas():
        return (lax.broadcasted_iota(jnp.int32, (8, 128), 0), lax.broadcasted_iota(jnp.int32, (8, 128), 1))

    packed = set()

    def tile(kind, r0, n, cols=slice(None)):
        src, dst = (xb, xp) if kind == "x" else (ub, up)
        parts = []
        for r in range(r0, r0 + n, 64):
            key = (kind, r, cols.start)
            if key in packed:
                parts.append(_bf(dst[r // 2:r // 2 + 32, cols]))
            else:
                packed.add(key)
                v = src[r:r + 64, cols]
                dst[r // 2:r // 2 + 32, cols] = pltpu.bitcast(v, U32)
                parts.append(v)
        return parts[0] if len(parts) == 1 else jnp.concatenate(parts, axis=0)

    def dt_row():
        return jnp.exp(ldt[...].reshape(1, D).astype(F32)).astype(BF16).astype(F32)

    def setup_dt_first():
        sub, _ = iotas()
        b = jnp.broadcast_to(dt_row()[:, 0:128], (8, 128))
        for v in range(16):
            dtb[v * 8:v * 8 + 8, :] = jnp.take_along_axis(b, sub + 8 * v, axis=1)

    def setup_dt_rest():
        row = dt_row()
        for j in range(1, 4):
            dtb[j * 128:(j + 1) * 128, :] = jnp.broadcast_to(row[:, j * 128:(j + 1) * 128], (128, 128)).T

    def setup_g():
        for i in range(8):
            gb[i] = jnp.broadcast_to(fi[128 + i:129 + i, :], (128, 128)).T

    def perm_rows(ref):
        return jnp.concatenate([ref[pl.ds(t, 64, stride=4), :] for t in range(4)], axis=0)

    def wq_perm_a():
        for a in range(4):
            for b in range(4):
                t = wb[a * 128:(a + 1) * 128, b * 128:(b + 1) * 128].T
                wqt[a, b * 64:(b + 1) * 64, :] = pltpu.bitcast(t, U32)

    def wq_perm_b():
        for b in range(4):
            for a in range(4):
                t = _bf(wqt[a, pl.ds(b, 64, stride=4), :]).T
                wqp[a * 64:(a + 1) * 64, b * 128:(b + 1) * 128] = pltpu.bitcast(t, U32)

    def wk_transpose():
        for b in range(4):
            for a in range(4):
                t = wb[a * 128:(a + 1) * 128, D + b * 128:D + (b + 1) * 128].T
                wkt[b * 64:(b + 1) * 64, a * 128:(a + 1) * 128] = pltpu.bitcast(t, U32)

    def w1_rows(r0, exact):
        rows = pl.ds(r0, 16)
        dt = dtb[rows, :]
        ar = dt * prm[0, rows, :].astype(F32)
        ai = dt * prm[1, rows, :].astype(F32)
        mag = jnp.exp(ar)
        sn, cs = (jnp.sin(ai), jnp.cos(ai)) if exact else _sincos(ai)
        w1s[0, rows, :] = mag * cs
        w1s[1, rows, :] = mag * sn

    def range_check(i, r0, r1):
        m = jnp.max(jnp.abs(prm[1, r0:r1, :].astype(F32)).reshape((r1 - r0) // 8, 8, 128), axis=0)
        dmax = jnp.max(dtb[r0:r1, :].reshape((r1 - r0) // 8, 8, 128), axis=0)
        bound = jnp.max(m) * jnp.max(dmax)
        flag[i] = jnp.where(bound <= _SC_LIMIT, 0, 1).astype(jnp.int32)

    def stage1():
        for r in range(G0 // 2, 32):
            w1_rows(r * 16, False)
            yield 90

    def stage1_exact():
        @pl.when(flag[0] != 0)
        def _():
            def body(r, c):
                w1_rows(pl.multiple_of(r * 16, 16), True)
                return c
            lax.fori_loop(G0 // 2, 32, body, 0)

    def stage2(r):
        r0 = r * 16 if isinstance(r, int) else pl.multiple_of(r * 16, 16)
        rows = pl.ds(r0, 16)
        dt = dtb[rows, :]
        w1 = (w1s[0, rows, :], w1s[1, rows, :])
        db = (dt * prm[2, rows, :].astype(F32), dt * prm[3, rows, :].astype(F32))
        c = _cmul((prm[4, rows, :].astype(F32), prm[5, rows, :].astype(F32)), db)
        cr[rows, :] = c[0]
        lo = (lax.broadcasted_iota(jnp.int32, (16, 128), 0) & 4) == 0

        def put(i, v0, v1=None):
            for t in range(2):
                ev, od = (v0[t], v0[t]) if v1 is None else (jnp.where(lo, v0[t], v1[t]), jnp.where(lo, v1[t], v0[t]))
                base[2 * i + t, pl.ds(2 * r0, 16, stride=2), :] = ev
                base[2 * i + t, pl.ds(2 * r0 + 1, 16, stride=2), :] = od
        put(B_W1, w1)
        w2 = _csq(w1)
        put(B_W2, w2)
        w4 = _csq(w2)
        cw1 = _cmul(c, w1)
        put(B_N0, cw1, _cmul(cw1, w4))
        yield 80
        w8 = _csq(w4)
        put(B_W8C, (w8[0], -w8[1]))
        w128 = _csq(_csq(_csq(_csq(w8))))
        put(B_E0, (jnp.ones((16, 128), F32), jnp.zeros((16, 128), F32)), (w128[0], -w128[1]))
        w256 = _csq(w128)
        put(B_W256, w256)
        put(B_W512, _csq(w256))
        yield 84

    def stage2_fill(r0, r1):
        for r in range(r0, r1):
            yield from stage2(r)

    def early_prep():
        range_check(1, 0, R0)
        for r in range(G0 // 2):
            w1_rows(r * 16, False)
        for _ in stage2_fill(0, G0 // 2):
            pass

    def early_exact():
        @pl.when(flag[1] != 0)
        def _():
            def body(r, c):
                w1_rows(pl.multiple_of(r * 16, 16), True)
                for _ in stage2(r):
                    pass
                return c
            lax.fori_loop(0, G0 // 2, body, 0)

    def kgen_pieces(g0, g1):
        st = {}

        def half(gi, g):
            sub, lane = iotas()
            odd = (sub & 1) == 1
            rows = slice(gi * 16 + g * 8, gi * 16 + g * 8 + 8)

            def ld(i):
                return base[2 * i, rows, :], base[2 * i + 1, rows, :]
            hi = odd if g == 0 else jnp.logical_not(odd)
            w8c = ld(B_W8C)
            e0 = [ld(B_E0)]
            for _ in range(1, 16):
                e0.append(_cmul(e0[-1], w8c))
            e0 = e0[::-1]
            w1, w2, w256, w512 = ld(B_W1), ld(B_W2), ld(B_W256), ld(B_W512)
            n0 = ld(B_N0)
            n1 = _cmul(n0, w1)
            n2 = _cmul(n0, w2)
            n3 = _cmul(n1, w2)
            n4 = _cmul(n1, w256)
            n5 = _cmul(n3, w256)
            n6 = _cmul(n5, w256)
            n7 = _cmul(n6, w256)
            sh = 7 if g == 0 else 1
            t = (jnp.where(hi, n7[0], pltpu.roll(n6[0], sh, 0)), jnp.where(hi, n7[1], pltpu.roll(n6[1], sh, 0)))
            n8 = _cmul(t, w512)
            n9 = _cmul(n8, w512)
            e1 = [n0, n1, n2, n3, n4, n5, n6, n7, n8, n9]
            lhs = jnp.concatenate([jnp.concatenate([v[0] for v in e1], axis=0),
                                   jnp.concatenate([v[1] for v in e1], axis=0)], axis=1)
            rhs = jnp.concatenate([jnp.concatenate([v[0] for v in e0], axis=0),
                                   jnp.concatenate([v[1] for v in e0], axis=0)], axis=1)
            o = _nt(lhs, rhs)
            o = [o[8 * i:8 * i + 8, :] for i in range(10)]

            emask = ((sub >> 1) - (lane >> 1)) & 3
            ea, xa = (lane >> 1) & 3, lane & 1
            lidx_a = (lane & 120) | ((((sub >> 1) - ea) & 3) << 1) | (xa ^ (sub & 1))
            sidx_a = ((((sub & 3) + ea) & 3) << 1) | (xa ^ (sub >> 2))

            def put(acc, src, e):
                if e == 0:
                    return src
                return jnp.where(emask == e, pltpu.roll(src, 2 * e, 0), acc)

            s = None
            for e in range(4):
                s = put(s, o[e], e)
            s = jnp.take_along_axis(s, lidx_a, axis=1)
            a2 = jnp.take_along_axis(s, sidx_a, axis=0)
            if g == 0:
                st["a"] = a2
                st["b"] = [put(o[4 + 2 * q], o[5 + 2 * q], 1) for q in range(3)]
                return
            hp, ab, hh = (lane >> 2) & 1, (lane >> 1) & 1, lane & 1
            gg = hp ^ (sub & 1)
            lidx_b = (lane & 120) | ((((sub >> 1) - (2 * gg + ab)) & 3) << 1) | (hh ^ gg)
            g2 = sub >> 2
            sidx_b = ((((sub & 3) + 2 * g2 + ab) & 3) << 1) | (hp ^ g2)
            lo = sub < 4
            res = [jnp.where(lo, st["a"], a2), pltpu.roll(jnp.where(lo, a2, st["a"]), 4, 0)]
            for q in range(3):
                s = put(put(st["b"][q], o[4 + 2 * q], 2), o[5 + 2 * q], 3)
                s = jnp.take_along_axis(s, lidx_b, axis=1)
                res.append(jnp.take_along_axis(s, sidx_b, axis=0))
            if gi % 2 == 0:
                st["r"] = res
            else:
                for q in range(5):
                    wt[q, (gi // 2) * 8:(gi // 2) * 8 + 8, :] = _pk(jnp.concatenate([st["r"][q], res[q]], axis=0))

        return _group([(functools.partial(half, gi, g), 40, 180) for gi in range(g0, g1) for g in range(2)], 2)

    def k0_all():
        k0s[...] = _nt(jnp.ones((8, 128), F32), cr[...]) + dsk[...].reshape(1, D).astype(F32)

    def kdft_pieces(j, extra):
        def wtile(k):
            return _bf(wt[_TILE_OF_CHUNK[k], j * 64:(j + 1) * 64, :])

        def near(k, hf):
            o = FK_OFF[k] // 2 + hf * 64
            if k in (1, 3):
                r = _nt(_bf(fk[o:o + 72, :]), wtile(k))
                bv[j, k // 2, hf * 8:hf * 8 + 8, :] = r[128:136] if hf == 0 else r[0:8]
                r = r[:128] if hf == 0 else r[16:]
            else:
                r = _nt(_bf(fk[o:o + 64, :]), wtile(k))
            rr, ri = _reim(r)
            rows = slice(hf * 64, hf * 64 + 64)
            if k == 0:
                rr = rr + jnp.concatenate([k0s[:, j * 128:(j + 1) * 128]] * 8, axis=0)
            elif k == 2:
                bval = jnp.concatenate([bv[j, 0]] * 4, axis=0)
                rr = rr + gb[0, rows, :] * bval
                ri = ri + gb[1, rows, :] * bval
            kw[j, 0, k, rows, :] = rr
            kw[j, 1, k, rows, :] = ri
            kw[j, 2, k, rows, :] = rr + ri

        def far(k):
            per = 32 if k < 8 else 16
            n = 16 + 4 * per
            o = FK_OFF[k] // 2
            r = _nt(_bf(fk[o:o + n // 2, :]), wtile(k))
            if k in (4, 8):
                e0 = 16 + 2 * per
                v0 = bv[j, 1] if k == 4 else jnp.concatenate([kf[j, 3, 8:16, :]] * 2, axis=0)
                r = jnp.concatenate([v0[0:8], r[8:e0], r[e0:e0 + per] + 0.5 * jnp.concatenate([v0] * (per // 16), axis=0),
                                     r[e0 + per:]], axis=0)
            kf[j, k - 4, 0:n, :] = r

        def nears(ks, v):
            return _group([(functools.partial(near, k, hf), 32, v + extra) for k in ks for hf in range(2)], 4)

        def fars(ks):
            return _group([(functools.partial(far, k), 36 if k < 8 else 20, extra) for k in ks], 4)
        return (nears((1, 3), 8) + fars((12, 13, 14, 15)) + fars((7, 6, 5, 4))
                + nears((0, 2), 28) + fars((9, 10, 11, 8)))

    def udft_pieces(j):
        def piece(ib, qf):
            o = FK_FU // 2 + qf * 32
            w = jnp.concatenate([tile("u", i * 128, 128, slice(j * 128, (j + 1) * 128))
                                 for i in range(ib * 4, ib * 4 + 4)], axis=1)
            r = _nn(_bf(fk[o:o + 32, :]), w)
            rows = slice(qf * 32, qf * 32 + 32)
            for t in range(4):
                rr, ri = r[:32, t * 128:(t + 1) * 128], r[32:, t * 128:(t + 1) * 128]
                u3[j, 0, ib * 4 + t, rows, :] = rr
                u3[j, 1, ib * 4 + t, rows, :] = ri
                u3[j, 2, ib * 4 + t, rows, :] = rr + ri
        return [(functools.partial(piece, ib, qf), 64, 16) for ib in range(4) for qf in range(4)]

    def conv_ops(items):
        return sum((68, 204, 300, 396)[ib] for _, i0, i1 in items for ib in range(i0, i1))

    def conv(items):
        for pos, ib0, ib1 in items:
            j, p = divmod(pos, 16)
            rs = slice(p * 8, p * 8 + 8)
            prev = None if ib0 == 0 else (zc[0, rs, :], zc[1, rs, :])
            for ib in range(ib0, ib1):
                if ib > 0:
                    t0 = 2 if ib == 1 else 5
                    d_od, d_ev, sh = gb[t0, rs, :], gb[t0 + 1, rs, :], gb[t0 + 2, rs, :]
                    per = 32 if ib == 1 else 16
                    h = 16 + (8 * p) % per
                    left = sh * kf[j, 4 * ib - 4, 0:8, :]
                    for k in range(4 * ib, 4 * ib + 4):
                        o_r, o_i, e_r, e_i = (kf[j, k - 4, per * t + h:per * t + h + 8, :] for t in range(4))
                        right = sh * kf[j, k - 4, 8:16, :]
                        rr = d_od * o_r + d_ev * e_r - right
                        ri = d_od * o_i + d_ev * e_i + left
                        left = right
                        kw[j, 0, k, rs, :] = rr
                        kw[j, 1, k, rs, :] = ri
                        kw[j, 2, k, rs, :] = rr + ri
                        if k % 2:
                            yield 20
                a = zr = None
                for c in range(3):
                    acc = [None] * 4
                    uc = {}
                    n = 0
                    for k in range(4 * ib + 4):
                        kk = kw[j, c, k, rs, :]
                        for o in range(4):
                            t = 4 * ib + o - k
                            if t < 0:
                                continue
                            if t not in uc:
                                uc[t] = u3[j, c, t, rs, :]
                            pr = uc[t] * kk
                            if acc[o] is None:
                                acc[o] = pr - a[o] if c == 2 else pr
                            else:
                                acc[o] = acc[o] + pr
                            n += 2
                        if k % 4 == 3 and k < 4 * ib:
                            yield n
                            n = 0
                    if c == 0:
                        a = acc
                    elif c == 1:
                        zr = [a[o] - acc[o] for o in range(4)]
                        a = [a[o] + acc[o] for o in range(4)]
                    else:
                        for o in range(4):
                            zi = acc[o]
                            if prev is None:
                                yr, yi = zi, -zr[o]
                            else:
                                yr, yi = prev[0] + zi, prev[1] - zr[o]
                            y[j, 0, ib * 4 + o, rs, :] = yr
                            y[j, 1, ib * 4 + o, rs, :] = yi
                            prev = (zr[o], zi)
                        n += 8
                        if ib == ib1 - 1 and ib1 < 4:
                            zc[0, rs, :], zc[1, rs, :] = prev
                    yield n

    def inv_pieces(j):
        def piece(i):
            sub, _ = iotas()
            s = _nn(fi[0:64, :], y[j, 0, i])
            a = _nn(fi[64:128, :], y[j, 1, i])
            lo = s + a
            hi = s - a
            hi = jnp.concatenate(
                [jnp.take_along_axis(hi[8 * v:8 * v + 8], 7 - sub, axis=0) for v in range(7, -1, -1)], axis=0)
            stb[j, i * 128:(i + 1) * 128, :] = jnp.concatenate([lo, hi], axis=0).astype(BF16)
        return _group([(functools.partial(piece, i), 32, 32) for i in range(16)], 2)

    def kt_pieces(pb0, pb1, fb_outer=False):
        def piece(fb, pb):
            pk = _phi(_nt(_bf(wkt[fb * 64:(fb + 1) * 64, :]), tile("x", pb * 128, 128)))
            pkt[fb * 64:(fb + 1) * 64, pb * 128:(pb + 1) * 128] = _pk(pk)
            rows = slice(fb * 128, (fb + 1) * 128)
            if pb == 0:
                zacc[rows, :] = pk
            else:
                zacc[rows, :] += pk
        idx = [(fb, pb) for pb in range(pb0, pb1) for fb in range(4)]
        if fb_outer:
            idx.sort()
        return [(functools.partial(piece, fb, pb), 128, 230) for fb, pb in idx]

    def g_pieces():
        st = {}

        def piece(fb, cb, kb):
            r = _nn(_bf(pkt[fb * 32:(fb + 1) * 32, kb * 512:(kb + 1) * 512]),
                    _bf(xp[kb * 256:(kb + 1) * 256, cb * 128:(cb + 1) * 128]))
            if kb > 0:
                r = r + st["acc"]
            if kb == 3:
                gp[fb * 32:(fb + 1) * 32, cb * 128:(cb + 1) * 128] = _pk(r)
            else:
                st["acc"] = r
        return [(functools.partial(piece, fb, cb, kb), 64, 32)
                for fb in range(8) for cb in range(4) for kb in range(4)]

    def mid_pieces():
        st = {}

        def bd():
            r128 = lax.broadcasted_iota(jnp.int32, (128, 128), 0)
            c128 = lax.broadcasted_iota(jnp.int32, (128, 128), 1)
            return (r128 >> 4) == (c128 >> 4)

        def kv(fb):
            g = fb // 2
            r = _nn(_bf(gp[fb * 32:(fb + 1) * 32, :]), wb[:, 2 * D + g * 128:2 * D + (g + 1) * 128])
            st[fb] = jnp.where(bd()[(fb % 2) * 64:(fb % 2) * 64 + 64], r, 0.0).astype(BF16)

        def mm(fb):
            g = fb // 2
            m = _pk(_nn(st[fb], wob[g * 128:(g + 1) * 128, :]))
            for c in range(4):
                mp[c, fb * 32:(fb + 1) * 32, :] = m[:, c * 128:(c + 1) * 128]

        def zz():
            for g in range(4):
                za = zacc[g * 128:(g + 1) * 128, :]
                z = jnp.sum(za, axis=1, keepdims=True)
                zb[g] = jnp.where(bd(), jnp.broadcast_to(z, (128, 128)), 0.0)
                zpk[g * 64:(g + 1) * 64, :] = _pk(za)
            zrow[...] = _nt(jnp.ones((16, 128), BF16), _bf(perm_rows(zpk)))[0:8]
        return ([(functools.partial(kv, fb), 64, 40) for fb in range(8)],
                [(functools.partial(mm, fb), 64, 16) for fb in range(8)], [(zz, 64, 120)])

    def q_pieces(rb0, rb1):
        def piece(rb, g):
            w = wb[:, g * 128:(g + 1) * 128] if rb < QOLD else _bf(wqp[:, g * 128:(g + 1) * 128])
            pq[rb * 64:(rb + 1) * 64, g * 128:(g + 1) * 128] = _phi(_nn(tile("x", rb * 64, 64), w))
        return [(functools.partial(piece, rb, g), 64, 64) for rb in range(rb0, rb1) for g in range(4)]

    def o_stream(rb0, rb1, q0):
        st = {}

        def den_mxu(rb):
            rows = slice(rb * 64, (rb + 1) * 64)
            for g in range(4):
                cols = slice(g * 128, (g + 1) * 128)
                d = _nn(pq[rows, cols], zb[g]) + 1e-6
                pp[rb * 32:(rb + 1) * 32, cols] = _pk(pq[rows, cols] * pl.reciprocal(d, approx=True))

        def den_vpu(rb):
            _, lane = iotas()
            for v in range(rb * 4, rb * 4 + 4):
                rs = []
                for r0 in (v * 16, v * 16 + 8):
                    t = None
                    for g in range(4):
                        cols = slice(g * 128, (g + 1) * 128)
                        p = pq[r0:r0 + 8, cols] * zrow[:, cols]
                        t = p if t is None else t + p
                    t = t + jnp.take_along_axis(t, lane ^ 2, axis=1)
                    t = t + jnp.take_along_axis(t, lane ^ 1, axis=1)
                    rs.append(pl.reciprocal(t + 1e-6, approx=True))
                r = jnp.concatenate(rs, axis=0)
                for g in range(4):
                    cols = slice(g * 128, (g + 1) * 128)
                    pp[v * 8:v * 8 + 8, cols] = _pk(pq[v * 16:v * 16 + 16, cols] * r)

        def out(rb, g):
            m = mp[g, 0:D // 2, :] if rb < QOLD else perm_rows(mp.at[g])
            r = _nn(_bf(pp[rb * 32:(rb + 1) * 32, :]), _bf(m))
            if g % 2 == 0:
                st["r"] = r
            else:
                sta[rb * 64:(rb + 1) * 64, (g - 1) * 128:(g + 1) * 128] = jnp.concatenate(
                    [st["r"], r], axis=1).astype(BF16)

        res = []
        for t in range(rb0 - 2, rb1):
            step = []
            ov = 60 if t + 1 >= q0 else 28
            if q0 <= t + 2 < rb1:
                step += q_pieces(t + 2, t + 3)
            if rb0 <= t:
                step += [(functools.partial(out, t, g), 64, ov) for g in (0, 1)]
            if rb0 <= t + 1 < rb1:
                step.append((functools.partial(den_mxu, t + 1), 64, 80) if t + 1 < QOLD
                            else (functools.partial(den_vpu, t + 1), 0, 128))
            if rb0 <= t:
                step += [(functools.partial(out, t, g), 64, ov) for g in (2, 3)]
            res.append(step)

        def seg(a, b):
            return [p for step in res[a - rb0 + 2:b - rb0 + 2] for p in step]
        return seg

    prm_hbm = (are_hbm, aim_hbm, bre_hbm, bim_hbm, cre_hbm, cim_hbm)

    def prm_rest(i):
        return prm_hbm[i].at[R0:D], prm.at[i, R0:D]

    srcs = {"ldt": (ldt_hbm, ldt)}
    srcs.update({"a%d" % i: (prm_hbm[i].at[0:R0], prm.at[i, 0:R0]) for i in range(6)})
    srcs.update({
        "wq": (w_hbm.at[:, 0:D], wb.at[:, 0:D]),
        "x0": (x_hbm.at[0:X0], xb.at[0:X0]),
        "dsk": (dsk_hbm, dsk),
        "p0": prm_rest(0),
        "p1": prm_rest(1),
        "wk": (w_hbm.at[:, D:2 * D], wb.at[:, D:2 * D]),
        "p2": prm_rest(2),
        "p3": prm_rest(3),
        "p4": prm_rest(4),
        "p5": prm_rest(5),
        "x1": (x_hbm.at[X0:X1], xb.at[X0:X1]),
        "fi": (fi_hbm, fi),
        "fk": (fk_hbm, fk),
        "ua": (u_hbm.at[:, 0:256], ub.at[:, 0:256]),
        "x2": (x_hbm.at[X1:S], xb.at[X1:S]),
        "ub": (u_hbm.at[:, 256:D], ub.at[:, 256:D]),
        "wv": (w_hbm.at[:, 2 * D:3 * D], wb.at[:, 2 * D:3 * D]),
        "wo": (wo_hbm, wob),
    })
    cin = {k: pltpu.make_async_copy(a, b, sem_in.at[i]) for i, (k, (a, b)) in enumerate(srcs.items())}
    for c in cin.values():
        c.start()
    couts = []

    def wait(*names):
        for n in names:
            cin[n].wait()

    def out_copy(i, kind, a, b):
        if kind == "a":
            return pltpu.make_async_copy(sta.at[a * 64:b * 64], o_hbm.at[a * 64:b * 64, 0:D], sem_out.at[i])
        c0 = D + kind * 128
        return pltpu.make_async_copy(stb.at[kind, a * 128:b * 128],
                                     o_hbm.at[a * 128:b * 128, c0:c0 + 128], sem_out.at[i])

    def store(*box):
        out_copy(len(couts), *box).start()
        couts.append(box)

    q0, q1 = X0 // 64, X1 // 64
    p0, p1 = X0 // 128, X1 // 128
    qe = q_pieces(q1, q1 + 3)
    mid1, mid2, midz = mid_pieces()
    gps = g_pieces()
    gs = []
    for fb in range(8):
        blk = gps[fb * 16:(fb + 1) * 16]
        if fb:
            blk = blk[:4] + [mid1[fb - 1]] + blk[4:9] + [mid2[fb - 1]] + blk[9:]
        gs += blk
    kds = [kdft_pieces(j, 20 if j >= 2 else 0) for j in range(4)]
    uds = [udft_pieces(j) for j in range(4)]
    cv = [[(p, 0, 4) for p in range(32)],
          [(p, 0, 4) for p in range(32, 48)],
          [(p, 0, 3) for p in range(48, 64)] + [(p, 3, 4) for p in range(48, C3)],
          [(p, 3, 4) for p in range(C3, 64)]]
    oseg = o_stream(0, O3, q1 + 3)
    oseg2 = o_stream(O3, 32, O3)

    main3 = uds[0][:8] + [(k0_all, 8, 0)] + uds[0][8:] + kds[0] + uds[1][:10] + kds[1] + uds[1][10:]
    blk3 = main3[:3] + _merge(main3[3:-4], kgen_pieces(G0, 64)) + main3[-4:]
    ql = q_pieces(q0 - 1, q0)
    blk4 = (uds[2][:2] + _merge(kt_pieces(p1, 16), uds[2][2:13]) + uds[2][13:]
            + _merge(gs[:GS], midz + kds[2] + kds[3], uds[3]))
    blk5 = _merge(gs[GS:] + qe[:4] + [mid1[7]] + oseg(-2, 0) + qe[4:8] + [mid2[7]] + qe[8:] + oseg(0, O1),
                  inv_pieces(0) + inv_pieces(1))
    blk5 = [(f, c, v + (50 if 8 <= i < 32 else 0)) for i, (f, c, v) in enumerate(blk5)]
    last = oseg2(O4, 32)
    ta = oseg2(O3, O4)
    blk8 = oseg2(O3 - 2, O3) + ta[:-5] + inv_pieces(3)[6:] + [p for p in last if p[1] == 0] + ta[-5:]
    blk9 = [p for p in last if p[1] != 0]

    steps = [
        (lambda: wait("ldt"), setup_dt_first),
        (lambda: wait("a0", "a1", "a2", "a3", "a4", "a5"), early_prep),
        (early_exact, lambda: _emit(kgen_pieces(0, G0))),
        (lambda: wait("wq", "x0", "dsk"),
         lambda: (setup_dt_rest(), wq_perm_a(), _emit(q_pieces(0, q0 - 1)))),
        (lambda: wait("p0", "p1", "wk"),
         lambda: (wk_transpose(), range_check(0, R0, D),
                  _emit(ql[:3] + kt_pieces(0, p0, True), stage1(), (32 - G0 // 2) * 90))),
        (lambda: (stage1_exact(), wait("p2", "p3", "p4", "p5", "x1")),
         lambda: (wq_perm_b(),
                  _emit(ql[3:] + kt_pieces(p0, p1) + q_pieces(q0, q1), stage2_fill(G0 // 2, 32), (32 - G0 // 2) * 164))),
        (lambda: wait("fi", "fk", "ua"), lambda: (setup_g(), _emit(blk3))),
        (lambda: wait("x2", "ub", "wv", "wo"), lambda: _emit(blk4, conv(cv[0]), conv_ops(cv[0]))),
        (None, lambda: _emit(blk5, conv(cv[1]), conv_ops(cv[1]))),
        (lambda: (store(0, 0, 16), store(1, 0, 16), store("a", 0, O1)),
         lambda: _emit(_merge(oseg(O1, O2), inv_pieces(2)), conv(cv[2]), conv_ops(cv[2]))),
        (lambda: (store(2, 0, 16), store("a", O1, O2)),
         lambda: _emit(_merge(oseg(O2, O3), inv_pieces(3)[:6]), conv(cv[3]), conv_ops(cv[3]))),
        (lambda: (store(3, 0, 12), store("a", O2, O3)), lambda: _emit(blk8)),
        (lambda: (store(3, 12, 16), store("a", O3, O4)), lambda: _emit(blk9)),
        (lambda: store("a", O4, 32), None),
    ]

    def outer(i, c):
        packed.clear()
        couts.clear()
        for k in range(len(steps) - 1):
            @pl.when(i + k == k)
            def _():
                steps[k][1]()
                if steps[k + 1][0] is not None:
                    steps[k + 1][0]()
        return c

    steps[0][0]()
    lax.fori_loop(0, 2, outer, 0)
    for i, box in enumerate(couts):
        out_copy(i, *box).wait()


@jax.jit
def pallas_concat_heads__linear_attn_block__ssm_conv_s4__prompt_kernel(
    A_x, A_wqkv, A_wo, B_u, B_A_re, B_A_im, B_B_re, B_B_im, B_C_re, B_C_im, B_log_dt, B_Dskip,
):
    fk, fi = _tables()
    V = pltpu.VMEM
    out = pl.pallas_call(
        _kernel,
        out_shape=jax.ShapeDtypeStruct((S, 2 * D), BF16),
        in_specs=[pl.BlockSpec(memory_space=pl.ANY)] * 14,
        out_specs=pl.BlockSpec(memory_space=pl.ANY),
        scratch_shapes=[
            V((S // 2, D), U32),
            V((D, 3 * D), BF16),
            V((D, D), BF16),
            V((S // 2, D), U32),
            V((6, D, 128), BF16),
            V((D,), BF16),
            V((D,), BF16),
            V((S, D), BF16),
            V((S, D), BF16),
            V((FK_ROWS // 2, 128), U32),
            V((136, 128), F32),
            V((S, D), BF16),
            V((4, S, 128), BF16),
            V((2, D, 128), F32),
            pltpu.SMEM((2,), jnp.int32),
            V((D, 128), F32),
            V((8, 128, 128), F32),
            V((14, 2 * D + 8, 128), F32),
            V((D, 128), F32),
            V((5, D // 2, 128), U32),
            V((4, 2, 16, 128), F32),
            V((8, D), F32),
            V((4, 3, 16, 128, 128), F32),
            V((4, 3, 16, 128, 128), F32),
            V((4, 2, 16, 128, 128), F32),
            V((D // 2, D), U32),
            V((D // 2, S), U32),
            V((D, 128), F32),
            V((D // 2, D), U32),
            V((4, D // 2 + 8, 128), U32),
            V((4, 128, 128), F32),
            V((S, D), F32),
            V((S // 2, D), U32),
            V((4, D // 2 + 8, 128), U32),
            V((D // 2, D), U32),
            V((D // 2 + 8, 128), U32),
            V((8, D), F32),
            V((4, 12, 144, 128), F32),
            V((2, 128, 128), F32),
            pltpu.SemaphoreType.DMA((25,)),
            pltpu.SemaphoreType.DMA((10,)),
        ],
        compiler_params=pltpu.CompilerParams(vmem_limit_bytes=110 * 2**20, disable_semaphore_checks=True),
    )(A_x.reshape(S, D), A_wqkv, A_wo, B_u.reshape(S, D), B_A_re, B_A_im, B_B_re, B_B_im, B_C_re, B_C_im,
      B_log_dt, B_Dskip, jnp.asarray(fk), jnp.asarray(fi))
    return out.reshape(1, S, 2 * D)
```

```python
import functools

import numpy as np
import jax
import jax.numpy as jnp
from jax import lax
import jax.experimental.pallas as pl
import jax.experimental.pallas.tpu as pltpu

S = 2048
D = 512
F32 = jnp.float32
BF16 = jnp.bfloat16
U32 = jnp.uint32

_BASE = np.array([[1, 5], [2, 6], [3, 7], [4, 8], [258, 262], [260, 264],
                  [516, 520], [772, 776], [1032, 1288], [1544, 1800]])
_TILE_OF_CHUNK = [0, 1, 2, 2, 3, 3, 3, 3] + [4] * 8

FK_OFF = [0, 256, 528, 784] + [1056 + 144 * k for k in range(4)] + [1632 + 80 * k for k in range(8)]
FK_FU = 1632 + 640
FK_ROWS = FK_FU + 256

X0, X1 = 384, 896
QOLD = X0 // 64
G0 = 12
R0 = 8 * G0
O1, O2, O3, O4 = 15, 24, 29, 31
GS = 120
C3 = 51

B_W1, B_W2, B_W8C, B_W256, B_W512, B_E0, B_N0 = range(7)
_SC_LIMIT = 8192.0


def _bf16_bits(v):
    u = np.ascontiguousarray(v, np.float32).view(np.uint32)
    return ((u + 0x7FFF + ((u >> 16) & 1)) >> 16).astype(np.uint32)


def _pack_rows(v):
    b = _bf16_bits(v)
    return b[0::2] | (b[1::2] << 16)


@functools.lru_cache(maxsize=None)
def _tables():
    lr = (_bf16_bits(np.arange(S)) << 16).view(np.float32).astype(np.int64)
    val = np.zeros((5, 128), np.int64)
    for lam in range(128):
        mu, tau = 15 - (lam >> 3), lam & 7
        e, x = tau >> 1, tau & 1
        for h in range(2):
            val[h, lam] = _BASE[e, x ^ h] + 8 * (mu + 16 * h)
        hp, ab, h = tau >> 2, (tau >> 1) & 1, tau & 1
        for q in range(3):
            val[2 + q, lam] = _BASE[4 + 2 * q + ab, hp] + 8 * (mu + 16 * h)
    om = 2 * np.pi * (np.arange(128) + 0.25) / 128.0
    phase = np.exp(1j * om * 191.5)

    def stack(z):
        return np.concatenate([p[32 * t:32 * t + 32] for t in range(4) for p in (z.real, z.imag)], axis=0)

    fk = []
    g = np.zeros(128, np.complex128)
    for k in range(4):
        slot = {int(v): i for i, v in enumerate(val[_TILE_OF_CHUNK[k]])}
        m = np.zeros((128, 128), np.complex128)
        for p in range(1, 129):
            lag = 128 * k + p
            v = int(lr[lag])
            z = np.exp(-1j * om * p) * (0.5 if lag == 512 else 1.0)
            if v in slot:
                m[:, slot[v]] += z
            else:
                assert v == 256 and k == 2
                g += z
        if k in (1, 3):
            sel = np.zeros((16, 128))
            sel[:, slot[128 * (k + 1)]] = 1.0
            fk += [stack(m)[:128], sel, stack(m)[128:]]
        else:
            fk.append(stack(m))
    for k in range(4, 16):
        st = 4 if k < 8 else 8
        per = 128 // st
        slot = {int(v): i for i, v in enumerate(val[_TILE_OF_CHUNK[k]])}
        for lag in range(128 * k + 1, min(128 * k + 128, S)):
            m_ = int(lr[lag]) // st
            assert int(lr[lag]) % st == 0 and abs(lag - st * m_) <= (st // 2 if m_ % 2 == 0 else st // 2 - 1)
        od = np.zeros((per, 128), np.complex128)
        ev = np.zeros((per, 128), np.complex128)
        edge = np.zeros((16, 128))
        for m_ in range(per + 1):
            v = 128 * k + st * m_
            if v not in slot:
                assert m_ == 0 and k in (4, 8)
                continue
            z = np.exp(-1j * om[:per] * st * m_)
            if m_ % 2:
                od[:, slot[v]] = z
            else:
                ev[:, slot[v]] = z * (0.5 if m_ in (0, per) else 1.0)
            if m_ in (0, per):
                edge[8 * (m_ // per):8 * (m_ // per) + 8, slot[v]] = 1.0
        fk += [edge, od.real, od.imag, ev.real, ev.imag]
    fk.append(stack(np.exp(-1j * om[:, None] * np.arange(128)[None, :]) * phase[:, None]))
    fk = np.concatenate(fk, axis=0)
    assert fk.shape[0] == FK_ROWS
    tabs = [g.real, g.imag]
    for h in (2, 4):
        tabs += [sum(np.cos(om * p) for p in range(1 - h, h)), sum(np.cos(om * p) for p in range(-h, h + 1)),
                 -sum(np.sin(om * p) for p in range(1, h + 1))]
    jj = np.arange(64)[:, None] - 63.5
    finv = np.concatenate([np.cos(om[None, :] * jj) / 128.0, -np.sin(om[None, :] * jj) / 128.0,
                           np.stack(tabs)], axis=0)
    return _pack_rows(fk), finv.astype(np.float32)


def _cmul(a, b):
    return a[0] * b[0] - a[1] * b[1], a[0] * b[1] + a[1] * b[0]


def _csq(a):
    return a[0] * a[0] - a[1] * a[1], (a[0] + a[0]) * a[1]


def _phi(t):
    return jnp.where(t > 0, t + 1.0, jnp.exp(t)) + 1e-6


def _nt(a, b):
    return lax.dot_general(a, b, (((1,), (1,)), ((), ())), preferred_element_type=F32)


def _nn(a, b):
    return jnp.dot(a, b, preferred_element_type=F32)


def _bf(v):
    return pltpu.bitcast(v, BF16)


def _pk(v):
    return pltpu.bitcast(v.astype(BF16), U32)


def _sincos(x):
    t = x * 0.6366197723675814 + 12582912.0
    n = pltpu.bitcast(t, jnp.int32) - 0x4B400000
    k = n.astype(F32)
    r = ((x - k * 1.5703125) - k * 4.837512969970703125e-4) - k * 7.54978995489188216e-8
    r2 = r * r
    sn = r + r * r2 * (-1.6666654611e-1 + r2 * (8.3321608736e-3 + r2 * -1.9515295891e-4))
    cs = 1.0 + r2 * (-0.5 + r2 * (4.166664568298827e-2 + r2 * (-1.388731625493765e-3 + r2 * 2.443315711809948e-5)))
    swap = (n & 1) == 1
    s_, c_ = jnp.where(swap, cs, sn), jnp.where(swap, sn, cs)
    ssign = (n & 2) << 30
    csign = ((n + 1) & 2) << 30
    s_ = pltpu.bitcast(pltpu.bitcast(s_, jnp.int32) ^ ssign, F32)
    c_ = pltpu.bitcast(pltpu.bitcast(c_, jnp.int32) ^ csign, F32)
    return s_, c_


def _emit(pieces, filler=None, fill_total=0, cap=3.0, tail=100):
    filler = iter(()) if filler is None else filler
    room = [max(cap * c - v, 0.0) for _, c, v in pieces]
    tot = sum(room[:-1]) or 1.0
    done, target = 0.0, 0.0
    for (fn, _, _), r in zip(pieces, room):
        fn()
        target += max(fill_total - tail, 0) * r / tot
        while done < target - 8:
            n = next(filler, None)
            if n is None:
                break
            done += n
    for _ in filler:
        pass


def _merge(*lists):
    tot = [sum(p[1] for p in l) or 1.0 for l in lists]
    pos = [0] * len(lists)
    acc = [0.0] * len(lists)
    out = []
    while True:
        best = None
        for i, l in enumerate(lists):
            if pos[i] < len(l):
                key = (acc[i] + 0.5 * l[pos[i]][1]) / tot[i]
                if best is None or key < best[0]:
                    best = (key, i)
        if best is None:
            return out
        i = best[1]
        out.append(lists[i][pos[i]])
        acc[i] += lists[i][pos[i]][1]
        pos[i] += 1


def _group(pieces, n):
    out = []
    for i in range(0, len(pieces), n):
        grp = pieces[i:i + n]

        def run(grp=grp):
            for f, _, _ in grp:
                f()
        out.append((run, sum(p[1] for p in grp), sum(p[2] for p in grp)))
    return out


def _reim(r):
    n = r.shape[0] // 64
    return (jnp.concatenate([r[64 * t:64 * t + 32] for t in range(n)], axis=0),
            jnp.concatenate([r[64 * t + 32:64 * t + 64] for t in range(n)], axis=0))


def _kernel(x_hbm, w_hbm, wo_hbm, u_hbm, are_hbm, aim_hbm, bre_hbm, bim_hbm, cre_hbm, cim_hbm,
            ldt_hbm, dsk_hbm, fk_hbm, fi_hbm, o_hbm,
            xp, wb, wob, up, prm, ldt, dsk, xb, ub, fk, fi, sta, stb, w1s, flag,
            dtb, gb, base, cr, wt, bv, k0s, kw, u3, y, wkt, pkt, zacc, gp, mp, zb, pq, pp,
            wqt, wqp, zpk, zrow, kf, zc, sem_in, sem_out):

    def iotas():
        return (lax.broadcasted_iota(jnp.int32, (8, 128), 0), lax.broadcasted_iota(jnp.int32, (8, 128), 1))

    packed = set()

    def tile(kind, r0, n, cols=slice(None)):
        src, dst = (xb, xp) if kind == "x" else (ub, up)
        parts = []
        for r in range(r0, r0 + n, 64):
            key = (kind, r, cols.start)
            if key in packed:
                parts.append(_bf(dst[r // 2:r // 2 + 32, cols]))
            else:
                packed.add(key)
                v = src[r:r + 64, cols]
                dst[r // 2:r // 2 + 32, cols] = pltpu.bitcast(v, U32)
                parts.append(v)
        return parts[0] if len(parts) == 1 else jnp.concatenate(parts, axis=0)

    def dt_row():
        return jnp.exp(ldt[...].reshape(1, D).astype(F32)).astype(BF16).astype(F32)

    def setup_dt_first():
        sub, _ = iotas()
        b = jnp.broadcast_to(dt_row()[:, 0:128], (8, 128))
        for v in range(16):
            dtb[v * 8:v * 8 + 8, :] = jnp.take_along_axis(b, sub + 8 * v, axis=1)

    def setup_dt_rest():
        row = dt_row()
        for j in range(1, 4):
            dtb[j * 128:(j + 1) * 128, :] = jnp.broadcast_to(row[:, j * 128:(j + 1) * 128], (128, 128)).T

    def setup_g():
        for i in range(8):
            gb[i] = jnp.broadcast_to(fi[128 + i:129 + i, :], (128, 128)).T

    def perm_rows(ref):
        return jnp.concatenate([ref[pl.ds(t, 64, stride=4), :] for t in range(4)], axis=0)

    def wq_perm_a():
        for a in range(4):
            for b in range(4):
                t = wb[a * 128:(a + 1) * 128, b * 128:(b + 1) * 128].T
                wqt[a, b * 64:(b + 1) * 64, :] = pltpu.bitcast(t, U32)

    def wq_perm_b():
        for b in range(4):
            for a in range(4):
                t = _bf(wqt[a, pl.ds(b, 64, stride=4), :]).T
                wqp[a * 64:(a + 1) * 64, b * 128:(b + 1) * 128] = pltpu.bitcast(t, U32)

    def wk_transpose():
        for b in range(4):
            for a in range(4):
                t = wb[a * 128:(a + 1) * 128, D + b * 128:D + (b + 1) * 128].T
                wkt[b * 64:(b + 1) * 64, a * 128:(a + 1) * 128] = pltpu.bitcast(t, U32)

    def w1_rows(r0, exact):
        rows = pl.ds(r0, 16)
        dt = dtb[rows, :]
        ar = dt * prm[0, rows, :].astype(F32)
        ai = dt * prm[1, rows, :].astype(F32)
        mag = jnp.exp(ar)
        sn, cs = (jnp.sin(ai), jnp.cos(ai)) if exact else _sincos(ai)
        w1s[0, rows, :] = mag * cs
        w1s[1, rows, :] = mag * sn

    def range_check(i, r0, r1):
        m = jnp.max(jnp.abs(prm[1, r0:r1, :].astype(F32)).reshape((r1 - r0) // 8, 8, 128), axis=0)
        dmax = jnp.max(dtb[r0:r1, :].reshape((r1 - r0) // 8, 8, 128), axis=0)
        bound = jnp.max(m) * jnp.max(dmax)
        flag[i] = jnp.where(bound <= _SC_LIMIT, 0, 1).astype(jnp.int32)

    def stage1():
        for r in range(G0 // 2, 32):
            w1_rows(r * 16, False)
            yield 90

    def stage1_exact():
        @pl.when(flag[0] != 0)
        def _():
            def body(r, c):
                w1_rows(pl.multiple_of(r * 16, 16), True)
                return c
            lax.fori_loop(G0 // 2, 32, body, 0)

    def stage2(r):
        r0 = r * 16 if isinstance(r, int) else pl.multiple_of(r * 16, 16)
        rows = pl.ds(r0, 16)
        dt = dtb[rows, :]
        w1 = (w1s[0, rows, :], w1s[1, rows, :])
        db = (dt * prm[2, rows, :].astype(F32), dt * prm[3, rows, :].astype(F32))
        c = _cmul((prm[4, rows, :].astype(F32), prm[5, rows, :].astype(F32)), db)
        cr[rows, :] = c[0]
        lo = (lax.broadcasted_iota(jnp.int32, (16, 128), 0) & 4) == 0

        def put(i, v0, v1=None):
            for t in range(2):
                ev, od = (v0[t], v0[t]) if v1 is None else (jnp.where(lo, v0[t], v1[t]), jnp.where(lo, v1[t], v0[t]))
                base[2 * i + t, pl.ds(2 * r0, 16, stride=2), :] = ev
                base[2 * i + t, pl.ds(2 * r0 + 1, 16, stride=2), :] = od
        put(B_W1, w1)
        w2 = _csq(w1)
        put(B_W2, w2)
        w4 = _csq(w2)
        cw1 = _cmul(c, w1)
        put(B_N0, cw1, _cmul(cw1, w4))
        yield 80
        w8 = _csq(w4)
        put(B_W8C, (w8[0], -w8[1]))
        w128 = _csq(_csq(_csq(_csq(w8))))
        put(B_E0, (jnp.ones((16, 128), F32), jnp.zeros((16, 128), F32)), (w128[0], -w128[1]))
        w256 = _csq(w128)
        put(B_W256, w256)
        put(B_W512, _csq(w256))
        yield 84

    def stage2_fill(r0, r1):
        for r in range(r0, r1):
            yield from stage2(r)

    def early_prep():
        range_check(1, 0, R0)
        for r in range(G0 // 2):
            w1_rows(r * 16, False)
        for _ in stage2_fill(0, G0 // 2):
            pass

    def early_exact():
        @pl.when(flag[1] != 0)
        def _():
            def body(r, c):
                w1_rows(pl.multiple_of(r * 16, 16), True)
                for _ in stage2(r):
                    pass
                return c
            lax.fori_loop(0, G0 // 2, body, 0)

    def kgen_pieces(g0, g1):
        st = {}

        def group(gi):
            sub, lane = iotas()
            odd = (sub & 1) == 1
            rows = slice(gi * 16, gi * 16 + 16)

            def ld(i):
                return base[2 * i, rows, :], base[2 * i + 1, rows, :]
            w8c = ld(B_W8C)
            e0 = [ld(B_E0)]
            for _ in range(1, 16):
                e0.append(_cmul(e0[-1], w8c))
            e0 = e0[::-1]
            w1, w2, w256, w512 = ld(B_W1), ld(B_W2), ld(B_W256), ld(B_W512)
            n0 = ld(B_N0)
            n1 = _cmul(n0, w1)
            n2 = _cmul(n0, w2)
            n3 = _cmul(n1, w2)
            n4 = _cmul(n1, w256)
            n5 = _cmul(n3, w256)
            n6 = _cmul(n5, w256)
            n7 = _cmul(n6, w256)
            t = tuple(jnp.concatenate([jnp.where(odd, n7[c][0:8], pltpu.roll(n6[c][0:8], 7, 0)),
                                       jnp.where(odd, pltpu.roll(n6[c][8:16], 1, 0), n7[c][8:16])], axis=0)
                      for c in range(2))
            n8 = _cmul(t, w512)
            n9 = _cmul(n8, w512)
            e1 = [n0, n1, n2, n3, n4, n5, n6, n7, n8, n9]

            def operands(es):
                v = jnp.concatenate([jnp.concatenate([e[0] for e in es], axis=0),
                                     jnp.concatenate([e[1] for e in es], axis=0)], axis=1)
                v = v.reshape(len(es), 2, 8, 256)
                return [v[:, g].reshape(len(es) * 8, 256) for g in range(2)]
            o = []
            for lhs, rhs in zip(operands(e1), operands(e0)):
                r = _nt(lhs, rhs)
                o.append([r[8 * i:8 * i + 8, :] for i in range(10)])

            emask = ((sub >> 1) - (lane >> 1)) & 3
            ea, xa = (lane >> 1) & 3, lane & 1
            lidx_a = (lane & 120) | ((((sub >> 1) - ea) & 3) << 1) | (xa ^ (sub & 1))
            sidx_a = ((((sub & 3) + ea) & 3) << 1) | (xa ^ (sub >> 2))
            hp, ab, hh = (lane >> 2) & 1, (lane >> 1) & 1, lane & 1
            gg = hp ^ (sub & 1)
            lidx_b = (lane & 120) | ((((sub >> 1) - (2 * gg + ab)) & 3) << 1) | (hh ^ gg)
            g2 = sub >> 2
            sidx_b = ((((sub & 3) + 2 * g2 + ab) & 3) << 1) | (hp ^ g2)

            def compact(srcs, lidx, sidx):
                s = srcs[0]
                for e in range(1, 4):
                    s = jnp.where(emask == e, pltpu.roll(srcs[e], 2 * e, 0), s)
                s = jnp.take_along_axis(s, lidx, axis=1)
                return jnp.take_along_axis(s, sidx, axis=0)

            a2 = [compact(o[g][0:4], lidx_a, sidx_a) for g in range(2)]
            lo = sub < 4
            res = [jnp.where(lo, a2[0], a2[1]), pltpu.roll(jnp.where(lo, a2[1], a2[0]), 4, 0)]
            for q in range(3):
                res.append(compact(o[0][4 + 2 * q:6 + 2 * q] + o[1][4 + 2 * q:6 + 2 * q], lidx_b, sidx_b))
            if gi % 2 == 0:
                st["r"] = res
            else:
                for q in range(5):
                    wt[q, (gi // 2) * 8:(gi // 2) * 8 + 8, :] = _pk(jnp.concatenate([st["r"][q], res[q]], axis=0))

        return [(functools.partial(group, gi), 80, 360) for gi in range(g0, g1)]

    def k0_all():
        k0s[...] = _nt(jnp.ones((8, 128), F32), cr[...]) + dsk[...].reshape(1, D).astype(F32)

    def kdft_pieces(j, extra):
        def wtile(k):
            return _bf(wt[_TILE_OF_CHUNK[k], j * 64:(j + 1) * 64, :])

        def near(k, hf):
            o = FK_OFF[k] // 2 + hf * 64
            if k in (1, 3):
                r = _nt(_bf(fk[o:o + 72, :]), wtile(k))
                bv[j, k // 2, hf * 8:hf * 8 + 8, :] = r[128:136] if hf == 0 else r[0:8]
                r = r[:128] if hf == 0 else r[16:]
            else:
                r = _nt(_bf(fk[o:o + 64, :]), wtile(k))
            rr, ri = _reim(r)
            rows = slice(hf * 64, hf * 64 + 64)
            if k == 0:
                rr = rr + jnp.concatenate([k0s[:, j * 128:(j + 1) * 128]] * 8, axis=0)
            elif k == 2:
                bval = jnp.concatenate([bv[j, 0]] * 4, axis=0)
                rr = rr + gb[0, rows, :] * bval
                ri = ri + gb[1, rows, :] * bval
            kw[j, 0, k, rows, :] = rr
            kw[j, 1, k, rows, :] = ri
            kw[j, 2, k, rows, :] = rr + ri

        def far(k):
            per = 32 if k < 8 else 16
            n = 16 + 4 * per
            o = FK_OFF[k] // 2
            r = _nt(_bf(fk[o:o + n // 2, :]), wtile(k))
            if k in (4, 8):
                e0 = 16 + 2 * per
                v0 = bv[j, 1] if k == 4 else jnp.concatenate([kf[j, 3, 8:16, :]] * 2, axis=0)
                r = jnp.concatenate([v0[0:8], r[8:e0], r[e0:e0 + per] + 0.5 * jnp.concatenate([v0] * (per // 16), axis=0),
                                     r[e0 + per:]], axis=0)
            kf[j, k - 4, 0:n, :] = r

        def nears(ks, v):
            return _group([(functools.partial(near, k, hf), 32, v + extra) for k in ks for hf in range(2)], 4)

        def fars(ks):
            return _group([(functools.partial(far, k), 36 if k < 8 else 20, extra) for k in ks], 4)
        return (nears((1, 3), 8) + fars((12, 13, 14, 15)) + fars((7, 6, 5, 4))
                + nears((0, 2), 28) + fars((9, 10, 11, 8)))

    def udft_pieces(j):
        def piece(ib, qf):
            o = FK_FU // 2 + qf * 32
            w = jnp.concatenate([tile("u", i * 128, 128, slice(j * 128, (j + 1) * 128))
                                 for i in range(ib * 4, ib * 4 + 4)], axis=1)
            r = _nn(_bf(fk[o:o + 32, :]), w)
            rows = slice(qf * 32, qf * 32 + 32)
            for t in range(4):
                rr, ri = r[:32, t * 128:(t + 1) * 128], r[32:, t * 128:(t + 1) * 128]
                u3[j, 0, ib * 4 + t, rows, :] = rr
                u3[j, 1, ib * 4 + t, rows, :] = ri
                u3[j, 2, ib * 4 + t, rows, :] = rr + ri
        return [(functools.partial(piece, ib, qf), 64, 16) for ib in range(4) for qf in range(4)]

    def conv_ops(items):
        return sum((68, 204, 300, 396)[ib] for _, i0, i1 in items for ib in range(i0, i1))

    def conv(items):
        for pos, ib0, ib1 in items:
            j, p = divmod(pos, 16)
            rs = slice(p * 8, p * 8 + 8)
            prev = None if ib0 == 0 else (zc[0:1, rs, :], zc[1:2, rs, :])
            for ib in range(ib0, ib1):
                if ib > 0:
                    t0 = 2 if ib == 1 else 5
                    d_od, d_ev, sh = (gb[t0 + t:t0 + t + 1, rs, :] for t in range(3))
                    per = 32 if ib == 1 else 16
                    h = 16 + (8 * p) % per
                    left = sh * kf[j, 4 * ib - 4:4 * ib - 3, 0:8, :]
                    for k in range(4 * ib, 4 * ib + 4, 2):
                        o_r, o_i, e_r, e_i = (kf[j, k - 4:k - 2, per * t + h:per * t + h + 8, :] for t in range(4))
                        right = sh * kf[j, k - 4:k - 2, 8:16, :]
                        rr = d_od * o_r + d_ev * e_r - right
                        ri = d_od * o_i + d_ev * e_i + jnp.concatenate([left, right[:1]], axis=0)
                        left = right[1:]
                        kw[j, 0, k:k + 2, rs, :] = rr
                        kw[j, 1, k:k + 2, rs, :] = ri
                        kw[j, 2, k:k + 2, rs, :] = rr + ri
                        yield 20
                a = zr = None
                for c in range(3):
                    acc = None
                    for k in range(4 * ib + 1):
                        pr = u3[j, c, 4 * ib - k:4 * ib - k + 4, rs, :] * kw[j, c, k:k + 1, rs, :]
                        if acc is None:
                            acc = pr - a if c == 2 else pr
                        else:
                            acc = acc + pr
                        if k % 4 == 3:
                            yield 32
                    for d in range(1, 4):
                        pr = u3[j, c, 0:4 - d, rs, :] * kw[j, c, 4 * ib + d:4 * ib + d + 1, rs, :]
                        acc = jnp.concatenate([acc[:d], acc[d:] + pr], axis=0)
                    n = 20
                    if c == 0:
                        a = acc
                    elif c == 1:
                        zr = a - acc
                        a = a + acc
                    else:
                        if prev is None:
                            yr = jnp.concatenate([acc[:1], zr[:3] + acc[1:]], axis=0)
                            yi = jnp.concatenate([-zr[:1], acc[:3] - zr[1:]], axis=0)
                        else:
                            yr = jnp.concatenate([prev[0], zr[:3]], axis=0) + acc
                            yi = jnp.concatenate([prev[1], acc[:3]], axis=0) - zr
                        y[j, 0, ib * 4:ib * 4 + 4, rs, :] = yr
                        y[j, 1, ib * 4:ib * 4 + 4, rs, :] = yi
                        prev = (zr[3:], acc[3:])
                        n += 8
                        if ib == ib1 - 1 and ib1 < 4:
                            zc[0:1, rs, :], zc[1:2, rs, :] = prev
                    yield n

    def inv_pieces(j):
        def piece(i):
            sub, _ = iotas()
            s = _nn(fi[0:64, :], y[j, 0, i])
            a = _nn(fi[64:128, :], y[j, 1, i])
            lo = s + a
            hi = s - a
            hi = jnp.concatenate(
                [jnp.take_along_axis(hi[8 * v:8 * v + 8], 7 - sub, axis=0) for v in range(7, -1, -1)], axis=0)
            stb[j, i * 128:(i + 1) * 128, :] = jnp.concatenate([lo, hi], axis=0).astype(BF16)
        return _group([(functools.partial(piece, i), 32, 32) for i in range(16)], 2)

    def kt_pieces(pb0, pb1, fb_outer=False):
        def piece(fb, pb):
            pk = _phi(_nt(_bf(wkt[fb * 64:(fb + 1) * 64, :]), tile("x", pb * 128, 128)))
            pkt[fb * 64:(fb + 1) * 64, pb * 128:(pb + 1) * 128] = _pk(pk)
            rows = slice(fb * 128, (fb + 1) * 128)
            if pb == 0:
                zacc[rows, :] = pk
            else:
                zacc[rows, :] += pk
        idx = [(fb, pb) for pb in range(pb0, pb1) for fb in range(4)]
        if fb_outer:
            idx.sort()
        return [(functools.partial(piece, fb, pb), 128, 230) for fb, pb in idx]

    def g_pieces():
        st = {}

        def piece(fb, cb, kb):
            r = _nn(_bf(pkt[fb * 32:(fb + 1) * 32, kb * 512:(kb + 1) * 512]),
                    _bf(xp[kb * 256:(kb + 1) * 256, cb * 128:(cb + 1) * 128]))
            if kb > 0:
                r = r + st["acc"]
            if kb == 3:
                gp[fb * 32:(fb + 1) * 32, cb * 128:(cb + 1) * 128] = _pk(r)
            else:
                st["acc"] = r
        return [(functools.partial(piece, fb, cb, kb), 64, 32)
                for fb in range(8) for cb in range(4) for kb in range(4)]

    def mid_pieces():
        st = {}

        def bd():
            r128 = lax.broadcasted_iota(jnp.int32, (128, 128), 0)
            c128 = lax.broadcasted_iota(jnp.int32, (128, 128), 1)
            return (r128 >> 4) == (c128 >> 4)

        def kv(fb):
            g = fb // 2
            r = _nn(_bf(gp[fb * 32:(fb + 1) * 32, :]), wb[:, 2 * D + g * 128:2 * D + (g + 1) * 128])
            st[fb] = jnp.where(bd()[(fb % 2) * 64:(fb % 2) * 64 + 64], r, 0.0).astype(BF16)

        def mm(fb):
            g = fb // 2
            m = _pk(_nn(st[fb], wob[g * 128:(g + 1) * 128, :]))
            for c in range(4):
                mp[c, fb * 32:(fb + 1) * 32, :] = m[:, c * 128:(c + 1) * 128]

        def zz():
            for g in range(4):
                za = zacc[g * 128:(g + 1) * 128, :]
                z = jnp.sum(za, axis=1, keepdims=True)
                zb[g] = jnp.where(bd(), jnp.broadcast_to(z, (128, 128)), 0.0)
                zpk[g * 64:(g + 1) * 64, :] = _pk(za)
            zrow[...] = _nt(jnp.ones((16, 128), BF16), _bf(perm_rows(zpk)))
        return ([(functools.partial(kv, fb), 64, 40) for fb in range(8)],
                [(functools.partial(mm, fb), 64, 16) for fb in range(8)], [(zz, 64, 120)])

    def q_pieces(rb0, rb1):
        def piece(rb, g):
            w = wb[:, g * 128:(g + 1) * 128] if rb < QOLD else _bf(wqp[:, g * 128:(g + 1) * 128])
            pq[rb * 64:(rb + 1) * 64, g * 128:(g + 1) * 128] = _phi(_nn(tile("x", rb * 64, 64), w))
        return [(functools.partial(piece, rb, g), 64, 64) for rb in range(rb0, rb1) for g in range(4)]

    def o_stream(rb0, rb1, q0):
        st = {}

        def den_mxu(rb):
            rows = slice(rb * 64, (rb + 1) * 64)
            for g in range(4):
                cols = slice(g * 128, (g + 1) * 128)
                d = _nn(pq[rows, cols], zb[g]) + 1e-6
                pp[rb * 32:(rb + 1) * 32, cols] = _pk(pq[rows, cols] * pl.reciprocal(d, approx=True))

        def den_vpu(rb):
            lane = lax.broadcasted_iota(jnp.int32, (16, 128), 1)
            for v in range(rb * 4, rb * 4 + 4):
                p = pq[v * 16:v * 16 + 16, :] * zrow[...]
                t = ((p[:, 0:128] + p[:, 128:256]) + p[:, 256:384]) + p[:, 384:512]
                t = t + jnp.take_along_axis(t, lane ^ 2, axis=1)
                t = t + jnp.take_along_axis(t, lane ^ 1, axis=1)
                r = pl.reciprocal(t + 1e-6, approx=True)
                pp[v * 8:v * 8 + 8, :] = _pk(pq[v * 16:v * 16 + 16, :] * jnp.concatenate([r] * 4, axis=1))

        def out(rb, g):
            m = mp[g, 0:D // 2, :] if rb < QOLD else perm_rows(mp.at[g])
            r = _nn(_bf(pp[rb * 32:(rb + 1) * 32, :]), _bf(m))
            if g % 2 == 0:
                st["r"] = r
            else:
                sta[rb * 64:(rb + 1) * 64, (g - 1) * 128:(g + 1) * 128] = jnp.concatenate(
                    [st["r"], r], axis=1).astype(BF16)

        res = []
        for t in range(rb0 - 2, rb1):
            step = []
            ov = 60 if t + 1 >= q0 else 28
            if q0 <= t + 2 < rb1:
                step += q_pieces(t + 2, t + 3)
            if rb0 <= t:
                step += [(functools.partial(out, t, g), 64, ov) for g in (0, 1)]
            if rb0 <= t + 1 < rb1:
                step.append((functools.partial(den_mxu, t + 1), 64, 80) if t + 1 < QOLD
                            else (functools.partial(den_vpu, t + 1), 0, 128))
            if rb0 <= t:
                step += [(functools.partial(out, t, g), 64, ov) for g in (2, 3)]
            res.append(step)

        def seg(a, b):
            return [p for step in res[a - rb0 + 2:b - rb0 + 2] for p in step]
        return seg

    prm_hbm = (are_hbm, aim_hbm, bre_hbm, bim_hbm, cre_hbm, cim_hbm)

    def prm_rest(i):
        return prm_hbm[i].at[R0:D], prm.at[i, R0:D]

    srcs = {"ldt": (ldt_hbm, ldt)}
    srcs.update({"a%d" % i: (prm_hbm[i].at[0:R0], prm.at[i, 0:R0]) for i in range(6)})
    srcs.update({
        "wq": (w_hbm.at[:, 0:D], wb.at[:, 0:D]),
        "x0": (x_hbm.at[0:X0], xb.at[0:X0]),
        "dsk": (dsk_hbm, dsk),
        "p0": prm_rest(0),
        "p1": prm_rest(1),
        "wk": (w_hbm.at[:, D:2 * D], wb.at[:, D:2 * D]),
        "p2": prm_rest(2),
        "p3": prm_rest(3),
        "p4": prm_rest(4),
        "p5": prm_rest(5),
        "x1": (x_hbm.at[X0:X1], xb.at[X0:X1]),
        "fi": (fi_hbm, fi),
        "fk": (fk_hbm, fk),
        "ua": (u_hbm.at[:, 0:256], ub.at[:, 0:256]),
        "x2": (x_hbm.at[X1:S], xb.at[X1:S]),
        "ub": (u_hbm.at[:, 256:D], ub.at[:, 256:D]),
        "wv": (w_hbm.at[:, 2 * D:3 * D], wb.at[:, 2 * D:3 * D]),
        "wo": (wo_hbm, wob),
    })
    cin = {k: pltpu.make_async_copy(a, b, sem_in.at[i]) for i, (k, (a, b)) in enumerate(srcs.items())}
    for c in cin.values():
        c.start()
    couts = []

    def wait(*names):
        for n in names:
            cin[n].wait()

    def out_copy(i, kind, a, b):
        if kind == "a":
            return pltpu.make_async_copy(sta.at[a * 64:b * 64], o_hbm.at[a * 64:b * 64, 0:D], sem_out.at[i])
        c0 = D + kind * 128
        return pltpu.make_async_copy(stb.at[kind, a * 128:b * 128],
                                     o_hbm.at[a * 128:b * 128, c0:c0 + 128], sem_out.at[i])

    def store(*box):
        out_copy(len(couts), *box).start()
        couts.append(box)

    q0, q1 = X0 // 64, X1 // 64
    p0, p1 = X0 // 128, X1 // 128
    qe = q_pieces(q1, q1 + 3)
    mid1, mid2, midz = mid_pieces()
    gps = g_pieces()
    gs = []
    for fb in range(8):
        blk = gps[fb * 16:(fb + 1) * 16]
        if fb:
            blk = blk[:4] + [mid1[fb - 1]] + blk[4:9] + [mid2[fb - 1]] + blk[9:]
        gs += blk
    kds = [kdft_pieces(j, 20 if j >= 2 else 0) for j in range(4)]
    uds = [udft_pieces(j) for j in range(4)]
    cv = [[(p, 0, 4) for p in range(32)],
          [(p, 0, 4) for p in range(32, 48)],
          [(p, 0, 3) for p in range(48, 64)] + [(p, 3, 4) for p in range(48, C3)],
          [(p, 3, 4) for p in range(C3, 64)]]
    oseg = o_stream(0, O3, q1 + 3)
    oseg2 = o_stream(O3, 32, O3)

    main3 = uds[0][:8] + [(k0_all, 8, 0)] + uds[0][8:] + kds[0] + uds[1][:10] + kds[1] + uds[1][10:]
    blk3 = main3[:1] + _merge(main3[1:-3], kgen_pieces(G0, 64)) + main3[-3:]
    ql = q_pieces(q0 - 1, q0)
    blk4 = (uds[2][:2] + _merge(kt_pieces(p1, 16), uds[2][2:13]) + uds[2][13:]
            + _merge(gs[:GS], midz + kds[2] + kds[3], uds[3]))
    blk5 = _merge(gs[GS:] + qe[:4] + [mid1[7]] + oseg(-2, 0) + qe[4:8] + [mid2[7]] + qe[8:] + oseg(0, O1),
                  inv_pieces(0) + inv_pieces(1))
    blk5 = [(f, c, v + (50 if 8 <= i < 32 else 0)) for i, (f, c, v) in enumerate(blk5)]
    last = oseg2(O4, 32)
    ta = oseg2(O3, O4)
    blk8 = oseg2(O3 - 2, O3) + ta[:-5] + inv_pieces(3)[6:] + [p for p in last if p[1] == 0] + ta[-5:]
    blk9 = [p for p in last if p[1] != 0]

    steps = [
        (lambda: wait("ldt"), setup_dt_first),
        (lambda: wait("a0", "a1", "a2", "a3", "a4", "a5"), early_prep),
        (early_exact, lambda: _emit(kgen_pieces(0, G0))),
        (lambda: wait("wq", "x0", "dsk"),
         lambda: (setup_dt_rest(), wq_perm_a(), _emit(q_pieces(0, q0 - 1)))),
        (lambda: wait("p0", "p1", "wk"),
         lambda: (wk_transpose(), range_check(0, R0, D),
                  _emit(ql[:3] + kt_pieces(0, p0, True), stage1(), (32 - G0 // 2) * 90, tail=130))),
        (lambda: (stage1_exact(), wait("p2", "p3", "p4", "p5", "x1")),
         lambda: (wq_perm_b(),
                  _emit(ql[3:] + kt_pieces(p0, p1) + q_pieces(q0, q1), stage2_fill(G0 // 2, 32), (32 - G0 // 2) * 164))),
        (lambda: wait("fi", "fk", "ua"), lambda: (setup_g(), _emit(blk3))),
        (lambda: wait("x2", "ub", "wv", "wo"), lambda: _emit(blk4, conv(cv[0]), conv_ops(cv[0]), 3.6)),
        (None, lambda: _emit(blk5, conv(cv[1]), conv_ops(cv[1]), 3.7)),
        (lambda: (store(0, 0, 16), store(1, 0, 16), store("a", 0, O1)),
         lambda: _emit(_merge(oseg(O1, O2), inv_pieces(2)), conv(cv[2]), conv_ops(cv[2]), 3.5)),
        (lambda: (store(2, 0, 16), store("a", O1, O2)),
         lambda: _emit(_merge(oseg(O2, O3), inv_pieces(3)[:6]), conv(cv[3]), conv_ops(cv[3]), 3.4)),
        (lambda: (store(3, 0, 12), store("a", O2, O3)), lambda: _emit(blk8)),
        (lambda: (store(3, 12, 16), store("a", O3, O4)), lambda: _emit(blk9)),
        (lambda: store("a", O4, 32), None),
    ]

    def outer(i, c):
        packed.clear()
        couts.clear()
        for k in range(len(steps) - 1):
            @pl.when(i + k == k)
            def _():
                steps[k][1]()
                if steps[k + 1][0] is not None:
                    steps[k + 1][0]()
        return c

    steps[0][0]()
    lax.fori_loop(0, 2, outer, 0)
    for i, box in enumerate(couts):
        out_copy(i, *box).wait()


@jax.jit
def pallas_concat_heads__linear_attn_block__ssm_conv_s4__prompt_kernel(
    A_x, A_wqkv, A_wo, B_u, B_A_re, B_A_im, B_B_re, B_B_im, B_C_re, B_C_im, B_log_dt, B_Dskip,
):
    fk, fi = _tables()
    V = pltpu.VMEM
    out = pl.pallas_call(
        _kernel,
        out_shape=jax.ShapeDtypeStruct((S, 2 * D), BF16),
        in_specs=[pl.BlockSpec(memory_space=pl.ANY)] * 14,
        out_specs=pl.BlockSpec(memory_space=pl.ANY),
        scratch_shapes=[
            V((S // 2, D), U32),
            V((D, 3 * D), BF16),
            V((D, D), BF16),
            V((S // 2, D), U32),
            V((6, D, 128), BF16),
            V((D,), BF16),
            V((D,), BF16),
            V((S, D), BF16),
            V((S, D), BF16),
            V((FK_ROWS // 2, 128), U32),
            V((136, 128), F32),
            V((S, D), BF16),
            V((4, S, 128), BF16),
            V((2, D, 128), F32),
            pltpu.SMEM((2,), jnp.int32),
            V((D, 128), F32),
            V((8, 128, 128), F32),
            V((14, 2 * D + 8, 128), F32),
            V((D, 128), F32),
            V((5, D // 2, 128), U32),
            V((4, 2, 16, 128), F32),
            V((8, D), F32),
            V((4, 3, 16, 128, 128), F32),
            V((4, 3, 16, 128, 128), F32),
            V((4, 2, 16, 128, 128), F32),
            V((D // 2, D), U32),
            V((D // 2, S), U32),
            V((D, 128), F32),
            V((D // 2, D), U32),
            V((4, D // 2 + 8, 128), U32),
            V((4, 128, 128), F32),
            V((S, D), F32),
            V((S // 2, D), U32),
            V((4, D // 2 + 8, 128), U32),
            V((D // 2, D), U32),
            V((D // 2 + 8, 128), U32),
            V((16, D), F32),
            V((4, 12, 144, 128), F32),
            V((2, 128, 128), F32),
            pltpu.SemaphoreType.DMA((25,)),
            pltpu.SemaphoreType.DMA((10,)),
        ],
        compiler_params=pltpu.CompilerParams(vmem_limit_bytes=110 * 2**20, disable_semaphore_checks=True),
    )(A_x.reshape(S, D), A_wqkv, A_wo, B_u.reshape(S, D), B_A_re, B_A_im, B_B_re, B_B_im, B_C_re, B_C_im,
      B_log_dt, B_Dskip, jnp.asarray(fk), jnp.asarray(fi))
    return out.reshape(1, S, 2 * D)
```

```python
import functools

import numpy as np
import jax
import jax.numpy as jnp
from jax import lax
import jax.experimental.pallas as pl
import jax.experimental.pallas.tpu as pltpu

S = 2048
D = 512
F32 = jnp.float32
BF16 = jnp.bfloat16
U32 = jnp.uint32

_BASE = np.array([[1, 5], [2, 6], [3, 7], [4, 8], [258, 262], [260, 264],
                  [516, 520], [772, 776], [1032, 1288], [1544, 1800]])
_TILE_OF_CHUNK = [0, 1, 2, 2, 3, 3, 3, 3] + [4] * 8

FK_OFF = [0, 256, 528, 784] + [1056 + 144 * k for k in range(4)] + [1632 + 80 * k for k in range(8)]
FK_FU = 1632 + 640
FK_ROWS = FK_FU + 256

X0, X1 = 384, 896
QOLD = X0 // 64
G0 = 12
R0 = 8 * G0
O1, O2, O3, O4 = 15, 24, 29, 31
GS = 120
C3 = 51

B_W1, B_W2, B_W8C, B_W256, B_W512, B_E0, B_N0 = range(7)
_SC_LIMIT = 8192.0


def _bf16_bits(v):
    u = np.ascontiguousarray(v, np.float32).view(np.uint32)
    return ((u + 0x7FFF + ((u >> 16) & 1)) >> 16).astype(np.uint32)


def _pack_rows(v):
    b = _bf16_bits(v)
    return b[0::2] | (b[1::2] << 16)


@functools.lru_cache(maxsize=None)
def _tables():
    lr = (_bf16_bits(np.arange(S)) << 16).view(np.float32).astype(np.int64)
    val = np.zeros((5, 128), np.int64)
    for lam in range(128):
        mu, tau = 15 - (lam >> 3), lam & 7
        e, x = tau >> 1, tau & 1
        for h in range(2):
            val[h, lam] = _BASE[e, x ^ h] + 8 * (mu + 16 * h)
        hp, ab, h = tau >> 2, (tau >> 1) & 1, tau & 1
        for q in range(3):
            val[2 + q, lam] = _BASE[4 + 2 * q + ab, hp] + 8 * (mu + 16 * h)
    om = 2 * np.pi * (np.arange(128) + 0.25) / 128.0
    phase = np.exp(1j * om * 191.5)

    def stack(z):
        return np.concatenate([p[32 * t:32 * t + 32] for t in range(4) for p in (z.real, z.imag)], axis=0)

    fk = []
    g = np.zeros(128, np.complex128)
    for k in range(4):
        slot = {int(v): i for i, v in enumerate(val[_TILE_OF_CHUNK[k]])}
        m = np.zeros((128, 128), np.complex128)
        for p in range(1, 129):
            lag = 128 * k + p
            v = int(lr[lag])
            z = np.exp(-1j * om * p) * (0.5 if lag == 512 else 1.0)
            if v in slot:
                m[:, slot[v]] += z
            else:
                assert v == 256 and k == 2
                g += z
        if k in (1, 3):
            sel = np.zeros((16, 128))
            sel[:, slot[128 * (k + 1)]] = 1.0
            fk += [stack(m)[:128], sel, stack(m)[128:]]
        else:
            fk.append(stack(m))
    for k in range(4, 16):
        st = 4 if k < 8 else 8
        per = 128 // st
        slot = {int(v): i for i, v in enumerate(val[_TILE_OF_CHUNK[k]])}
        for lag in range(128 * k + 1, min(128 * k + 128, S)):
            m_ = int(lr[lag]) // st
            assert int(lr[lag]) % st == 0 and abs(lag - st * m_) <= (st // 2 if m_ % 2 == 0 else st // 2 - 1)
        od = np.zeros((per, 128), np.complex128)
        ev = np.zeros((per, 128), np.complex128)
        edge = np.zeros((16, 128))
        for m_ in range(per + 1):
            v = 128 * k + st * m_
            if v not in slot:
                assert m_ == 0 and k in (4, 8)
                continue
            z = np.exp(-1j * om[:per] * st * m_)
            if m_ % 2:
                od[:, slot[v]] = z
            else:
                ev[:, slot[v]] = z * (0.5 if m_ in (0, per) else 1.0)
            if m_ in (0, per):
                edge[8 * (m_ // per):8 * (m_ // per) + 8, slot[v]] = 1.0
        fk += [edge, od.real, od.imag, ev.real, ev.imag]
    fk.append(stack(np.exp(-1j * om[:, None] * np.arange(128)[None, :]) * phase[:, None]))
    fk = np.concatenate(fk, axis=0)
    assert fk.shape[0] == FK_ROWS
    tabs = [g.real, g.imag]
    for h in (2, 4):
        tabs += [sum(np.cos(om * p) for p in range(1 - h, h)), sum(np.cos(om * p) for p in range(-h, h + 1)),
                 -sum(np.sin(om * p) for p in range(1, h + 1))]
    jj = np.arange(64)[:, None] - 63.5
    finv = np.concatenate([np.cos(om[None, :] * jj) / 128.0, -np.sin(om[None, :] * jj) / 128.0,
                           np.stack(tabs)], axis=0)
    return _pack_rows(fk), finv.astype(np.float32)


def _cmul(a, b):
    return a[0] * b[0] - a[1] * b[1], a[0] * b[1] + a[1] * b[0]


def _csq(a):
    return a[0] * a[0] - a[1] * a[1], (a[0] + a[0]) * a[1]


def _phi(t):
    return jnp.where(t > 0, t + 1.0, jnp.exp(t)) + 1e-6


def _nt(a, b):
    return lax.dot_general(a, b, (((1,), (1,)), ((), ())), preferred_element_type=F32)


def _nn(a, b):
    return jnp.dot(a, b, preferred_element_type=F32)


def _bf(v):
    return pltpu.bitcast(v, BF16)


def _pk(v):
    return pltpu.bitcast(v.astype(BF16), U32)


def _sincos(x):
    t = x * 0.6366197723675814 + 12582912.0
    n = pltpu.bitcast(t, jnp.int32) - 0x4B400000
    k = n.astype(F32)
    r = ((x - k * 1.5703125) - k * 4.837512969970703125e-4) - k * 7.54978995489188216e-8
    r2 = r * r
    sn = r + r * r2 * (-1.6666654611e-1 + r2 * (8.3321608736e-3 + r2 * -1.9515295891e-4))
    cs = 1.0 + r2 * (-0.5 + r2 * (4.166664568298827e-2 + r2 * (-1.388731625493765e-3 + r2 * 2.443315711809948e-5)))
    swap = (n & 1) == 1
    s_, c_ = jnp.where(swap, cs, sn), jnp.where(swap, sn, cs)
    ssign = (n & 2) << 30
    csign = ((n + 1) & 2) << 30
    s_ = pltpu.bitcast(pltpu.bitcast(s_, jnp.int32) ^ ssign, F32)
    c_ = pltpu.bitcast(pltpu.bitcast(c_, jnp.int32) ^ csign, F32)
    return s_, c_


def _emit(pieces, filler=None, fill_total=0, cap=3.0, tail=100):
    filler = iter(()) if filler is None else filler
    room = [max(cap * c - v, 0.0) for _, c, v in pieces]
    tot = sum(room[:-1]) or 1.0
    done, target = 0.0, 0.0
    for (fn, _, _), r in zip(pieces, room):
        fn()
        target += max(fill_total - tail, 0) * r / tot
        while done < target - 8:
            n = next(filler, None)
            if n is None:
                break
            done += n
    for _ in filler:
        pass


def _merge(*lists):
    tot = [sum(p[1] for p in l) or 1.0 for l in lists]
    pos = [0] * len(lists)
    acc = [0.0] * len(lists)
    out = []
    while True:
        best = None
        for i, l in enumerate(lists):
            if pos[i] < len(l):
                key = (acc[i] + 0.5 * l[pos[i]][1]) / tot[i]
                if best is None or key < best[0]:
                    best = (key, i)
        if best is None:
            return out
        i = best[1]
        out.append(lists[i][pos[i]])
        acc[i] += lists[i][pos[i]][1]
        pos[i] += 1


def _group(pieces, n):
    out = []
    for i in range(0, len(pieces), n):
        grp = pieces[i:i + n]

        def run(grp=grp):
            for f, _, _ in grp:
                f()
        out.append((run, sum(p[1] for p in grp), sum(p[2] for p in grp)))
    return out


def _reim(r):
    n = r.shape[0] // 64
    return (jnp.concatenate([r[64 * t:64 * t + 32] for t in range(n)], axis=0),
            jnp.concatenate([r[64 * t + 32:64 * t + 64] for t in range(n)], axis=0))


def _kernel(x_hbm, w_hbm, wo_hbm, u_hbm, are_hbm, aim_hbm, bre_hbm, bim_hbm, cre_hbm, cim_hbm,
            ldt_hbm, dsk_hbm, fk_hbm, fi_hbm, o_hbm,
            xp, wb, wob, up, prm, ldt, dsk, xb, ub, fk, fi, sta, stb, w1s, flag,
            dtb, gb, base, cr, wt, bv, k0s, kw, u3, y, wkt, pkt, zacc, gp, mp, zb, pq, pp,
            wqt, wqp, zpk, zrow, kf, zc, sem_in, sem_out):

    def iotas():
        return (lax.broadcasted_iota(jnp.int32, (8, 128), 0), lax.broadcasted_iota(jnp.int32, (8, 128), 1))

    packed = set()

    def tile(kind, r0, n, cols=slice(None)):
        src, dst = (xb, xp) if kind == "x" else (ub, up)
        parts = []
        for r in range(r0, r0 + n, 64):
            key = (kind, r, cols.start)
            if key in packed:
                parts.append(_bf(dst[r // 2:r // 2 + 32, cols]))
            else:
                packed.add(key)
                v = src[r:r + 64, cols]
                dst[r // 2:r // 2 + 32, cols] = pltpu.bitcast(v, U32)
                parts.append(v)
        return parts[0] if len(parts) == 1 else jnp.concatenate(parts, axis=0)

    def dt_row():
        return jnp.exp(ldt[...].reshape(1, D).astype(F32)).astype(BF16).astype(F32)

    def setup_dt_first():
        sub, _ = iotas()
        b = jnp.broadcast_to(dt_row()[:, 0:128], (8, 128))
        for v in range(16):
            dtb[v * 8:v * 8 + 8, :] = jnp.take_along_axis(b, sub + 8 * v, axis=1)

    def setup_dt_rest():
        row = dt_row()
        for j in range(1, 4):
            dtb[j * 128:(j + 1) * 128, :] = jnp.broadcast_to(row[:, j * 128:(j + 1) * 128], (128, 128)).T

    def setup_g():
        for i in range(8):
            gb[i] = jnp.broadcast_to(fi[128 + i:129 + i, :], (128, 128)).T

    def perm_rows(ref):
        return jnp.concatenate([ref[pl.ds(t, 64, stride=4), :] for t in range(4)], axis=0)

    def wq_perm_a():
        for a in range(4):
            for b in range(4):
                t = wb[a * 128:(a + 1) * 128, b * 128:(b + 1) * 128].T
                wqt[a, b * 64:(b + 1) * 64, :] = pltpu.bitcast(t, U32)

    def wq_perm_b():
        for b in range(4):
            for a in range(4):
                t = _bf(wqt[a, pl.ds(b, 64, stride=4), :]).T
                wqp[a * 64:(a + 1) * 64, b * 128:(b + 1) * 128] = pltpu.bitcast(t, U32)

    def wk_transpose():
        for b in range(4):
            for a in range(4):
                t = wb[a * 128:(a + 1) * 128, D + b * 128:D + (b + 1) * 128].T
                wkt[b * 64:(b + 1) * 64, a * 128:(a + 1) * 128] = pltpu.bitcast(t, U32)

    def w1_rows(r0, exact):
        rows = pl.ds(r0, 16)
        dt = dtb[rows, :]
        ar = dt * prm[0, rows, :].astype(F32)
        ai = dt * prm[1, rows, :].astype(F32)
        mag = jnp.exp(ar)
        sn, cs = (jnp.sin(ai), jnp.cos(ai)) if exact else _sincos(ai)
        w1s[0, rows, :] = mag * cs
        w1s[1, rows, :] = mag * sn

    def range_check(i, r0, r1):
        m = jnp.max(jnp.abs(prm[1, r0:r1, :].astype(F32)).reshape((r1 - r0) // 8, 8, 128), axis=0)
        dmax = jnp.max(dtb[r0:r1, :].reshape((r1 - r0) // 8, 8, 128), axis=0)
        bound = jnp.max(m) * jnp.max(dmax)
        flag[i] = jnp.where(bound <= _SC_LIMIT, 0, 1).astype(jnp.int32)

    def stage1():
        for r in range(G0 // 2, 32):
            w1_rows(r * 16, False)
            yield 90

    def stage1_exact():
        @pl.when(flag[0] != 0)
        def _():
            def body(r, c):
                w1_rows(pl.multiple_of(r * 16, 16), True)
                return c
            lax.fori_loop(G0 // 2, 32, body, 0)

    def stage2(r):
        r0 = r * 16 if isinstance(r, int) else pl.multiple_of(r * 16, 16)
        rows = pl.ds(r0, 16)
        dt = dtb[rows, :]
        w1 = (w1s[0, rows, :], w1s[1, rows, :])
        db = (dt * prm[2, rows, :].astype(F32), dt * prm[3, rows, :].astype(F32))
        c = _cmul((prm[4, rows, :].astype(F32), prm[5, rows, :].astype(F32)), db)
        cr[rows, :] = c[0]
        lo = (lax.broadcasted_iota(jnp.int32, (16, 128), 0) & 4) == 0

        def put(i, v0, v1=None):
            for t in range(2):
                ev, od = (v0[t], v0[t]) if v1 is None else (jnp.where(lo, v0[t], v1[t]), jnp.where(lo, v1[t], v0[t]))
                base[2 * i + t, pl.ds(2 * r0, 16, stride=2), :] = ev
                base[2 * i + t, pl.ds(2 * r0 + 1, 16, stride=2), :] = od
        put(B_W1, w1)
        w2 = _csq(w1)
        put(B_W2, w2)
        w4 = _csq(w2)
        cw1 = _cmul(c, w1)
        put(B_N0, cw1, _cmul(cw1, w4))
        yield 80
        w8 = _csq(w4)
        put(B_W8C, (w8[0], -w8[1]))
        w128 = _csq(_csq(_csq(_csq(w8))))
        put(B_E0, (jnp.ones((16, 128), F32), jnp.zeros((16, 128), F32)), (w128[0], -w128[1]))
        w256 = _csq(w128)
        put(B_W256, w256)
        put(B_W512, _csq(w256))
        yield 84

    def stage2_fill(r0, r1):
        for r in range(r0, r1):
            yield from stage2(r)

    def early_prep():
        range_check(1, 0, R0)
        for r in range(G0 // 2):
            w1_rows(r * 16, False)
        for _ in stage2_fill(0, G0 // 2):
            pass

    def early_exact():
        @pl.when(flag[1] != 0)
        def _():
            def body(r, c):
                w1_rows(pl.multiple_of(r * 16, 16), True)
                for _ in stage2(r):
                    pass
                return c
            lax.fori_loop(0, G0 // 2, body, 0)

    def kgen_pieces(g0, g1):
        st = {}

        def group(gi):
            sub, lane = iotas()
            odd = (sub & 1) == 1
            rows = slice(gi * 16, gi * 16 + 16)

            def ld(i):
                return base[2 * i, rows, :], base[2 * i + 1, rows, :]
            w8c = ld(B_W8C)
            e0 = [ld(B_E0)]
            for _ in range(1, 16):
                e0.append(_cmul(e0[-1], w8c))
            e0 = e0[::-1]
            w1, w2, w256, w512 = ld(B_W1), ld(B_W2), ld(B_W256), ld(B_W512)
            n0 = ld(B_N0)
            n1 = _cmul(n0, w1)
            n2 = _cmul(n0, w2)
            n3 = _cmul(n1, w2)
            n4 = _cmul(n1, w256)
            n5 = _cmul(n3, w256)
            n6 = _cmul(n5, w256)
            n7 = _cmul(n6, w256)
            t = tuple(jnp.concatenate([jnp.where(odd, n7[c][0:8], pltpu.roll(n6[c][0:8], 7, 0)),
                                       jnp.where(odd, pltpu.roll(n6[c][8:16], 1, 0), n7[c][8:16])], axis=0)
                      for c in range(2))
            n8 = _cmul(t, w512)
            n9 = _cmul(n8, w512)
            e1 = [n0, n1, n2, n3, n4, n5, n6, n7, n8, n9]

            def operands(es):
                v = jnp.concatenate([jnp.concatenate([e[0] for e in es], axis=0),
                                     jnp.concatenate([e[1] for e in es], axis=0)], axis=1)
                v = v.reshape(len(es), 2, 8, 256)
                return [v[:, g].reshape(len(es) * 8, 256) for g in range(2)]
            o = []
            for lhs, rhs in zip(operands(e1), operands(e0)):
                r = _nt(lhs, rhs)
                o.append([r[8 * i:8 * i + 8, :] for i in range(10)])

            emask = ((sub >> 1) - (lane >> 1)) & 3
            ea, xa = (lane >> 1) & 3, lane & 1
            lidx_a = (lane & 120) | ((((sub >> 1) - ea) & 3) << 1) | (xa ^ (sub & 1))
            sidx_a = ((((sub & 3) + ea) & 3) << 1) | (xa ^ (sub >> 2))
            hp, ab, hh = (lane >> 2) & 1, (lane >> 1) & 1, lane & 1
            gg = hp ^ (sub & 1)
            lidx_b = (lane & 120) | ((((sub >> 1) - (2 * gg + ab)) & 3) << 1) | (hh ^ gg)
            g2 = sub >> 2
            sidx_b = ((((sub & 3) + 2 * g2 + ab) & 3) << 1) | (hp ^ g2)

            def compact(srcs, lidx, sidx):
                s = srcs[0]
                for e in range(1, 4):
                    s = jnp.where(emask == e, pltpu.roll(srcs[e], 2 * e, 0), s)
                s = jnp.take_along_axis(s, lidx, axis=1)
                return jnp.take_along_axis(s, sidx, axis=0)

            a2 = [compact(o[g][0:4], lidx_a, sidx_a) for g in range(2)]
            lo = sub < 4
            res = [jnp.where(lo, a2[0], a2[1]), pltpu.roll(jnp.where(lo, a2[1], a2[0]), 4, 0)]
            for q in range(3):
                res.append(compact(o[0][4 + 2 * q:6 + 2 * q] + o[1][4 + 2 * q:6 + 2 * q], lidx_b, sidx_b))
            if gi % 2 == 0:
                st["r"] = res
            else:
                for q in range(5):
                    wt[q, (gi // 2) * 8:(gi // 2) * 8 + 8, :] = _pk(jnp.concatenate([st["r"][q], res[q]], axis=0))

        return [(functools.partial(group, gi), 80, 360) for gi in range(g0, g1)]

    def k0_all():
        k0s[...] = _nt(jnp.ones((8, 128), F32), cr[...]) + dsk[...].reshape(1, D).astype(F32)

    def kdft_pieces(j, extra):
        def wtile(k):
            return _bf(wt[_TILE_OF_CHUNK[k], j * 64:(j + 1) * 64, :])

        def near(k, hf):
            o = FK_OFF[k] // 2 + hf * 64
            if k in (1, 3):
                r = _nt(_bf(fk[o:o + 72, :]), wtile(k))
                bv[j, k // 2, hf * 8:hf * 8 + 8, :] = r[128:136] if hf == 0 else r[0:8]
                r = r[:128] if hf == 0 else r[16:]
            else:
                r = _nt(_bf(fk[o:o + 64, :]), wtile(k))
            rr, ri = _reim(r)
            rows = slice(hf * 64, hf * 64 + 64)
            if k == 0:
                rr = rr + jnp.concatenate([k0s[:, j * 128:(j + 1) * 128]] * 8, axis=0)
            elif k == 2:
                bval = jnp.concatenate([bv[j, 0]] * 4, axis=0)
                rr = rr + gb[0, rows, :] * bval
                ri = ri + gb[1, rows, :] * bval
            kw[j, 0, k, rows, :] = rr
            kw[j, 1, k, rows, :] = ri
            kw[j, 2, k, rows, :] = rr + ri

        def far(k):
            per = 32 if k < 8 else 16
            n = 16 + 4 * per
            o = FK_OFF[k] // 2
            r = _nt(_bf(fk[o:o + n // 2, :]), wtile(k))
            if k in (4, 8):
                e0 = 16 + 2 * per
                v0 = bv[j, 1] if k == 4 else jnp.concatenate([kf[j, 3, 8:16, :]] * 2, axis=0)
                r = jnp.concatenate([v0[0:8], r[8:e0], r[e0:e0 + per] + 0.5 * jnp.concatenate([v0] * (per // 16), axis=0),
                                     r[e0 + per:]], axis=0)
            kf[j, k - 4, 0:n, :] = r

        def nears(ks, v):
            return _group([(functools.partial(near, k, hf), 32, v + extra) for k in ks for hf in range(2)], 4)

        def fars(ks):
            return _group([(functools.partial(far, k), 36 if k < 8 else 20, extra) for k in ks], 4)
        return (nears((1, 3), 8) + fars((12, 13, 14, 15)) + fars((7, 6, 5, 4))
                + nears((0, 2), 28) + fars((9, 10, 11, 8)))

    def udft_pieces(j):
        def piece(ib, qf):
            o = FK_FU // 2 + qf * 32
            w = jnp.concatenate([tile("u", i * 128, 128, slice(j * 128, (j + 1) * 128))
                                 for i in range(ib * 4, ib * 4 + 4)], axis=1)
            r = _nn(_bf(fk[o:o + 32, :]), w)
            rows = slice(qf * 32, qf * 32 + 32)
            for t in range(4):
                rr, ri = r[:32, t * 128:(t + 1) * 128], r[32:, t * 128:(t + 1) * 128]
                u3[j, 0, ib * 4 + t, rows, :] = rr
                u3[j, 1, ib * 4 + t, rows, :] = ri
                u3[j, 2, ib * 4 + t, rows, :] = rr + ri
        return [(functools.partial(piece, ib, qf), 64, 16) for ib in range(4) for qf in range(4)]

    def conv_ops(items):
        return sum((68, 204, 300, 396)[ib] for _, i0, i1 in items for ib in range(i0, i1))

    def conv(items):
        for pos, ib0, ib1 in items:
            j, p = divmod(pos, 16)
            rs = slice(p * 8, p * 8 + 8)
            prev = None if ib0 == 0 else (zc[0:1, rs, :], zc[1:2, rs, :])
            for ib in range(ib0, ib1):
                if ib > 0:
                    t0 = 2 if ib == 1 else 5
                    d_od, d_ev, sh = (gb[t0 + t:t0 + t + 1, rs, :] for t in range(3))
                    per = 32 if ib == 1 else 16
                    h = 16 + (8 * p) % per
                    left = sh * kf[j, 4 * ib - 4:4 * ib - 3, 0:8, :]
                    for k in range(4 * ib, 4 * ib + 4, 2):
                        o_r, o_i, e_r, e_i = (kf[j, k - 4:k - 2, per * t + h:per * t + h + 8, :] for t in range(4))
                        right = sh * kf[j, k - 4:k - 2, 8:16, :]
                        rr = d_od * o_r + d_ev * e_r - right
                        ri = d_od * o_i + d_ev * e_i + jnp.concatenate([left, right[:1]], axis=0)
                        left = right[1:]
                        kw[j, 0, k:k + 2, rs, :] = rr
                        kw[j, 1, k:k + 2, rs, :] = ri
                        kw[j, 2, k:k + 2, rs, :] = rr + ri
                        yield 20
                a = zr = None
                for c in range(3):
                    acc = None
                    for k in range(4 * ib + 1):
                        pr = u3[j, c, 4 * ib - k:4 * ib - k + 4, rs, :] * kw[j, c, k:k + 1, rs, :]
                        if acc is None:
                            acc = pr - a if c == 2 else pr
                        else:
                            acc = acc + pr
                        if k % 4 == 3:
                            yield 32
                    for d in range(1, 4):
                        pr = u3[j, c, 0:4 - d, rs, :] * kw[j, c, 4 * ib + d:4 * ib + d + 1, rs, :]
                        acc = jnp.concatenate([acc[:d], acc[d:] + pr], axis=0)
                    n = 20
                    if c == 0:
                        a = acc
                    elif c == 1:
                        zr = a - acc
                        a = a + acc
                    else:
                        if prev is None:
                            yr = jnp.concatenate([acc[:1], zr[:3] + acc[1:]], axis=0)
                            yi = jnp.concatenate([-zr[:1], acc[:3] - zr[1:]], axis=0)
                        else:
                            yr = jnp.concatenate([prev[0], zr[:3]], axis=0) + acc
                            yi = jnp.concatenate([prev[1], acc[:3]], axis=0) - zr
                        y[j, 0, ib * 4:ib * 4 + 4, rs, :] = yr
                        y[j, 1, ib * 4:ib * 4 + 4, rs, :] = yi
                        prev = (zr[3:], acc[3:])
                        n += 8
                        if ib == ib1 - 1 and ib1 < 4:
                            zc[0:1, rs, :], zc[1:2, rs, :] = prev
                    yield n

    def inv_pieces(j):
        def piece(i):
            sub, _ = iotas()
            s = _nn(fi[0:64, :], y[j, 0, i])
            a = _nn(fi[64:128, :], y[j, 1, i])
            lo = s + a
            hi = s - a
            hi = jnp.concatenate(
                [jnp.take_along_axis(hi[8 * v:8 * v + 8], 7 - sub, axis=0) for v in range(7, -1, -1)], axis=0)
            stb[j, i * 128:(i + 1) * 128, :] = jnp.concatenate([lo, hi], axis=0).astype(BF16)
        return _group([(functools.partial(piece, i), 32, 32) for i in range(16)], 2)

    def kt_pieces(pb0, pb1, fb_outer=False):
        def piece(fb, pb):
            pk = _phi(_nt(_bf(wkt[fb * 64:(fb + 1) * 64, :]), tile("x", pb * 128, 128)))
            pkt[fb * 64:(fb + 1) * 64, pb * 128:(pb + 1) * 128] = _pk(pk)
            rows = slice(fb * 128, (fb + 1) * 128)
            if pb == 0:
                zacc[rows, :] = pk
            else:
                zacc[rows, :] += pk
        idx = [(fb, pb) for pb in range(pb0, pb1) for fb in range(4)]
        if fb_outer:
            idx.sort()
        return [(functools.partial(piece, fb, pb), 128, 230) for fb, pb in idx]

    def g_pieces():
        st = {}

        def piece(fb, cb, kb):
            r = _nn(_bf(pkt[fb * 32:(fb + 1) * 32, kb * 512:(kb + 1) * 512]),
                    _bf(xp[kb * 256:(kb + 1) * 256, cb * 128:(cb + 1) * 128]))
            if kb > 0:
                r = r + st["acc"]
            if kb == 3:
                gp[fb * 32:(fb + 1) * 32, cb * 128:(cb + 1) * 128] = _pk(r)
            else:
                st["acc"] = r
        return [(functools.partial(piece, fb, cb, kb), 64, 32)
                for fb in range(8) for cb in range(4) for kb in range(4)]

    def mid_pieces():
        st = {}

        def bd():
            r128 = lax.broadcasted_iota(jnp.int32, (128, 128), 0)
            c128 = lax.broadcasted_iota(jnp.int32, (128, 128), 1)
            return (r128 >> 4) == (c128 >> 4)

        def kv(fb):
            g = fb // 2
            r = _nn(_bf(gp[fb * 32:(fb + 1) * 32, :]), wb[:, 2 * D + g * 128:2 * D + (g + 1) * 128])
            st[fb] = jnp.where(bd()[(fb % 2) * 64:(fb % 2) * 64 + 64], r, 0.0).astype(BF16)

        def mm(fb):
            g = fb // 2
            m = _pk(_nn(st[fb], wob[g * 128:(g + 1) * 128, :]))
            for c in range(4):
                mp[c, fb * 32:(fb + 1) * 32, :] = m[:, c * 128:(c + 1) * 128]

        def zz():
            for g in range(4):
                za = zacc[g * 128:(g + 1) * 128, :]
                z = jnp.sum(za, axis=1, keepdims=True)
                zb[g] = jnp.where(bd(), jnp.broadcast_to(z, (128, 128)), 0.0)
                zpk[g * 64:(g + 1) * 64, :] = _pk(za)
            zrow[...] = _nt(jnp.ones((16, 128), BF16), _bf(perm_rows(zpk)))
        return ([(functools.partial(kv, fb), 64, 40) for fb in range(8)],
                [(functools.partial(mm, fb), 64, 16) for fb in range(8)], [(zz, 64, 120)])

    def q_pieces(rb0, rb1):
        def piece(rb, g):
            w = wb[:, g * 128:(g + 1) * 128] if rb < QOLD else _bf(wqp[:, g * 128:(g + 1) * 128])
            pq[rb * 64:(rb + 1) * 64, g * 128:(g + 1) * 128] = _phi(_nn(tile("x", rb * 64, 64), w))
        return [(functools.partial(piece, rb, g), 64, 64) for rb in range(rb0, rb1) for g in range(4)]

    def o_stream(rb0, rb1, q0):
        st = {}

        def den_mxu(rb):
            rows = slice(rb * 64, (rb + 1) * 64)
            for g in range(4):
                cols = slice(g * 128, (g + 1) * 128)
                d = _nn(pq[rows, cols], zb[g]) + 1e-6
                pp[rb * 32:(rb + 1) * 32, cols] = _pk(pq[rows, cols] * pl.reciprocal(d, approx=True))

        def den_vpu(rb):
            lane = lax.broadcasted_iota(jnp.int32, (16, 128), 1)
            for v in range(rb * 4, rb * 4 + 4):
                p = pq[v * 16:v * 16 + 16, :] * zrow[...]
                t = ((p[:, 0:128] + p[:, 128:256]) + p[:, 256:384]) + p[:, 384:512]
                t = t + jnp.take_along_axis(t, lane ^ 2, axis=1)
                t = t + jnp.take_along_axis(t, lane ^ 1, axis=1)
                r = pl.reciprocal(t + 1e-6, approx=True)
                pp[v * 8:v * 8 + 8, :] = _pk(pq[v * 16:v * 16 + 16, :] * jnp.concatenate([r] * 4, axis=1))

        def out(rb, g):
            m = mp[g, 0:D // 2, :] if rb < QOLD else perm_rows(mp.at[g])
            r = _nn(_bf(pp[rb * 32:(rb + 1) * 32, :]), _bf(m))
            if g % 2 == 0:
                st["r"] = r
            else:
                sta[rb * 64:(rb + 1) * 64, (g - 1) * 128:(g + 1) * 128] = jnp.concatenate(
                    [st["r"], r], axis=1).astype(BF16)

        res = []
        for t in range(rb0 - 2, rb1):
            step = []
            ov = 60 if t + 1 >= q0 else 28
            if q0 <= t + 2 < rb1:
                step += q_pieces(t + 2, t + 3)
            if rb0 <= t:
                step += [(functools.partial(out, t, g), 64, ov) for g in (0, 1)]
            if rb0 <= t + 1 < rb1:
                step.append((functools.partial(den_mxu, t + 1), 64, 80) if t + 1 < QOLD
                            else (functools.partial(den_vpu, t + 1), 0, 128))
            if rb0 <= t:
                step += [(functools.partial(out, t, g), 64, ov) for g in (2, 3)]
            res.append(step)

        def seg(a, b):
            return [p for step in res[a - rb0 + 2:b - rb0 + 2] for p in step]
        return seg

    prm_hbm = (are_hbm, aim_hbm, bre_hbm, bim_hbm, cre_hbm, cim_hbm)

    def prm_rest(i):
        return prm_hbm[i].at[R0:D], prm.at[i, R0:D]

    srcs = {"ldt": (ldt_hbm, ldt)}
    srcs.update({"a%d" % i: (prm_hbm[i].at[0:R0], prm.at[i, 0:R0]) for i in range(6)})
    srcs.update({
        "wq": (w_hbm.at[:, 0:D], wb.at[:, 0:D]),
        "x0": (x_hbm.at[0:X0], xb.at[0:X0]),
        "dsk": (dsk_hbm, dsk),
        "p0": prm_rest(0),
        "p1": prm_rest(1),
        "wk": (w_hbm.at[:, D:2 * D], wb.at[:, D:2 * D]),
        "p2": prm_rest(2),
        "p3": prm_rest(3),
        "p4": prm_rest(4),
        "p5": prm_rest(5),
        "x1": (x_hbm.at[X0:X1], xb.at[X0:X1]),
        "fi": (fi_hbm, fi),
        "fk": (fk_hbm, fk),
        "ua": (u_hbm.at[:, 0:256], ub.at[:, 0:256]),
        "x2": (x_hbm.at[X1:S], xb.at[X1:S]),
        "ub": (u_hbm.at[:, 256:D], ub.at[:, 256:D]),
        "wv": (w_hbm.at[:, 2 * D:3 * D], wb.at[:, 2 * D:3 * D]),
        "wo": (wo_hbm, wob),
    })
    cin = {k: pltpu.make_async_copy(a, b, sem_in.at[i]) for i, (k, (a, b)) in enumerate(srcs.items())}
    for c in cin.values():
        c.start()
    couts = []

    def wait(*names):
        for n in names:
            cin[n].wait()

    def out_copy(i, kind, a, b):
        if kind == "a":
            return pltpu.make_async_copy(sta.at[a * 64:b * 64], o_hbm.at[a * 64:b * 64, 0:D], sem_out.at[i])
        c0 = D + kind * 128
        return pltpu.make_async_copy(stb.at[kind, a * 128:b * 128],
                                     o_hbm.at[a * 128:b * 128, c0:c0 + 128], sem_out.at[i])

    def store(*box):
        out_copy(len(couts), *box).start()
        couts.append(box)

    q0, q1 = X0 // 64, X1 // 64
    p0, p1 = X0 // 128, X1 // 128
    qe = q_pieces(q1, q1 + 3)
    mid1, mid2, midz = mid_pieces()
    gps = g_pieces()
    gs = []
    for fb in range(8):
        blk = gps[fb * 16:(fb + 1) * 16]
        if fb:
            blk = blk[:4] + [mid1[fb - 1]] + blk[4:9] + [mid2[fb - 1]] + blk[9:]
        gs += blk
    kds = [kdft_pieces(j, 20 if j >= 2 else 0) for j in range(4)]
    uds = [udft_pieces(j) for j in range(4)]
    cv = [[(p, 0, 4) for p in range(32)],
          [(p, 0, 4) for p in range(32, 48)],
          [(p, 0, 3) for p in range(48, 64)] + [(p, 3, 4) for p in range(48, C3)],
          [(p, 3, 4) for p in range(C3, 64)]]
    oseg = o_stream(0, O3, q1 + 3)
    oseg2 = o_stream(O3, 32, O3)

    main3 = uds[0][:8] + [(k0_all, 8, 0)] + uds[0][8:] + kds[0] + uds[1][:10] + kds[1] + uds[1][10:]
    blk3 = main3[:1] + _merge(main3[1:-3], kgen_pieces(G0, 64)) + main3[-3:]
    ql = q_pieces(q0 - 1, q0)
    blk4 = (uds[2][:2] + _merge(kt_pieces(p1, 16), uds[2][2:13]) + uds[2][13:]
            + _merge(gs[:GS], midz + kds[2] + kds[3], uds[3]))
    blk5 = _merge(gs[GS:] + qe[:4] + [mid1[7]] + oseg(-2, 0) + qe[4:8] + [mid2[7]] + qe[8:] + oseg(0, O1),
                  inv_pieces(0) + inv_pieces(1))
    blk5 = [(f, c, v + (50 if 8 <= i < 32 else 0)) for i, (f, c, v) in enumerate(blk5)]
    last = oseg2(O4, 32)
    ta = oseg2(O3, O4)
    blk8 = oseg2(O3 - 2, O3) + ta[:-5] + inv_pieces(3)[6:] + [p for p in last if p[1] == 0] + ta[-5:]
    blk9 = [p for p in last if p[1] != 0]

    steps = [
        (lambda: wait("ldt"), setup_dt_first),
        (lambda: wait("a0", "a1", "a2", "a3", "a4", "a5"), early_prep),
        (early_exact, lambda: _emit(kgen_pieces(0, G0))),
        (lambda: wait("wq", "x0", "dsk"),
         lambda: (setup_dt_rest(), wq_perm_a(), _emit(q_pieces(0, q0 - 1)))),
        (lambda: wait("p0", "p1", "wk"),
         lambda: (wk_transpose(), range_check(0, R0, D),
                  _emit(ql[:3] + kt_pieces(0, p0, True), stage1(), (32 - G0 // 2) * 90, tail=130))),
        (lambda: (stage1_exact(), wait("p2", "p3", "p4", "p5", "x1")),
         lambda: (wq_perm_b(),
                  _emit(ql[3:] + kt_pieces(p0, p1) + q_pieces(q0, q1), stage2_fill(G0 // 2, 32), (32 - G0 // 2) * 164))),
        (lambda: wait("fi", "fk", "ua"), lambda: (setup_g(), _emit(blk3))),
        (lambda: wait("x2", "ub", "wv", "wo"), lambda: _emit(blk4, conv(cv[0]), conv_ops(cv[0]), 3.6)),
        (None, lambda: _emit(blk5, conv(cv[1]), conv_ops(cv[1]), 3.7)),
        (lambda: (store(0, 0, 16), store(1, 0, 16), store("a", 0, O1)),
         lambda: _emit(_merge(oseg(O1, O2), inv_pieces(2)), conv(cv[2]), conv_ops(cv[2]), 3.5)),
        (lambda: (store(2, 0, 16), store("a", O1, O2)),
         lambda: _emit(_merge(oseg(O2, O3), inv_pieces(3)[:6]), conv(cv[3]), conv_ops(cv[3]), 3.4)),
        (lambda: (store(3, 0, 12), store("a", O2, O3)), lambda: _emit(blk8)),
        (lambda: (store(3, 12, 16), store("a", O3, O4)), lambda: _emit(blk9)),
        (lambda: store("a", O4, 32), None),
    ]

    def outer(i, c):
        packed.clear()
        couts.clear()
        for k in range(len(steps) - 1):
            @pl.when(i + k == k)
            def _():
                steps[k][1]()
                if steps[k + 1][0] is not None:
                    steps[k + 1][0]()
        return c

    steps[0][0]()
    lax.fori_loop(0, 2, outer, 0)
    for i, box in enumerate(couts):
        out_copy(i, *box).wait()


@jax.jit
def pallas_concat_heads__linear_attn_block__ssm_conv_s4__prompt_kernel(
    A_x, A_wqkv, A_wo, B_u, B_A_re, B_A_im, B_B_re, B_B_im, B_C_re, B_C_im, B_log_dt, B_Dskip,
):
    fk, fi = _tables()
    V = pltpu.VMEM
    params = dict(vmem_limit_bytes=110 * 2**20)
    if hasattr(pltpu.CompilerParams, "disable_semaphore_checks"):
        params["disable_semaphore_checks"] = True
    out = pl.pallas_call(
        _kernel,
        out_shape=jax.ShapeDtypeStruct((S, 2 * D), BF16),
        in_specs=[pl.BlockSpec(memory_space=pl.ANY)] * 14,
        out_specs=pl.BlockSpec(memory_space=pl.ANY),
        scratch_shapes=[
            V((S // 2, D), U32),
            V((D, 3 * D), BF16),
            V((D, D), BF16),
            V((S // 2, D), U32),
            V((6, D, 128), BF16),
            V((D,), BF16),
            V((D,), BF16),
            V((S, D), BF16),
            V((S, D), BF16),
            V((FK_ROWS // 2, 128), U32),
            V((136, 128), F32),
            V((S, D), BF16),
            V((4, S, 128), BF16),
            V((2, D, 128), F32),
            pltpu.SMEM((2,), jnp.int32),
            V((D, 128), F32),
            V((8, 128, 128), F32),
            V((14, 2 * D + 8, 128), F32),
            V((D, 128), F32),
            V((5, D // 2, 128), U32),
            V((4, 2, 16, 128), F32),
            V((8, D), F32),
            V((4, 3, 16, 128, 128), F32),
            V((4, 3, 16, 128, 128), F32),
            V((4, 2, 16, 128, 128), F32),
            V((D // 2, D), U32),
            V((D // 2, S), U32),
            V((D, 128), F32),
            V((D // 2, D), U32),
            V((4, D // 2 + 8, 128), U32),
            V((4, 128, 128), F32),
            V((S, D), F32),
            V((S // 2, D), U32),
            V((4, D // 2 + 8, 128), U32),
            V((D // 2, D), U32),
            V((D // 2 + 8, 128), U32),
            V((16, D), F32),
            V((4, 12, 144, 128), F32),
            V((2, 128, 128), F32),
            pltpu.SemaphoreType.DMA((25,)),
            pltpu.SemaphoreType.DMA((10,)),
        ],
        compiler_params=pltpu.CompilerParams(**params),
    )(A_x.reshape(S, D), A_wqkv, A_wo, B_u.reshape(S, D), B_A_re, B_A_im, B_B_re, B_B_im, B_C_re, B_C_im,
      B_log_dt, B_Dskip, jnp.asarray(fk), jnp.asarray(fi))
    return out.reshape(1, S, 2 * D)
```

```python
import functools

import numpy as np
import jax
import jax.numpy as jnp
from jax import lax
import jax.experimental.pallas as pl
import jax.experimental.pallas.tpu as pltpu

S = 2048
D = 512
F32 = jnp.float32
BF16 = jnp.bfloat16
U32 = jnp.uint32

_BASE = np.array([[1, 5], [2, 6], [3, 7], [4, 8], [258, 262], [260, 264],
                  [516, 520], [772, 776], [1032, 1288], [1544, 1800]])
_TILE_OF_CHUNK = [0, 1, 2, 2, 3, 3, 3, 3] + [4] * 8

FK_OFF = [0, 256, 528, 784] + [1056 + 144 * k for k in range(4)] + [1632 + 80 * k for k in range(8)]
FK_FU = 1632 + 640
FK_ROWS = FK_FU + 256

X0, X1 = 384, 896
QOLD = X0 // 64
G0 = 12
R0 = 8 * G0
O1, O2, O3, O4 = 15, 24, 29, 31
GS = 120
C3 = 51

B_W1, B_W2, B_W8C, B_W256, B_W512, B_E0, B_N0 = range(7)
_SC_LIMIT = 8192.0


def _bf16_bits(v):
    u = np.ascontiguousarray(v, np.float32).view(np.uint32)
    return ((u + 0x7FFF + ((u >> 16) & 1)) >> 16).astype(np.uint32)


def _pack_rows(v):
    b = _bf16_bits(v)
    return b[0::2] | (b[1::2] << 16)


@functools.lru_cache(maxsize=None)
def _tables():
    lr = (_bf16_bits(np.arange(S)) << 16).view(np.float32).astype(np.int64)
    val = np.zeros((5, 128), np.int64)
    for lam in range(128):
        mu, tau = 15 - (lam >> 3), lam & 7
        e, x = tau >> 1, tau & 1
        for h in range(2):
            val[h, lam] = _BASE[e, x ^ h] + 8 * (mu + 16 * h)
        hp, ab, h = tau >> 2, (tau >> 1) & 1, tau & 1
        for q in range(3):
            val[2 + q, lam] = _BASE[4 + 2 * q + ab, hp] + 8 * (mu + 16 * h)
    om = 2 * np.pi * (np.arange(128) + 0.25) / 128.0
    phase = np.exp(1j * om * 191.5)

    def stack(z):
        return np.concatenate([p[32 * t:32 * t + 32] for t in range(4) for p in (z.real, z.imag)], axis=0)

    fk = []
    g = np.zeros(128, np.complex128)
    for k in range(4):
        slot = {int(v): i for i, v in enumerate(val[_TILE_OF_CHUNK[k]])}
        m = np.zeros((128, 128), np.complex128)
        for p in range(1, 129):
            lag = 128 * k + p
            v = int(lr[lag])
            z = np.exp(-1j * om * p) * (0.5 if lag == 512 else 1.0)
            if v in slot:
                m[:, slot[v]] += z
            else:
                assert v == 256 and k == 2
                g += z
        if k in (1, 3):
            sel = np.zeros((16, 128))
            sel[:, slot[128 * (k + 1)]] = 1.0
            fk += [stack(m)[:128], sel, stack(m)[128:]]
        else:
            fk.append(stack(m))
    for k in range(4, 16):
        st = 4 if k < 8 else 8
        per = 128 // st
        slot = {int(v): i for i, v in enumerate(val[_TILE_OF_CHUNK[k]])}
        for lag in range(128 * k + 1, min(128 * k + 128, S)):
            m_ = int(lr[lag]) // st
            assert int(lr[lag]) % st == 0 and abs(lag - st * m_) <= (st // 2 if m_ % 2 == 0 else st // 2 - 1)
        od = np.zeros((per, 128), np.complex128)
        ev = np.zeros((per, 128), np.complex128)
        edge = np.zeros((16, 128))
        for m_ in range(per + 1):
            v = 128 * k + st * m_
            if v not in slot:
                assert m_ == 0 and k in (4, 8)
                continue
            z = np.exp(-1j * om[:per] * st * m_)
            if m_ % 2:
                od[:, slot[v]] = z
            else:
                ev[:, slot[v]] = z * (0.5 if m_ in (0, per) else 1.0)
            if m_ in (0, per):
                edge[8 * (m_ // per):8 * (m_ // per) + 8, slot[v]] = 1.0
        fk += [edge, od.real, od.imag, ev.real, ev.imag]
    fk.append(stack(np.exp(-1j * om[:, None] * np.arange(128)[None, :]) * phase[:, None]))
    fk = np.concatenate(fk, axis=0)
    assert fk.shape[0] == FK_ROWS
    tabs = [g.real, g.imag]
    for h in (2, 4):
        tabs += [sum(np.cos(om * p) for p in range(1 - h, h)), sum(np.cos(om * p) for p in range(-h, h + 1)),
                 -sum(np.sin(om * p) for p in range(1, h + 1))]
    jj = np.arange(64)[:, None] - 63.5
    finv = np.concatenate([np.cos(om[None, :] * jj) / 128.0, -np.sin(om[None, :] * jj) / 128.0,
                           np.stack(tabs)], axis=0)
    return _pack_rows(fk), finv.astype(np.float32)


def _cmul(a, b):
    return a[0] * b[0] - a[1] * b[1], a[0] * b[1] + a[1] * b[0]


def _csq(a):
    return a[0] * a[0] - a[1] * a[1], (a[0] + a[0]) * a[1]


def _phi(t):
    return jnp.where(t > 0, t + 1.0, jnp.exp(t)) + 1e-6


def _nt(a, b):
    return lax.dot_general(a, b, (((1,), (1,)), ((), ())), preferred_element_type=F32)


def _nn(a, b):
    return jnp.dot(a, b, preferred_element_type=F32)


def _bf(v):
    return pltpu.bitcast(v, BF16)


def _pk(v):
    return pltpu.bitcast(v.astype(BF16), U32)


def _sincos(x):
    t = x * 0.6366197723675814 + 12582912.0
    n = pltpu.bitcast(t, jnp.int32) - 0x4B400000
    k = n.astype(F32)
    r = ((x - k * 1.5703125) - k * 4.837512969970703125e-4) - k * 7.54978995489188216e-8
    r2 = r * r
    sn = r + r * r2 * (-1.6666654611e-1 + r2 * (8.3321608736e-3 + r2 * -1.9515295891e-4))
    cs = 1.0 + r2 * (-0.5 + r2 * (4.166664568298827e-2 + r2 * (-1.388731625493765e-3 + r2 * 2.443315711809948e-5)))
    swap = (n & 1) == 1
    s_, c_ = jnp.where(swap, cs, sn), jnp.where(swap, sn, cs)
    ssign = (n & 2) << 30
    csign = ((n + 1) & 2) << 30
    s_ = pltpu.bitcast(pltpu.bitcast(s_, jnp.int32) ^ ssign, F32)
    c_ = pltpu.bitcast(pltpu.bitcast(c_, jnp.int32) ^ csign, F32)
    return s_, c_


def _emit(pieces, filler=None, fill_total=0, cap=3.0, tail=100):
    filler = iter(()) if filler is None else filler
    room = [max(cap * c - v, 0.0) for _, c, v in pieces]
    tot = sum(room[:-1]) or 1.0
    done, target = 0.0, 0.0
    for (fn, _, _), r in zip(pieces, room):
        fn()
        target += max(fill_total - tail, 0) * r / tot
        while done < target - 8:
            n = next(filler, None)
            if n is None:
                break
            done += n
    for _ in filler:
        pass


def _merge(*lists):
    tot = [sum(p[1] for p in l) or 1.0 for l in lists]
    pos = [0] * len(lists)
    acc = [0.0] * len(lists)
    out = []
    while True:
        best = None
        for i, l in enumerate(lists):
            if pos[i] < len(l):
                key = (acc[i] + 0.5 * l[pos[i]][1]) / tot[i]
                if best is None or key < best[0]:
                    best = (key, i)
        if best is None:
            return out
        i = best[1]
        out.append(lists[i][pos[i]])
        acc[i] += lists[i][pos[i]][1]
        pos[i] += 1


def _group(pieces, n):
    out = []
    for i in range(0, len(pieces), n):
        grp = pieces[i:i + n]

        def run(grp=grp):
            for f, _, _ in grp:
                f()
        out.append((run, sum(p[1] for p in grp), sum(p[2] for p in grp)))
    return out


def _reim(r):
    n = r.shape[0] // 64
    return (jnp.concatenate([r[64 * t:64 * t + 32] for t in range(n)], axis=0),
            jnp.concatenate([r[64 * t + 32:64 * t + 64] for t in range(n)], axis=0))


def _kernel(x_hbm, w_hbm, wo_hbm, u_hbm, are_hbm, aim_hbm, bre_hbm, bim_hbm, cre_hbm, cim_hbm,
            ldt_hbm, dsk_hbm, fk_hbm, fi_hbm, o_hbm,
            xp, wb, wob, up, prm, ldt, dsk, xb, ub, fk, fi, sta, stb, w1s, flag,
            dtb, gb, base, cr, wt, bv, k0s, kw, u3, y, wkt, pkt, zacc, gp, mp, zb, pq, pp,
            wqt, wqp, zpk, zrow, kf, zc, sem_in, sem_out):

    def iotas():
        return (lax.broadcasted_iota(jnp.int32, (8, 128), 0), lax.broadcasted_iota(jnp.int32, (8, 128), 1))

    packed = set()

    def tile(kind, r0, n, cols=slice(None)):
        src, dst = (xb, xp) if kind == "x" else (ub, up)
        parts = []
        for r in range(r0, r0 + n, 64):
            key = (kind, r, cols.start)
            if key in packed:
                parts.append(_bf(dst[r // 2:r // 2 + 32, cols]))
            else:
                packed.add(key)
                v = src[r:r + 64, cols]
                dst[r // 2:r // 2 + 32, cols] = pltpu.bitcast(v, U32)
                parts.append(v)
        return parts[0] if len(parts) == 1 else jnp.concatenate(parts, axis=0)

    def dt_row():
        return jnp.exp(ldt[...].reshape(1, D).astype(F32)).astype(BF16).astype(F32)

    def setup_dt_first():
        sub, _ = iotas()
        b = jnp.broadcast_to(dt_row()[:, 0:128], (8, 128))
        for v in range(16):
            dtb[v * 8:v * 8 + 8, :] = jnp.take_along_axis(b, sub + 8 * v, axis=1)

    def setup_dt_rest():
        row = dt_row()
        for j in range(1, 4):
            dtb[j * 128:(j + 1) * 128, :] = jnp.broadcast_to(row[:, j * 128:(j + 1) * 128], (128, 128)).T

    def setup_g():
        for i in range(8):
            gb[i] = jnp.broadcast_to(fi[128 + i:129 + i, :], (128, 128)).T

    def perm_rows(ref):
        return jnp.concatenate([ref[pl.ds(t, 64, stride=4), :] for t in range(4)], axis=0)

    def wq_perm_a():
        for a in range(4):
            for b in range(4):
                t = wb[a * 128:(a + 1) * 128, b * 128:(b + 1) * 128].T
                wqt[a, b * 64:(b + 1) * 64, :] = pltpu.bitcast(t, U32)

    def wq_perm_b():
        for b in range(4):
            for a in range(4):
                t = _bf(wqt[a, pl.ds(b, 64, stride=4), :]).T
                wqp[a * 64:(a + 1) * 64, b * 128:(b + 1) * 128] = pltpu.bitcast(t, U32)

    def wk_transpose():
        for b in range(4):
            for a in range(4):
                t = wb[a * 128:(a + 1) * 128, D + b * 128:D + (b + 1) * 128].T
                wkt[b * 64:(b + 1) * 64, a * 128:(a + 1) * 128] = pltpu.bitcast(t, U32)

    def w1_rows(r0, exact):
        rows = pl.ds(r0, 16)
        dt = dtb[rows, :]
        ar = dt * prm[0, rows, :].astype(F32)
        ai = dt * prm[1, rows, :].astype(F32)
        mag = jnp.exp(ar)
        sn, cs = (jnp.sin(ai), jnp.cos(ai)) if exact else _sincos(ai)
        w1s[0, rows, :] = mag * cs
        w1s[1, rows, :] = mag * sn

    def range_check(i, r0, r1):
        m = jnp.max(jnp.abs(prm[1, r0:r1, :].astype(F32)).reshape((r1 - r0) // 8, 8, 128), axis=0)
        dmax = jnp.max(dtb[r0:r1, :].reshape((r1 - r0) // 8, 8, 128), axis=0)
        bound = jnp.max(m) * jnp.max(dmax)
        flag[i] = jnp.where(bound <= _SC_LIMIT, 0, 1).astype(jnp.int32)

    def stage1():
        for r in range(G0 // 2, 32):
            w1_rows(r * 16, False)
            yield 90

    def stage1_exact():
        @pl.when(flag[0] != 0)
        def _():
            def body(r, c):
                w1_rows(pl.multiple_of(r * 16, 16), True)
                return c
            lax.fori_loop(G0 // 2, 32, body, 0)

    def stage2(r):
        r0 = r * 16 if isinstance(r, int) else pl.multiple_of(r * 16, 16)
        rows = pl.ds(r0, 16)
        dt = dtb[rows, :]
        w1 = (w1s[0, rows, :], w1s[1, rows, :])
        db = (dt * prm[2, rows, :].astype(F32), dt * prm[3, rows, :].astype(F32))
        c = _cmul((prm[4, rows, :].astype(F32), prm[5, rows, :].astype(F32)), db)
        cr[rows, :] = c[0]
        lo = (lax.broadcasted_iota(jnp.int32, (16, 128), 0) & 4) == 0

        def put(i, v0, v1=None):
            for t in range(2):
                ev, od = (v0[t], v0[t]) if v1 is None else (jnp.where(lo, v0[t], v1[t]), jnp.where(lo, v1[t], v0[t]))
                base[2 * i + t, pl.ds(2 * r0, 16, stride=2), :] = ev
                base[2 * i + t, pl.ds(2 * r0 + 1, 16, stride=2), :] = od
        put(B_W1, w1)
        w2 = _csq(w1)
        put(B_W2, w2)
        w4 = _csq(w2)
        cw1 = _cmul(c, w1)
        put(B_N0, cw1, _cmul(cw1, w4))
        yield 80
        w8 = _csq(w4)
        put(B_W8C, (w8[0], -w8[1]))
        w128 = _csq(_csq(_csq(_csq(w8))))
        put(B_E0, (jnp.ones((16, 128), F32), jnp.zeros((16, 128), F32)), (w128[0], -w128[1]))
        w256 = _csq(w128)
        put(B_W256, w256)
        put(B_W512, _csq(w256))
        yield 84

    def stage2_fill(r0, r1):
        for r in range(r0, r1):
            yield from stage2(r)

    def early_prep():
        range_check(1, 0, R0)
        for r in range(G0 // 2):
            w1_rows(r * 16, False)
        for _ in stage2_fill(0, G0 // 2):
            pass

    def early_exact():
        @pl.when(flag[1] != 0)
        def _():
            def body(r, c):
                w1_rows(pl.multiple_of(r * 16, 16), True)
                for _ in stage2(r):
                    pass
                return c
            lax.fori_loop(0, G0 // 2, body, 0)

    def kgen_pieces(g0, g1):
        st = {}

        def group(gi):
            sub, lane = iotas()
            odd = (sub & 1) == 1
            rows = slice(gi * 16, gi * 16 + 16)

            def ld(i):
                return base[2 * i, rows, :], base[2 * i + 1, rows, :]
            w8c = ld(B_W8C)
            e0 = [ld(B_E0)]
            for _ in range(1, 16):
                e0.append(_cmul(e0[-1], w8c))
            e0 = e0[::-1]
            w1, w2, w256, w512 = ld(B_W1), ld(B_W2), ld(B_W256), ld(B_W512)
            n0 = ld(B_N0)
            n1 = _cmul(n0, w1)
            n2 = _cmul(n0, w2)
            n3 = _cmul(n1, w2)
            n4 = _cmul(n1, w256)
            n5 = _cmul(n3, w256)
            n6 = _cmul(n5, w256)
            n7 = _cmul(n6, w256)
            t = tuple(jnp.concatenate([jnp.where(odd, n7[c][0:8], pltpu.roll(n6[c][0:8], 7, 0)),
                                       jnp.where(odd, pltpu.roll(n6[c][8:16], 1, 0), n7[c][8:16])], axis=0)
                      for c in range(2))
            n8 = _cmul(t, w512)
            n9 = _cmul(n8, w512)
            e1 = [n0, n1, n2, n3, n4, n5, n6, n7, n8, n9]

            def operands(es):
                v = jnp.concatenate([jnp.concatenate([e[0] for e in es], axis=0),
                                     jnp.concatenate([e[1] for e in es], axis=0)], axis=1)
                v = v.reshape(len(es), 2, 8, 256)
                return [v[:, g].reshape(len(es) * 8, 256) for g in range(2)]
            o = []
            for lhs, rhs in zip(operands(e1), operands(e0)):
                r = _nt(lhs, rhs)
                o.append([r[8 * i:8 * i + 8, :] for i in range(10)])

            emask = ((sub >> 1) - (lane >> 1)) & 3
            ea, xa = (lane >> 1) & 3, lane & 1
            lidx_a = (lane & 120) | ((((sub >> 1) - ea) & 3) << 1) | (xa ^ (sub & 1))
            sidx_a = ((((sub & 3) + ea) & 3) << 1) | (xa ^ (sub >> 2))
            hp, ab, hh = (lane >> 2) & 1, (lane >> 1) & 1, lane & 1
            gg = hp ^ (sub & 1)
            lidx_b = (lane & 120) | ((((sub >> 1) - (2 * gg + ab)) & 3) << 1) | (hh ^ gg)
            g2 = sub >> 2
            sidx_b = ((((sub & 3) + 2 * g2 + ab) & 3) << 1) | (hp ^ g2)

            def compact(srcs, lidx, sidx):
                s = srcs[0]
                for e in range(1, 4):
                    s = jnp.where(emask == e, pltpu.roll(srcs[e], 2 * e, 0), s)
                s = jnp.take_along_axis(s, lidx, axis=1)
                return jnp.take_along_axis(s, sidx, axis=0)

            a2 = [compact(o[g][0:4], lidx_a, sidx_a) for g in range(2)]
            lo = sub < 4
            res = [jnp.where(lo, a2[0], a2[1]), pltpu.roll(jnp.where(lo, a2[1], a2[0]), 4, 0)]
            for q in range(3):
                res.append(compact(o[0][4 + 2 * q:6 + 2 * q] + o[1][4 + 2 * q:6 + 2 * q], lidx_b, sidx_b))
            if gi % 2 == 0:
                st["r"] = res
            else:
                for q in range(5):
                    wt[q, (gi // 2) * 8:(gi // 2) * 8 + 8, :] = _pk(jnp.concatenate([st["r"][q], res[q]], axis=0))

        return [(functools.partial(group, gi), 80, 360) for gi in range(g0, g1)]

    def k0_all():
        k0s[...] = _nt(jnp.ones((8, 128), F32), cr[...]) + dsk[...].reshape(1, D).astype(F32)

    def kdft_pieces(j, extra):
        def wtile(k):
            return _bf(wt[_TILE_OF_CHUNK[k], j * 64:(j + 1) * 64, :])

        def near(k, hf):
            o = FK_OFF[k] // 2 + hf * 64
            if k in (1, 3):
                r = _nt(_bf(fk[o:o + 72, :]), wtile(k))
                bv[j, k // 2, hf * 8:hf * 8 + 8, :] = r[128:136] if hf == 0 else r[0:8]
                r = r[:128] if hf == 0 else r[16:]
            else:
                r = _nt(_bf(fk[o:o + 64, :]), wtile(k))
            rr, ri = _reim(r)
            rows = slice(hf * 64, hf * 64 + 64)
            if k == 0:
                rr = rr + jnp.concatenate([k0s[:, j * 128:(j + 1) * 128]] * 8, axis=0)
            elif k == 2:
                bval = jnp.concatenate([bv[j, 0]] * 4, axis=0)
                rr = rr + gb[0, rows, :] * bval
                ri = ri + gb[1, rows, :] * bval
            kw[j, 0, k, rows, :] = rr
            kw[j, 1, k, rows, :] = ri
            kw[j, 2, k, rows, :] = rr + ri

        def far(k):
            per = 32 if k < 8 else 16
            n = 16 + 4 * per
            o = FK_OFF[k] // 2
            r = _nt(_bf(fk[o:o + n // 2, :]), wtile(k))
            if k in (4, 8):
                e0 = 16 + 2 * per
                v0 = bv[j, 1] if k == 4 else jnp.concatenate([kf[j, 3, 8:16, :]] * 2, axis=0)
                r = jnp.concatenate([v0[0:8], r[8:e0], r[e0:e0 + per] + 0.5 * jnp.concatenate([v0] * (per // 16), axis=0),
                                     r[e0 + per:]], axis=0)
            kf[j, k - 4, 0:n, :] = r

        def nears(ks, v):
            return _group([(functools.partial(near, k, hf), 32, v + extra) for k in ks for hf in range(2)], 4)

        def fars(ks):
            return _group([(functools.partial(far, k), 36 if k < 8 else 20, extra) for k in ks], 4)
        return (nears((1, 3), 8) + fars((12, 13, 14, 15)) + fars((7, 6, 5, 4))
                + nears((0, 2), 28) + fars((9, 10, 11, 8)))

    def udft_pieces(j):
        def piece(ib, qf):
            o = FK_FU // 2 + qf * 32
            w = jnp.concatenate([tile("u", i * 128, 128, slice(j * 128, (j + 1) * 128))
                                 for i in range(ib * 4, ib * 4 + 4)], axis=1)
            r = _nn(_bf(fk[o:o + 32, :]), w)
            rows = slice(qf * 32, qf * 32 + 32)
            for t in range(4):
                rr, ri = r[:32, t * 128:(t + 1) * 128], r[32:, t * 128:(t + 1) * 128]
                u3[j, 0, ib * 4 + t, rows, :] = rr
                u3[j, 1, ib * 4 + t, rows, :] = ri
                u3[j, 2, ib * 4 + t, rows, :] = rr + ri
        return [(functools.partial(piece, ib, qf), 64, 16) for ib in range(4) for qf in range(4)]

    def conv_ops(items):
        return sum((68, 204, 300, 396)[ib] for _, i0, i1 in items for ib in range(i0, i1))

    def conv(items):
        for pos, ib0, ib1 in items:
            j, p = divmod(pos, 16)
            rs = slice(p * 8, p * 8 + 8)
            prev = None if ib0 == 0 else (zc[0:1, rs, :], zc[1:2, rs, :])
            for ib in range(ib0, ib1):
                if ib > 0:
                    t0 = 2 if ib == 1 else 5
                    d_od, d_ev, sh = (gb[t0 + t:t0 + t + 1, rs, :] for t in range(3))
                    per = 32 if ib == 1 else 16
                    h = 16 + (8 * p) % per
                    left = sh * kf[j, 4 * ib - 4:4 * ib - 3, 0:8, :]
                    for k in range(4 * ib, 4 * ib + 4, 2):
                        o_r, o_i, e_r, e_i = (kf[j, k - 4:k - 2, per * t + h:per * t + h + 8, :] for t in range(4))
                        right = sh * kf[j, k - 4:k - 2, 8:16, :]
                        rr = d_od * o_r + d_ev * e_r - right
                        ri = d_od * o_i + d_ev * e_i + jnp.concatenate([left, right[:1]], axis=0)
                        left = right[1:]
                        kw[j, 0, k:k + 2, rs, :] = rr
                        kw[j, 1, k:k + 2, rs, :] = ri
                        kw[j, 2, k:k + 2, rs, :] = rr + ri
                        yield 20
                a = zr = None
                for c in range(3):
                    acc = None
                    for k in range(4 * ib + 1):
                        pr = u3[j, c, 4 * ib - k:4 * ib - k + 4, rs, :] * kw[j, c, k:k + 1, rs, :]
                        if acc is None:
                            acc = pr - a if c == 2 else pr
                        else:
                            acc = acc + pr
                        if k % 4 == 3:
                            yield 32
                    for d in range(1, 4):
                        pr = u3[j, c, 0:4 - d, rs, :] * kw[j, c, 4 * ib + d:4 * ib + d + 1, rs, :]
                        acc = jnp.concatenate([acc[:d], acc[d:] + pr], axis=0)
                    n = 20
                    if c == 0:
                        a = acc
                    elif c == 1:
                        zr = a - acc
                        a = a + acc
                    else:
                        if prev is None:
                            yr = jnp.concatenate([acc[:1], zr[:3] + acc[1:]], axis=0)
                            yi = jnp.concatenate([-zr[:1], acc[:3] - zr[1:]], axis=0)
                        else:
                            yr = jnp.concatenate([prev[0], zr[:3]], axis=0) + acc
                            yi = jnp.concatenate([prev[1], acc[:3]], axis=0) - zr
                        y[j, 0, ib * 4:ib * 4 + 4, rs, :] = yr
                        y[j, 1, ib * 4:ib * 4 + 4, rs, :] = yi
                        prev = (zr[3:], acc[3:])
                        n += 8
                        if ib == ib1 - 1 and ib1 < 4:
                            zc[0:1, rs, :], zc[1:2, rs, :] = prev
                    yield n

    def inv_pieces(j):
        def piece(i):
            sub, _ = iotas()
            s = _nn(fi[0:64, :], y[j, 0, i])
            a = _nn(fi[64:128, :], y[j, 1, i])
            lo = s + a
            hi = s - a
            hi = jnp.concatenate(
                [jnp.take_along_axis(hi[8 * v:8 * v + 8], 7 - sub, axis=0) for v in range(7, -1, -1)], axis=0)
            stb[j, i * 128:(i + 1) * 128, :] = jnp.concatenate([lo, hi], axis=0).astype(BF16)
        return _group([(functools.partial(piece, i), 32, 32) for i in range(16)], 2)

    def kt_pieces(pb0, pb1, fb_outer=False):
        def piece(fb, pb):
            pk = _phi(_nt(_bf(wkt[fb * 64:(fb + 1) * 64, :]), tile("x", pb * 128, 128)))
            pkt[fb * 64:(fb + 1) * 64, pb * 128:(pb + 1) * 128] = _pk(pk)
            rows = slice(fb * 128, (fb + 1) * 128)
            if pb == 0:
                zacc[rows, :] = pk
            else:
                zacc[rows, :] += pk
        idx = [(fb, pb) for pb in range(pb0, pb1) for fb in range(4)]
        if fb_outer:
            idx.sort()
        return [(functools.partial(piece, fb, pb), 128, 230) for fb, pb in idx]

    def g_pieces():
        st = {}

        def piece(fb, cb, kb):
            r = _nn(_bf(pkt[fb * 32:(fb + 1) * 32, kb * 512:(kb + 1) * 512]),
                    _bf(xp[kb * 256:(kb + 1) * 256, cb * 128:(cb + 1) * 128]))
            if kb > 0:
                r = r + st["acc"]
            if kb == 3:
                gp[fb * 32:(fb + 1) * 32, cb * 128:(cb + 1) * 128] = _pk(r)
            else:
                st["acc"] = r
        return [(functools.partial(piece, fb, cb, kb), 64, 32)
                for fb in range(8) for cb in range(4) for kb in range(4)]

    def mid_pieces():
        st = {}

        def bd():
            r128 = lax.broadcasted_iota(jnp.int32, (128, 128), 0)
            c128 = lax.broadcasted_iota(jnp.int32, (128, 128), 1)
            return (r128 >> 4) == (c128 >> 4)

        def kv(fb):
            g = fb // 2
            r = _nn(_bf(gp[fb * 32:(fb + 1) * 32, :]), wb[:, 2 * D + g * 128:2 * D + (g + 1) * 128])
            st[fb] = jnp.where(bd()[(fb % 2) * 64:(fb % 2) * 64 + 64], r, 0.0).astype(BF16)

        def mm(fb):
            g = fb // 2
            m = _pk(_nn(st[fb], wob[g * 128:(g + 1) * 128, :]))
            for c in range(4):
                mp[c, fb * 32:(fb + 1) * 32, :] = m[:, c * 128:(c + 1) * 128]

        def zz():
            for g in range(4):
                za = zacc[g * 128:(g + 1) * 128, :]
                z = jnp.sum(za, axis=1, keepdims=True)
                zb[g] = jnp.where(bd(), jnp.broadcast_to(z, (128, 128)), 0.0)
                zpk[g * 64:(g + 1) * 64, :] = _pk(za)
            zrow[...] = _nt(jnp.ones((16, 128), BF16), _bf(perm_rows(zpk)))
        return ([(functools.partial(kv, fb), 64, 40) for fb in range(8)],
                [(functools.partial(mm, fb), 64, 16) for fb in range(8)], [(zz, 64, 120)])

    def q_pieces(rb0, rb1):
        def piece(rb, g):
            w = wb[:, g * 128:(g + 1) * 128] if rb < QOLD else _bf(wqp[:, g * 128:(g + 1) * 128])
            pq[rb * 64:(rb + 1) * 64, g * 128:(g + 1) * 128] = _phi(_nn(tile("x", rb * 64, 64), w))
        return [(functools.partial(piece, rb, g), 64, 64) for rb in range(rb0, rb1) for g in range(4)]

    def o_stream(rb0, rb1, q0):
        st = {}

        def den_mxu(rb):
            rows = slice(rb * 64, (rb + 1) * 64)
            for g in range(4):
                cols = slice(g * 128, (g + 1) * 128)
                d = _nn(pq[rows, cols], zb[g]) + 1e-6
                pp[rb * 32:(rb + 1) * 32, cols] = _pk(pq[rows, cols] * pl.reciprocal(d, approx=True))

        def den_vpu(rb):
            lane = lax.broadcasted_iota(jnp.int32, (16, 128), 1)
            for v in range(rb * 4, rb * 4 + 4):
                p = pq[v * 16:v * 16 + 16, :] * zrow[...]
                t = ((p[:, 0:128] + p[:, 128:256]) + p[:, 256:384]) + p[:, 384:512]
                t = t + jnp.take_along_axis(t, lane ^ 2, axis=1)
                t = t + jnp.take_along_axis(t, lane ^ 1, axis=1)
                r = pl.reciprocal(t + 1e-6, approx=True)
                pp[v * 8:v * 8 + 8, :] = _pk(pq[v * 16:v * 16 + 16, :] * jnp.concatenate([r] * 4, axis=1))

        def out(rb, g):
            m = mp[g, 0:D // 2, :] if rb < QOLD else perm_rows(mp.at[g])
            r = _nn(_bf(pp[rb * 32:(rb + 1) * 32, :]), _bf(m))
            if g % 2 == 0:
                st["r"] = r
            else:
                sta[rb * 64:(rb + 1) * 64, (g - 1) * 128:(g + 1) * 128] = jnp.concatenate(
                    [st["r"], r], axis=1).astype(BF16)

        res = []
        for t in range(rb0 - 2, rb1):
            step = []
            ov = 60 if t + 1 >= q0 else 28
            if q0 <= t + 2 < rb1:
                step += q_pieces(t + 2, t + 3)
            if rb0 <= t:
                step += [(functools.partial(out, t, g), 64, ov) for g in (0, 1)]
            if rb0 <= t + 1 < rb1:
                step.append((functools.partial(den_mxu, t + 1), 64, 80) if t + 1 < QOLD
                            else (functools.partial(den_vpu, t + 1), 0, 128))
            if rb0 <= t:
                step += [(functools.partial(out, t, g), 64, ov) for g in (2, 3)]
            res.append(step)

        def seg(a, b):
            return [p for step in res[a - rb0 + 2:b - rb0 + 2] for p in step]
        return seg

    prm_hbm = (are_hbm, aim_hbm, bre_hbm, bim_hbm, cre_hbm, cim_hbm)

    def prm_rest(i):
        return prm_hbm[i].at[R0:D], prm.at[i, R0:D]

    srcs = {"ldt": (ldt_hbm, ldt)}
    srcs.update({"a%d" % i: (prm_hbm[i].at[0:R0], prm.at[i, 0:R0]) for i in range(6)})
    srcs.update({
        "wq": (w_hbm.at[:, 0:D], wb.at[:, 0:D]),
        "x0": (x_hbm.at[0:X0], xb.at[0:X0]),
        "dsk": (dsk_hbm, dsk),
        "p0": prm_rest(0),
        "p1": prm_rest(1),
        "wk": (w_hbm.at[:, D:2 * D], wb.at[:, D:2 * D]),
        "p2": prm_rest(2),
        "p3": prm_rest(3),
        "p4": prm_rest(4),
        "p5": prm_rest(5),
        "x1": (x_hbm.at[X0:X1], xb.at[X0:X1]),
        "fi": (fi_hbm, fi),
        "fk": (fk_hbm, fk),
        "ua": (u_hbm.at[:, 0:256], ub.at[:, 0:256]),
        "x2": (x_hbm.at[X1:S], xb.at[X1:S]),
        "ub": (u_hbm.at[:, 256:D], ub.at[:, 256:D]),
        "wv": (w_hbm.at[:, 2 * D:3 * D], wb.at[:, 2 * D:3 * D]),
        "wo": (wo_hbm, wob),
    })
    cin = {k: pltpu.make_async_copy(a, b, sem_in.at[i]) for i, (k, (a, b)) in enumerate(srcs.items())}
    for c in cin.values():
        c.start()
    couts = []

    def wait(*names):
        for n in names:
            cin[n].wait()

    def out_copy(i, kind, a, b):
        if kind == "a":
            return pltpu.make_async_copy(sta.at[a * 64:b * 64], o_hbm.at[a * 64:b * 64, 0:D], sem_out.at[i])
        c0 = D + kind * 128
        return pltpu.make_async_copy(stb.at[kind, a * 128:b * 128],
                                     o_hbm.at[a * 128:b * 128, c0:c0 + 128], sem_out.at[i])

    def store(*box):
        out_copy(len(couts), *box).start()
        couts.append(box)

    q0, q1 = X0 // 64, X1 // 64
    p0, p1 = X0 // 128, X1 // 128
    qe = q_pieces(q1, q1 + 3)
    mid1, mid2, midz = mid_pieces()
    gps = g_pieces()
    gs = []
    for fb in range(8):
        blk = gps[fb * 16:(fb + 1) * 16]
        if fb:
            blk = blk[:4] + [mid1[fb - 1]] + blk[4:9] + [mid2[fb - 1]] + blk[9:]
        gs += blk
    kds = [kdft_pieces(j, 20 if j >= 2 else 0) for j in range(4)]
    uds = [udft_pieces(j) for j in range(4)]
    cv = [[(p, 0, 4) for p in range(32)],
          [(p, 0, 4) for p in range(32, 48)],
          [(p, 0, 3) for p in range(48, 64)] + [(p, 3, 4) for p in range(48, C3)],
          [(p, 3, 4) for p in range(C3, 64)]]
    oseg = o_stream(0, O3, q1 + 3)
    oseg2 = o_stream(O3, 32, O3)

    main3 = uds[0][:8] + [(k0_all, 8, 0)] + uds[0][8:] + kds[0] + uds[1][:10] + kds[1] + uds[1][10:]
    blk3 = main3[:1] + _merge(main3[1:-3], kgen_pieces(G0, 64)) + main3[-3:]
    ql = q_pieces(q0 - 1, q0)
    u23 = uds[2] + uds[3]
    blk4 = u23[:2]
    for n, pb in enumerate(range(p1, 16)):
        kp = kt_pieces(pb, pb + 1)
        blk4 += kp[:2] + [u23[2 + n]] + kp[2:]
    nu = 2 + 16 - p1
    blk4 += u23[nu:nu + 3] + _merge(gs[:GS], midz + kds[2] + kds[3], u23[nu + 3:])
    blk5 = _merge(gs[GS:] + qe[:4] + [mid1[7]] + oseg(-2, 0) + qe[4:8] + [mid2[7]] + qe[8:] + oseg(0, O1),
                  inv_pieces(0) + inv_pieces(1))
    blk5 = [(f, c, v + (50 if 8 <= i < 32 else 0)) for i, (f, c, v) in enumerate(blk5)]
    last = oseg2(O4, 32)
    ta = oseg2(O3, O4)
    blk8 = oseg2(O3 - 2, O3) + ta[:-5] + inv_pieces(3)[6:] + [p for p in last if p[1] == 0] + ta[-5:]
    blk9 = [p for p in last if p[1] != 0]

    steps = [
        (lambda: wait("ldt"), setup_dt_first),
        (lambda: wait("a0", "a1", "a2", "a3", "a4", "a5"), early_prep),
        (early_exact, lambda: _emit(kgen_pieces(0, G0))),
        (lambda: wait("wq", "x0", "dsk"),
         lambda: (setup_dt_rest(), wq_perm_a(), _emit(q_pieces(0, q0 - 1)))),
        (lambda: wait("p0", "p1", "wk"),
         lambda: (wk_transpose(), range_check(0, R0, D),
                  _emit(ql[:3] + kt_pieces(0, p0, True), stage1(), (32 - G0 // 2) * 90, tail=130))),
        (lambda: (stage1_exact(), wait("p2", "p3", "p4", "p5", "x1")),
         lambda: (wq_perm_b(),
                  _emit(ql[3:] + kt_pieces(p0, p1) + q_pieces(q0, q1), stage2_fill(G0 // 2, 32), (32 - G0 // 2) * 164))),
        (lambda: wait("fi", "fk", "ua"), lambda: (setup_g(), _emit(blk3))),
        (lambda: wait("x2", "ub", "wv", "wo"), lambda: _emit(blk4, conv(cv[0]), conv_ops(cv[0]), 3.6)),
        (None, lambda: _emit(blk5, conv(cv[1]), conv_ops(cv[1]), 3.7)),
        (lambda: (store(0, 0, 16), store(1, 0, 16), store("a", 0, O1)),
         lambda: _emit(_merge(oseg(O1, O2), inv_pieces(2)), conv(cv[2]), conv_ops(cv[2]), 3.5)),
        (lambda: (store(2, 0, 16), store("a", O1, O2)),
         lambda: _emit(_merge(oseg(O2, O3), inv_pieces(3)[:6]), conv(cv[3]), conv_ops(cv[3]), 3.4)),
        (lambda: (store(3, 0, 12), store("a", O2, O3)), lambda: _emit(blk8)),
        (lambda: (store(3, 12, 16), store("a", O3, O4)), lambda: _emit(blk9)),
        (lambda: store("a", O4, 32), None),
    ]

    def outer(i, c):
        packed.clear()
        couts.clear()
        for k in range(len(steps) - 1):
            @pl.when(i + k == k)
            def _():
                steps[k][1]()
                if steps[k + 1][0] is not None:
                    steps[k + 1][0]()
        return c

    steps[0][0]()
    lax.fori_loop(0, 2, outer, 0)
    for i, box in enumerate(couts):
        out_copy(i, *box).wait()


@jax.jit
def pallas_concat_heads__linear_attn_block__ssm_conv_s4__prompt_kernel(
    A_x, A_wqkv, A_wo, B_u, B_A_re, B_A_im, B_B_re, B_B_im, B_C_re, B_C_im, B_log_dt, B_Dskip,
):
    fk, fi = _tables()
    V = pltpu.VMEM
    params = dict(vmem_limit_bytes=110 * 2**20)
    if hasattr(pltpu.CompilerParams, "disable_semaphore_checks"):
        params["disable_semaphore_checks"] = True
    out = pl.pallas_call(
        _kernel,
        out_shape=jax.ShapeDtypeStruct((S, 2 * D), BF16),
        in_specs=[pl.BlockSpec(memory_space=pl.ANY)] * 14,
        out_specs=pl.BlockSpec(memory_space=pl.ANY),
        scratch_shapes=[
            V((S // 2, D), U32),
            V((D, 3 * D), BF16),
            V((D, D), BF16),
            V((S // 2, D), U32),
            V((6, D, 128), BF16),
            V((D,), BF16),
            V((D,), BF16),
            V((S, D), BF16),
            V((S, D), BF16),
            V((FK_ROWS // 2, 128), U32),
            V((136, 128), F32),
            V((S, D), BF16),
            V((4, S, 128), BF16),
            V((2, D, 128), F32),
            pltpu.SMEM((2,), jnp.int32),
            V((D, 128), F32),
            V((8, 128, 128), F32),
            V((14, 2 * D + 8, 128), F32),
            V((D, 128), F32),
            V((5, D // 2, 128), U32),
            V((4, 2, 16, 128), F32),
            V((8, D), F32),
            V((4, 3, 16, 128, 128), F32),
            V((4, 3, 16, 128, 128), F32),
            V((4, 2, 16, 128, 128), F32),
            V((D // 2, D), U32),
            V((D // 2, S), U32),
            V((D, 128), F32),
            V((D // 2, D), U32),
            V((4, D // 2 + 8, 128), U32),
            V((4, 128, 128), F32),
            V((S, D), F32),
            V((S // 2, D), U32),
            V((4, D // 2 + 8, 128), U32),
            V((D // 2, D), U32),
            V((D // 2 + 8, 128), U32),
            V((16, D), F32),
            V((4, 12, 144, 128), F32),
            V((2, 128, 128), F32),
            pltpu.SemaphoreType.DMA((25,)),
            pltpu.SemaphoreType.DMA((10,)),
        ],
        compiler_params=pltpu.CompilerParams(**params),
    )(A_x.reshape(S, D), A_wqkv, A_wo, B_u.reshape(S, D), B_A_re, B_A_im, B_B_re, B_B_im, B_C_re, B_C_im,
      B_log_dt, B_Dskip, jnp.asarray(fk), jnp.asarray(fi))
    return out.reshape(1, S, 2 * D)
```
